```python
import jax
import jax.numpy as jnp

def _softmax(x, axis=-1):
    return jax.nn.softmax(x, axis=axis)

def _gelu(x):
    return jax.nn.gelu(x, approximate=True)

def _silu(x):
    return jax.nn.silu(x)

def _sigmoid(x):
    return jax.nn.sigmoid(x)

def _layernorm(x, axis=-1, eps=1e-05):
    m = jnp.mean(x, axis=axis, keepdims=True)
    v = jnp.var(x, axis=axis, keepdims=True)
    return (x - m) / jnp.sqrt(v + eps)

def _scatter_add(tgt, idx, src, axis=0):
    return tgt.at[idx].add(src)

def _segment_sum(src, seg, n):
    return jax.ops.segment_sum(src, seg, n)

class _Rng:

    def __init__(self, key):
        self._k = key

    def _next(self):
        self._k, sub = jax.random.split(self._k)
        return sub

    def normal(self, shape):
        return jax.random.normal(self._next(), shape, dtype=jnp.bfloat16)

    def randint(self, lo, hi, shape):
        return jax.random.randint(self._next(), shape, lo, hi, dtype=jnp.int32)

    def uniform(self, shape, lo=0.0, hi=1.0):
        return jax.random.uniform(self._next(), shape, jnp.bfloat16, lo, hi)

    def permutation(self, n):
        return jax.random.permutation(self._next(), n)
kernel_name = 'adaLN_cond__memory_aug_recurrent_mem_tr__glu_gated_swiglu__prompt'

def setup_inputs():
    _rng = _Rng(jax.random.key(int.from_bytes(__import__("os").urandom(4), "little")))
    _w = lambda a: (lambda t: t.astype(jnp.bfloat16) if jnp.issubdtype(t.dtype, jnp.floating) else t)(jnp.asarray(a))

    def _A_setup():
        B, S, Dm = (1, 2048, 1024)
        H, Dh = (32, 128)
        M, seg = (8, 32)
        seg = min(seg, S)
        S = S // seg * seg
        return {'x': _w((lambda *s: _rng.normal(s) * 0.05)(B, S, Dm)), 'mem0': _w((lambda *s: _rng.normal(s) * 0.05)(B, M, Dm)), 'Wq': _w((lambda *s: _rng.normal(s) * 0.05)(Dm, H, Dh) * Dm ** (-0.5)), 'Wk': _w((lambda *s: _rng.normal(s) * 0.05)(Dm, H, Dh) * Dm ** (-0.5)), 'Wv': _w((lambda *s: _rng.normal(s) * 0.05)(Dm, H, Dh) * Dm ** (-0.5)), 'Wo': _w((lambda *s: _rng.normal(s) * 0.05)(H, Dh, Dm) * (H * Dh) ** (-0.5)), 'seg_len': seg}
    _A_in = _A_setup()

    def _B_setup():
        B, S, D, F = (1, 2048, 1024, 3584)
        return {'x': _w((lambda *s: _rng.normal(s) * 0.05)(B, S, D)), 'w1': _w((lambda *s: _rng.normal(s) * 0.05)(D, F) * (2.0 / D) ** 0.5), 'w3': _w((lambda *s: _rng.normal(s) * 0.05)(D, F) * (2.0 / D) ** 0.5), 'w2': _w((lambda *s: _rng.normal(s) * 0.05)(F, D) * (2.0 / F) ** 0.5)}
    _B_in = _B_setup()
    return {'A_x': _A_in['x'], 'A_mem0': _A_in['mem0'], 'A_Wq': _A_in['Wq'], 'A_Wk': _A_in['Wk'], 'A_Wv': _A_in['Wv'], 'A_Wo': _A_in['Wo'], 'A_seg_len': _A_in['seg_len'], 'B_x': _B_in['x'], 'B_w1': _B_in['w1'], 'B_w3': _B_in['w3'], 'B_w2': _B_in['w2'], 'c': _w((lambda *s: _rng.normal(s) * 0.05)(1, 1024)), 'w_mod': _w((lambda *s: _rng.normal(s) * 0.05)(1024, 6 * 1024) * 1024 ** (-0.5))}

def reference(A_x, A_mem0, A_Wq, A_Wk, A_Wv, A_Wo, A_seg_len, B_x, B_w1, B_w3, B_w2, c, w_mod):

    def _A_ref(x, mem0, Wq, Wk, Wv, Wo, seg_len):
        B, S, Dm = x.shape
        H, Dh = (Wq.shape[1], Wq.shape[2])
        M = mem0.shape[1]
        scale = Dh ** (-0.5)
        n_seg = S // seg_len
        L = M + seg_len
        idx = jnp.arange(L)
        mask = (idx[:, None] < M) | (idx[:, None] >= idx[None, :])
        mem = mem0
        outs = []
        for s in range(n_seg):
            xs = x[:, s * seg_len:(s + 1) * seg_len, :].copy()
            h = jnp.concatenate([mem, xs], axis=1)
            q = jnp.einsum('btd,dhe->bhte', h, Wq)
            k = jnp.einsum('btd,dhe->bhte', h, Wk)
            v = jnp.einsum('btd,dhe->bhte', h, Wv)
            scores = jnp.einsum('bhqe,bhke->bhqk', q, k) * scale
            scores = jnp.where(mask[None, None], scores, -1000000000.0)
            p = _softmax(scores, axis=-1)
            o = jnp.einsum('bhqk,bhke->bhqe', p, v)
            o = jnp.einsum('bhte,hed->btd', o, Wo)
            mem = o[:, :M, :].copy()
            outs.append(o[:, M:, :])
        return jnp.concatenate(outs, axis=1)

    def _B_ref(x, w1, w3, w2):
        gate = jnp.einsum('bsd,df->bsf', x, w1)
        up = jnp.einsum('bsd,df->bsf', x, w3)
        h = _silu(gate) * up
        out = jnp.einsum('bsf,fd->bsd', h, w2)
        return out
    x = A_x
    mod = (_silu(c) @ w_mod).reshape(c.shape[0], 6, 1, -1)
    sa, ca, ga, sb, cb, gb = (mod[:, 0].copy(), mod[:, 1].copy(), mod[:, 2].copy(), mod[:, 3].copy(), mod[:, 4].copy(), mod[:, 5].copy())
    h = _layernorm(x, axis=-1) * (1 + ca) + sa
    x = x + ga * _A_ref(h, A_mem0, A_Wq, A_Wk, A_Wv, A_Wo, A_seg_len)
    h = _layernorm(x, axis=-1) * (1 + cb) + sb
    x = x + gb * _B_ref(h, B_w1, B_w3, B_w2)
    return x
```

```python
import functools

import jax
import jax.numpy as jnp
from jax import lax
import jax.experimental.pallas as pl
import jax.experimental.pallas.tpu as pltpu

F32, BF16, U32 = jnp.float32, jnp.bfloat16, jnp.uint32
_NN = (((1,), (0,)), ((), ()))
_NT = (((1,), (1,)), ((), ()))


def _dot(a, b, dims=_NN):
    return lax.dot_general(a, b, dims, preferred_element_type=F32)


def _layernorm(x, eps=1e-5):
    m = jnp.mean(x, axis=-1, keepdims=True)
    d = x - m
    v = jnp.mean(d * d, axis=-1, keepdims=True)
    return d * lax.rsqrt(v + eps)


def _silu(x):
    return x / (1.0 + jnp.exp(-x))


def _body(x_hbm, mem0_ref, wq_hbm, wk_hbm, wv_hbm, wo_hbm, w1_hbm, w3_hbm, w2_hbm,
          c_ref, wm_hbm, out_hbm,
          wq32, wk32, wv32, wo32, x_v, h_v, mod_v, hs_v, o_v, att_v, sems,
          *, S, D, H, Dh, M, T, F, G, BM, FC):
    n_seg = S // T
    L = M + T
    HD = H * Dh
    KC = 128
    n_kc = D // KC

    def startup(wm_v, raw, raw_o, sem_m, sem_w, sem_o):
        cp_m = [pltpu.make_async_copy(wm_hbm.at[:, pl.ds(j * 2 * D, 2 * D)], wm_v.at[j], sem_m.at[j])
                for j in range(3)]
        cp_x = pltpu.make_async_copy(x_hbm, x_v, sems.at[0])
        srcs = (wq_hbm, wk_hbm, wv_hbm)
        cp_w = [[pltpu.make_async_copy(srcs[t].at[pl.ds(c * KC * H, KC * H)], raw.at[t * n_kc + c],
                                       sem_w.at[t * n_kc + c]) for c in range(n_kc)] for t in range(3)]
        cp_o = pltpu.make_async_copy(wo_hbm, raw_o, sem_o.at[0])
        cp_m[0].start()
        cp_x.start()
        for t in range(3):
            for c in range(n_kc):
                cp_w[t][c].start()
        cp_o.start()
        cp_m[1].start()
        cp_m[2].start()

        sc = _silu(c_ref[...].astype(F32))
        sc = jnp.broadcast_to(sc, (8, D)).astype(BF16)
        cp_m[0].wait()
        mod_v[:, 0:2 * D] = _dot(sc, wm_v[0])
        cp_x.wait()

        def ln_body(i, carry):
            r = pl.ds(pl.multiple_of(i * 128, 128), 128)
            h = _layernorm(x_v[r, :].astype(F32)) * (1.0 + mod_v[0:1, D:2 * D]) + mod_v[0:1, 0:D]
            h_v[r, :] = h.astype(BF16)
            return carry
        lax.fori_loop(0, S // 128, ln_body, 0)

        raw32 = raw.bitcast(U32)
        for t, dst in enumerate((wq32, wk32, wv32)):
            def relayout(c, carry, t=t, dst=dst):
                j = t * n_kc + c
                pltpu.make_async_copy(srcs[t].at[pl.ds(0, KC * H)], raw.at[j], sem_w.at[j]).wait()
                rows = pl.ds(pl.multiple_of(c * (KC // 2), KC // 2), KC // 2)
                for hp in range(H // 2):
                    a = raw32[j, pl.ds(hp, KC // 2, stride=H), :]
                    b = raw32[j, pl.ds(hp + H // 2, KC // 2, stride=H), :]
                    dst[rows, (2 * hp) * Dh:(2 * hp + 1) * Dh] = (a & 0xFFFF) | (b << 16)
                    dst[rows, (2 * hp + 1) * Dh:(2 * hp + 2) * Dh] = (a >> 16) | ((b >> 16) << 16)
                return carry
            lax.fori_loop(0, n_kc, relayout, 0)

        cp_o.wait()

        def copy_o(i, carry):
            src = pl.ds(pl.multiple_of(i * 256, 256), 256)
            dst = pl.ds(pl.multiple_of(i * 128, 128), 128)
            wo32[dst, :] = pltpu.bitcast(raw_o[src, :], U32)
            return carry
        lax.fori_loop(0, HD // 256, copy_o, 0)
        for j in (1, 2):
            cp_m[j].wait()
            mod_v[:, j * 2 * D:(j + 1) * 2 * D] = _dot(sc, wm_v[j])

    pl.run_scoped(startup,
                  pltpu.VMEM((3, D, 2 * D), BF16), pltpu.VMEM((3 * n_kc, KC * H, Dh), BF16),
                  pltpu.VMEM((HD, D), BF16),
                  pltpu.SemaphoreType.DMA((3,)), pltpu.SemaphoreType.DMA((3 * n_kc,)),
                  pltpu.SemaphoreType.DMA((1,)))

    def main(w1_v, w3_v, w2_v, x1_v, y_v, sem_f, sem_y):
        cp_f = [pltpu.make_async_copy(s, d, sem_f.at[i])
                for i, (s, d) in enumerate(((w1_hbm, w1_v), (w3_hbm, w3_v), (w2_hbm, w2_v)))]
        for cp in cp_f:
            cp.start()

        def post(seg):
            r = pl.ds(pl.multiple_of(seg * T, T), T)
            x1 = x_v[r, :].astype(F32) + mod_v[0:1, 2 * D:3 * D] * att_v[...]
            x1_v[r, :] = x1
            h2 = _layernorm(x1) * (1.0 + mod_v[0:1, 4 * D:5 * D]) + mod_v[0:1, 3 * D:4 * D]
            return r, h2.astype(BF16)

        hs_v[0:M, :] = mem0_ref[...].astype(F32)
        hs_v[M:L, :] = h_v[0:T, :].astype(F32)
        att_v[...] = jnp.zeros(att_v.shape, F32)
        scale = Dh ** -0.5
        n_g = H // G

        def step(s, carry):
            ri = lax.broadcasted_iota(jnp.int32, (2 * L, 2 * L), 0)
            ci = lax.broadcasted_iota(jnp.int32, (2 * L, 2 * L), 1)
            same = (ri >= L) == (ci >= L)
            rl = jnp.where(ri >= L, ri - L, ri)
            cl = jnp.where(ci >= L, ci - L, ci)
            keep = same & ((rl < M) | (rl >= cl))
            fill = jnp.where(same, -1e9, -jnp.inf).astype(F32)

            def stack(a, p):
                return jnp.concatenate([a[:, (2 * p) * Dh:(2 * p + 1) * Dh],
                                        a[:, (2 * p + 1) * Dh:(2 * p + 2) * Dh]], axis=0)

            def proj(g):
                cols = slice(g * G * Dh, (g + 1) * G * Dh)
                return [_dot(hs_v[...], pltpu.bitcast(w[:, cols], BF16)) for w in (wq32, wk32, wv32)]

            def scores(qkv):
                q, k, v = qkv
                res = []
                for p in range(G // 2):
                    sc = _dot(stack(q, p), stack(k, p).astype(BF16), _NT) * scale
                    sc = jnp.where(keep, sc, fill)
                    e = jnp.exp(sc - jnp.max(sc, axis=-1, keepdims=True))
                    res.append((e, 1.0 / jnp.sum(e, axis=-1, keepdims=True), stack(v, p).astype(BF16)))
                return res

            def values(g, res):
                for p, (e, inv, v) in enumerate(res):
                    o = _dot(e, v) * inv
                    h0 = g * G + 2 * p
                    o_v[:, h0 * Dh:(h0 + 1) * Dh] = o[0:L]
                    o_v[:, (h0 + 1) * Dh:(h0 + 2) * Dh] = o[L:2 * L]

            def outp(g0, g1):
                return _dot(o_v[:, g0 * G * Dh:g1 * G * Dh],
                            pltpu.bitcast(wo32[g0 * G * Dh // 2:g1 * G * Dh // 2, :], BF16))

            r_prev, h2_prev = post(jnp.maximum(s - 1, 0))
            qkv, sm = {}, {}
            for g in range(n_g):
                qkv[g] = proj(g)
                if g >= 1:
                    sm[g - 1] = scores(qkv.pop(g - 1))
                if g >= 2:
                    values(g - 2, sm.pop(g - 2))
            half = (n_g - 2) // 2
            acc = outp(0, half)
            sm[n_g - 1] = scores(qkv.pop(n_g - 1))
            values(n_g - 2, sm.pop(n_g - 2))
            acc = acc + outp(half, n_g - 2)
            values(n_g - 1, sm.pop(n_g - 1))
            acc = acc + outp(n_g - 2, n_g - 1)
            acc = acc + outp(n_g - 1, n_g)
            nxt = pl.ds(pl.multiple_of(jnp.minimum(s + 1, n_seg - 1) * T, T), T)
            hs_v[0:M, :] = acc[0:M]
            hs_v[M:L, :] = h_v[nxt, :].astype(F32)
            att_v[...] = acc[M:L]
            h_v[r_prev, :] = h2_prev
            return carry

        lax.fori_loop(0, n_seg, step, 0)
        r_last, h2_last = post(n_seg - 1)
        h_v[r_last, :] = h2_last

        for cp in cp_f:
            cp.wait()

        def out_copy(i):
            r = pl.ds(pl.multiple_of(i * BM, BM), BM)
            return pltpu.make_async_copy(y_v.at[r], out_hbm.at[r], sem_y.at[i])

        def ffn(i, carry):
            r = pl.ds(pl.multiple_of(i * BM, BM), BM)
            h2 = h_v[r, :]
            acc = None
            for f in range(F // FC):
                cols = slice(f * FC, (f + 1) * FC)
                a = (_silu(_dot(h2, w1_v[:, cols])) * _dot(h2, w3_v[:, cols])).astype(BF16)
                d = _dot(a, w2_v[cols, :])
                acc = d if acc is None else acc + d
            y_v[r, :] = (x1_v[r, :] + mod_v[0:1, 5 * D:6 * D] * acc).astype(y_v.dtype)
            out_copy(i).start()
            return carry

        lax.fori_loop(0, S // BM, ffn, 0)
        for i in range(S // BM):
            out_copy(i).wait()

    pl.run_scoped(main,
                  pltpu.VMEM((D, F), BF16), pltpu.VMEM((D, F), BF16), pltpu.VMEM((F, D), BF16),
                  pltpu.VMEM((S, D), F32), pltpu.VMEM((S, D), out_hbm.dtype),
                  pltpu.SemaphoreType.DMA((3,)), pltpu.SemaphoreType.DMA((S // BM,)))


@functools.partial(jax.jit, static_argnames=("A_seg_len",))
def pallas_adaLN_cond__memory_aug_recurrent_mem_tr__glu_gated_swiglu__prompt_kernel(
    A_x, A_mem0, A_Wq, A_Wk, A_Wv, A_Wo, A_seg_len, B_x, B_w1, B_w3, B_w2, c, w_mod,
):
    del B_x
    B, S, D = A_x.shape
    _, H, Dh = A_Wq.shape
    M, T, F = A_mem0.shape[1], int(A_seg_len), B_w1.shape[1]
    assert B == 1 and S % T == 0
    L, HD = M + T, H * Dh
    hbm = pl.BlockSpec(memory_space=pl.ANY)
    vmem = pl.BlockSpec(memory_space=pltpu.VMEM)
    body = functools.partial(_body, S=S, D=D, H=H, Dh=Dh, M=M, T=T, F=F, G=4, BM=256, FC=512)
    out = pl.pallas_call(
        body,
        out_shape=jax.ShapeDtypeStruct((S, D), A_x.dtype),
        in_specs=[hbm, vmem, hbm, hbm, hbm, hbm, hbm, hbm, hbm, vmem, hbm],
        out_specs=hbm,
        scratch_shapes=[
            pltpu.VMEM((D // 2, HD), U32), pltpu.VMEM((D // 2, HD), U32), pltpu.VMEM((D // 2, HD), U32),
            pltpu.VMEM((HD // 2, D), U32),
            pltpu.VMEM((S, D), A_x.dtype), pltpu.VMEM((S, D), BF16), pltpu.VMEM((8, 6 * D), F32),
            pltpu.VMEM((L, D), F32), pltpu.VMEM((L, HD), F32), pltpu.VMEM((T, D), F32),
            pltpu.SemaphoreType.DMA((1,)),
        ],
        compiler_params=pltpu.CompilerParams(vmem_limit_bytes=120 * 2**20),
    )(A_x.reshape(S, D), A_mem0.reshape(M, D),
      A_Wq.reshape(D * H, Dh), A_Wk.reshape(D * H, Dh), A_Wv.reshape(D * H, Dh), A_Wo.reshape(HD, D),
      B_w1, B_w3, B_w2, c, w_mod)
    return out.reshape(B, S, D)
```

```python
import functools

import jax
import jax.numpy as jnp
from jax import lax
import jax.experimental.pallas as pl
import jax.experimental.pallas.tpu as pltpu

F32, BF16, U32 = jnp.float32, jnp.bfloat16, jnp.uint32
_NN = (((1,), (0,)), ((), ()))
_NT = (((1,), (1,)), ((), ()))


def _dot(a, b, dims=_NN):
    return lax.dot_general(a, b, dims, preferred_element_type=F32)


def _layernorm(x, eps=1e-5):
    m = jnp.mean(x, axis=-1, keepdims=True)
    d = x - m
    v = jnp.mean(d * d, axis=-1, keepdims=True)
    return d * lax.rsqrt(v + eps)


def _silu(x):
    return x / (1.0 + jnp.exp(-x))


def _body(x_hbm, mem0_ref, wq_hbm, wk_hbm, wv_hbm, wo_hbm, w1_hbm, w3_hbm, w2_hbm,
          c_ref, wm_hbm, out_hbm,
          wq32, wk32, wv32, wo32, pq_v, pk_v, x_v, mod_v, hs_v, o_v, sems,
          *, S, D, H, Dh, M, T, F, G, BM, FC):
    n_seg = S // T
    L = M + T
    HD = H * Dh
    P = 8
    KC = 128
    n_kc = D // KC
    OC = HD // 2 // n_kc
    wo_src = wo_hbm.bitcast(U32)
    cp_x = pltpu.make_async_copy(x_hbm, x_v, sems.at[0])

    def silu_c():
        return jnp.broadcast_to(_silu(c_ref[...].astype(F32)), (8, D)).astype(BF16)

    def ada1(x):
        return _layernorm(x.astype(F32)) * (1.0 + mod_v[0:1, D:2 * D]) + mod_v[0:1, 0:D]

    def startup(wm_v, raw, xp_v, hp_v, sem_m, sem_w, sem_p):
        srcs = (wq_hbm, wk_hbm, wv_hbm)

        def cp_w(t, c):
            if t == 3:
                r = pl.ds(pl.multiple_of(c * OC, OC), OC)
                return pltpu.make_async_copy(wo_src.at[r], wo32.at[r], sem_w.at[3 * n_kc + c])
            r = pl.ds(pl.multiple_of(c * (KC * H), KC * H), KC * H)
            return pltpu.make_async_copy(srcs[t].at[r], raw.at[t * n_kc + c], sem_w.at[t * n_kc + c])

        n_m = 4
        mr = D // n_m
        cp_m = [pltpu.make_async_copy(wm_hbm.at[pl.ds(j * mr, mr), pl.ds(0, 2 * D)], wm_v.at[j], sem_m.at[j])
                for j in range(n_m)]
        cp_p = pltpu.make_async_copy(x_hbm.at[:, pl.ds(T - P, P), :], xp_v, sem_p.at[0])
        cp_p.start()
        for cp in cp_m:
            cp.start()
        cp_w(0, 0).start()

        def zero(i, carry):
            r = pl.ds(pl.multiple_of(i * 32, 32), 32)
            pq_v[r, :] = jnp.zeros((32, HD), F32)
            pk_v[r, :] = jnp.zeros((32, HD), F32)
            return carry
        lax.fori_loop(0, n_seg * P // 32, zero, 0)

        sc = silu_c()
        cp_p.wait()
        xn = _layernorm(xp_v[...].astype(F32).reshape(n_seg * P, D))
        mod = None
        for j in range(n_m):
            cp_m[j].wait()
            if j < 2:
                cp_w(0, j + 1).start()
            d = _dot(sc[:, j * mr:(j + 1) * mr], wm_v[j])
            mod = d if mod is None else mod + d
        mod_v[:, 0:2 * D] = mod
        hp = (xn * (1.0 + mod[0:1, D:2 * D]) + mod[0:1, 0:D]).astype(BF16)
        for c in range(n_kc):
            hp_v[c] = hp[:, c * KC:(c + 1) * KC]

        raw32 = raw.bitcast(U32)

        def retile(t, c, dst, pre):
            j = t * n_kc + c
            rows = pl.ds(pl.multiple_of(c * (KC // 2), KC // 2), KC // 2)
            for h4 in range(H // 4):
                tiles = []
                for hp2 in (2 * h4, 2 * h4 + 1):
                    a = raw32[j, pl.ds(hp2, KC // 2, stride=H), :]
                    b = raw32[j, pl.ds(hp2 + H // 2, KC // 2, stride=H), :]
                    tiles += [(a & 0xFFFF) | (b << 16), (a >> 16) | ((b >> 16) << 16)]
                w = jnp.concatenate(tiles, axis=1)
                cols = slice(4 * h4 * Dh, 4 * (h4 + 1) * Dh)
                dst[rows, cols] = w
                if pre is not None:
                    pre[:, cols] += _dot(hp_v[c], pltpu.bitcast(w, BF16))

        order = ([(0, c) for c in range(n_kc)] + [(t, c) for c in range(n_kc) for t in (1, 2)]
                 + [(3, c) for c in range(n_kc)])

        def issue(i, base):
            for it in range(n_kc):
                todo = order[3 + 2 * (base + it):5 + 2 * (base + it)]
                if todo:
                    @pl.when(i == it)
                    def _(todo=todo):
                        for t, c in todo:
                            cp_w(t, c).start()

        def q_phase(c, carry):
            cp_w(0, c).wait()
            issue(c, 0)
            retile(0, c, wq32, pq_v)
            return carry
        lax.fori_loop(0, n_kc, q_phase, 0)

        def k_phase(c, carry):
            cp_w(1, c).wait()
            cp_w(2, c).wait()
            issue(c, n_kc)

            @pl.when(c == n_kc - 2)
            def _():
                cp_x.start()
            retile(1, c, wk32, pk_v)
            retile(2, c, wv32, None)
            return carry
        lax.fori_loop(0, n_kc, k_phase, 0)
        for c in range(n_kc):
            cp_w(3, c).wait()

    pl.run_scoped(startup,
                  pltpu.VMEM((4, D // 4, 2 * D), BF16), pltpu.VMEM((3 * n_kc, KC * H, Dh), BF16),
                  pltpu.VMEM((n_seg, P, D), x_hbm.dtype), pltpu.VMEM((n_kc, n_seg * P, KC), BF16),
                  pltpu.SemaphoreType.DMA((4,)), pltpu.SemaphoreType.DMA((4 * n_kc,)),
                  pltpu.SemaphoreType.DMA((1,)))

    def main(w1_v, w3_v, w2_v, wm_v, att_v, h2_v, y_v, sem_f, sem_y):
        cp_f = [pltpu.make_async_copy(s, d, sem_f.at[i]) for i, (s, d) in enumerate((
            (wm_hbm.at[:, pl.ds(2 * D, 4 * D)], wm_v), (w1_hbm, w1_v), (w3_hbm, w3_v), (w2_hbm, w2_v)))]
        cp_x.wait()
        for cp in cp_f:
            cp.start()
        hs_v[0:M, :] = mem0_ref[...].astype(F32)
        hs_v[M:L, :] = ada1(x_v[0])
        scale = Dh ** -0.5
        n_g = H // G

        def step(s, carry):
            ri = lax.broadcasted_iota(jnp.int32, (2 * L, 2 * L), 0)
            ci = lax.broadcasted_iota(jnp.int32, (2 * L, 2 * L), 1)
            same = (ri >= L) == (ci >= L)
            rl = jnp.where(ri >= L, ri - L, ri)
            cl = jnp.where(ci >= L, ci - L, ci)
            keep = same & ((rl < M) | (rl >= cl))
            fill = jnp.where(same, -1e9, -jnp.inf).astype(F32)

            def stack(a, p):
                return jnp.concatenate([a[:, (2 * p) * Dh:(2 * p + 1) * Dh],
                                        a[:, (2 * p + 1) * Dh:(2 * p + 2) * Dh]], axis=0)

            early = pl.ds(pl.multiple_of(s * P, P), P)

            def proj(g):
                cols = slice(g * G * Dh, (g + 1) * G * Dh)
                q, k = [jnp.concatenate([_dot(hs_v[0:L - P, :], pltpu.bitcast(w[:, cols], BF16)),
                                         pre[early, cols]], axis=0)
                        for w, pre in ((wq32, pq_v), (wk32, pk_v))]
                return q, k, _dot(hs_v[...], pltpu.bitcast(wv32[:, cols], BF16))

            def scores(qkv):
                q, k, v = qkv
                res = []
                for p in range(G // 2):
                    sc = _dot(stack(q, p), stack(k, p).astype(BF16), _NT) * scale
                    sc = jnp.where(keep, sc, fill)
                    e = jnp.exp(sc - jnp.max(sc, axis=-1, keepdims=True))
                    res.append((e, 1.0 / jnp.sum(e, axis=-1, keepdims=True), stack(v, p).astype(BF16)))
                return res

            def values(g, res):
                for p, (e, inv, v) in enumerate(res):
                    o = _dot(e, v) * inv
                    h0 = g * G + 2 * p
                    o_v[:, h0 * Dh:(h0 + 1) * Dh] = o[0:L]
                    o_v[:, (h0 + 1) * Dh:(h0 + 2) * Dh] = o[L:2 * L]

            def outp(g0, g1):
                return _dot(o_v[:, g0 * G * Dh:g1 * G * Dh],
                            pltpu.bitcast(wo32[g0 * G * Dh // 2:g1 * G * Dh // 2, :], BF16))

            h_next = ada1(x_v[jnp.minimum(s + 1, n_seg - 1)])
            qkv, sm = {}, {}
            for g in range(n_g):
                qkv[g] = proj(g)
                if g >= 1:
                    sm[g - 1] = scores(qkv.pop(g - 1))
                if g >= 2:
                    values(g - 2, sm.pop(g - 2))
            half = (n_g - 2) // 2
            acc = outp(0, half)
            sm[n_g - 1] = scores(qkv.pop(n_g - 1))
            values(n_g - 2, sm.pop(n_g - 2))
            acc = acc + outp(half, n_g - 2)
            values(n_g - 1, sm.pop(n_g - 1))
            acc = acc + outp(n_g - 2, n_g - 1)
            acc = acc + outp(n_g - 1, n_g)
            hs_v[0:M, :] = acc[0:M]
            hs_v[M:L, :] = h_next
            att_v[pl.ds(pl.multiple_of(s * T, T), T), :] = acc[M:L]
            return carry

        lax.fori_loop(0, n_seg, step, 0)

        for cp in cp_f:
            cp.wait()
        mod_v[:, 2 * D:6 * D] = _dot(silu_c(), wm_v[...])

        def resid(i):
            x = x_v[pl.ds(i * (BM // T), BM // T)].astype(F32).reshape(BM, D)
            return x + mod_v[0:1, 2 * D:3 * D] * att_v[pl.ds(pl.multiple_of(i * BM, BM), BM), :]

        def ada2(i):
            h2 = _layernorm(resid(i)) * (1.0 + mod_v[0:1, 4 * D:5 * D]) + mod_v[0:1, 3 * D:4 * D]
            return h2.astype(BF16)

        h2_v[...] = ada2(0)

        def out_copy(i):
            r = pl.ds(pl.multiple_of(i * BM, BM), BM)
            return pltpu.make_async_copy(y_v.at[r], out_hbm.at[r], sem_y.at[i])

        def ffn(i, carry):
            r = pl.ds(pl.multiple_of(i * BM, BM), BM)
            h2 = h2_v[...]
            h2_next = ada2(jnp.minimum(i + 1, S // BM - 1))
            acc = None
            for f in range(F // FC):
                cols = slice(f * FC, (f + 1) * FC)
                a = (_silu(_dot(h2, w1_v[:, cols])) * _dot(h2, w3_v[:, cols])).astype(BF16)
                d = _dot(a, w2_v[cols, :])
                acc = d if acc is None else acc + d
            y_v[r, :] = (resid(i) + mod_v[0:1, 5 * D:6 * D] * acc).astype(y_v.dtype)
            h2_v[...] = h2_next
            out_copy(i).start()
            return carry

        lax.fori_loop(0, S // BM, ffn, 0)
        for i in range(S // BM):
            out_copy(i).wait()

    pl.run_scoped(main,
                  pltpu.VMEM((D, F), BF16), pltpu.VMEM((D, F), BF16), pltpu.VMEM((F, D), BF16),
                  pltpu.VMEM((D, 4 * D), BF16), pltpu.VMEM((S, D), F32), pltpu.VMEM((BM, D), BF16),
                  pltpu.VMEM((S, D), out_hbm.dtype),
                  pltpu.SemaphoreType.DMA((4,)), pltpu.SemaphoreType.DMA((S // BM,)))


@functools.partial(jax.jit, static_argnames=("A_seg_len",))
def pallas_adaLN_cond__memory_aug_recurrent_mem_tr__glu_gated_swiglu__prompt_kernel(
    A_x, A_mem0, A_Wq, A_Wk, A_Wv, A_Wo, A_seg_len, B_x, B_w1, B_w3, B_w2, c, w_mod,
):
    del B_x
    B, S, D = A_x.shape
    _, H, Dh = A_Wq.shape
    M, T, F = A_mem0.shape[1], int(A_seg_len), B_w1.shape[1]
    assert B == 1 and S % T == 0
    L, HD = M + T, H * Dh
    hbm = pl.BlockSpec(memory_space=pl.ANY)
    vmem = pl.BlockSpec(memory_space=pltpu.VMEM)
    body = functools.partial(_body, S=S, D=D, H=H, Dh=Dh, M=M, T=T, F=F, G=4, BM=256, FC=512)
    out = pl.pallas_call(
        body,
        out_shape=jax.ShapeDtypeStruct((S, D), A_x.dtype),
        in_specs=[hbm, vmem, hbm, hbm, hbm, hbm, hbm, hbm, hbm, vmem, hbm],
        out_specs=hbm,
        scratch_shapes=[
            pltpu.VMEM((D // 2, HD), U32), pltpu.VMEM((D // 2, HD), U32), pltpu.VMEM((D // 2, HD), U32),
            pltpu.VMEM((HD // 2, D), U32),
            pltpu.VMEM((S // T * 8, HD), F32), pltpu.VMEM((S // T * 8, HD), F32),
            pltpu.VMEM((S // T, T, D), A_x.dtype), pltpu.VMEM((8, 6 * D), F32),
            pltpu.VMEM((L, D), F32), pltpu.VMEM((L, HD), F32),
            pltpu.SemaphoreType.DMA((1,)),
        ],
        compiler_params=pltpu.CompilerParams(vmem_limit_bytes=120 * 2**20),
    )(A_x.reshape(S // T, T, D), A_mem0.reshape(M, D),
      A_Wq.reshape(D * H, Dh), A_Wk.reshape(D * H, Dh), A_Wv.reshape(D * H, Dh), A_Wo.reshape(HD, D),
      B_w1, B_w3, B_w2, c, w_mod)
    return out.reshape(B, S, D)
```

```python
import functools

import jax
import jax.numpy as jnp
from jax import lax
import jax.experimental.pallas as pl
import jax.experimental.pallas.tpu as pltpu

F32, BF16, U32 = jnp.float32, jnp.bfloat16, jnp.uint32
_NN = (((1,), (0,)), ((), ()))
_NT = (((1,), (1,)), ((), ()))


def _dot(a, b, dims=_NN):
    return lax.dot_general(a, b, dims, preferred_element_type=F32)


def _layernorm(x, eps=1e-5):
    m = jnp.mean(x, axis=-1, keepdims=True)
    d = x - m
    v = jnp.mean(d * d, axis=-1, keepdims=True)
    return d * lax.rsqrt(v + eps)


def _silu(x):
    return x / (1.0 + jnp.exp(-x))


def _body(x_hbm, mem0_ref, wq_hbm, wk_hbm, wv_hbm, wo_hbm, w1_hbm, w3_hbm, w2_hbm,
          c_ref, wm_hbm, out_hbm,
          wq32, wk32, wv32, wo32, pq_v, pk_v, x_v, mod_v, hs_v, o_v, sems,
          *, S, D, H, Dh, M, T, F, G, BM, FC):
    n_seg = S // T
    L = M + T
    HD = H * Dh
    P = 8
    KC = 128
    n_kc = D // KC
    OC = HD // 2 // n_kc
    wo_src = wo_hbm.bitcast(U32)
    wm_src = wm_hbm.bitcast(U32)
    HP = H + 8
    XA = min(8, n_seg - 1)
    cp_x = pltpu.make_async_copy(x_hbm.at[pl.ds(0, XA)], x_v.at[pl.ds(0, XA)], sems.at[0])
    cp_x2 = pltpu.make_async_copy(x_hbm.at[pl.ds(XA, n_seg - XA)], x_v.at[pl.ds(XA, n_seg - XA)], sems.at[1])

    def silu_c():
        return jnp.broadcast_to(_silu(c_ref[...].astype(F32)), (8, D)).astype(BF16)

    def ada1(x):
        return _layernorm(x.astype(F32)) * (1.0 + mod_v[0:1, D:2 * D]) + mod_v[0:1, 0:D]

    def startup(wm_v, raw, xp_v, hp_v, sem_m, sem_w, sem_p):
        srcs = [w.bitcast(U32) for w in (wq_hbm, wk_hbm, wv_hbm)]

        def cp_w(t, c):
            if t == 3:
                r = pl.ds(pl.multiple_of(c * OC, OC), OC)
                return pltpu.make_async_copy(wo_src.at[r], wo32.at[r], sem_w.at[3 * n_kc + c])
            j = t * n_kc + c
            return pltpu.make_async_copy(srcs[t].at[pl.ds(c * (KC // 2), KC // 2)],
                                         raw.at[pl.ds(j * (KC // 2), KC // 2), pl.ds(0, H)], sem_w.at[j])

        n_m = 4
        mr = D // n_m
        cp_m = [pltpu.make_async_copy(wm_src.at[pl.ds(j * mr // 2, mr // 2), pl.ds(0, 2 * D)], wm_v.at[j], sem_m.at[j])
                for j in range(n_m)]
        cp_p = pltpu.make_async_copy(x_hbm.at[:, pl.ds(T - P, P), :], xp_v, sem_p.at[0])
        cp_p.start()
        for cp in cp_m:
            cp.start()
        cp_w(0, 0).start()

        def zero(i, carry):
            r = pl.ds(pl.multiple_of(i * 32, 32), 32)
            pq_v[r, :] = jnp.zeros((32, HD), F32)
            pk_v[r, :] = jnp.zeros((32, HD), F32)
            return carry
        lax.fori_loop(0, n_seg * P // 32, zero, 0)

        sc = silu_c()
        cp_p.wait()
        xn = _layernorm(xp_v[...].astype(F32).reshape(n_seg * P, D))
        mod = None
        for j in range(n_m):
            cp_m[j].wait()
            if j < 2:
                cp_w(0, j + 1).start()
            d = _dot(sc[:, j * mr:(j + 1) * mr], pltpu.bitcast(wm_v[j], BF16))
            mod = d if mod is None else mod + d
        mod_v[:, 0:2 * D] = mod
        hp = (xn * (1.0 + mod[0:1, D:2 * D]) + mod[0:1, 0:D]).astype(BF16)
        for c in range(n_kc):
            hp_v[c] = hp[:, c * KC:(c + 1) * KC]

        raw2 = raw.reshape(3 * D // 2 * HP, Dh)

        def retile(c, jobs):
            rows = pl.ds(pl.multiple_of(c * (KC // 2), KC // 2), KC // 2)
            for h4 in range(H // 4):
                for t, dst, pre in jobs:
                    tiles = []
                    for hp2 in (2 * h4, 2 * h4 + 1):
                        base = (t * n_kc + c) * (KC // 2 * HP) + hp2
                        a = raw2[pl.ds(base, KC // 2, stride=HP), :]
                        b = raw2[pl.ds(base + H // 2, KC // 2, stride=HP), :]
                        tiles += [(a & 0xFFFF) | (b << 16), (a >> 16) | ((b >> 16) << 16)]
                    w = jnp.concatenate(tiles, axis=1)
                    cols = slice(4 * h4 * Dh, 4 * (h4 + 1) * Dh)
                    dst[rows, cols] = w
                    if pre is not None:
                        pre[:, cols] += _dot(hp_v[c], pltpu.bitcast(w, BF16))

        order = ([(0, c) for c in range(n_kc)] + [(t, c) for c in range(n_kc) for t in (1, 2)]
                 + [(3, c) for c in range(n_kc)])

        def issue(i, base):
            for it in range(n_kc):
                todo = order[3 + 2 * (base + it):5 + 2 * (base + it)]
                if todo:
                    @pl.when(i == it)
                    def _(todo=todo):
                        for t, c in todo:
                            cp_w(t, c).start()

        def q_phase(c, carry):
            cp_w(0, c).wait()
            issue(c, 0)
            retile(c, [(0, wq32, pq_v)])
            return carry
        lax.fori_loop(0, n_kc, q_phase, 0)

        def k_phase(c, carry):
            cp_w(1, c).wait()
            cp_w(2, c).wait()
            issue(c, n_kc)

            @pl.when(c == n_kc - 2)
            def _():
                cp_x.start()
            retile(c, [(1, wk32, pk_v), (2, wv32, None)])
            return carry
        lax.fori_loop(0, n_kc, k_phase, 0)
        for c in range(n_kc):
            cp_w(3, c).wait()

    pl.run_scoped(startup,
                  pltpu.VMEM((4, D // 8, 2 * D), U32), pltpu.VMEM((3 * D // 2, HP, Dh), U32),
                  pltpu.VMEM((n_seg, P, D), x_hbm.dtype), pltpu.VMEM((n_kc, n_seg * P, KC), BF16),
                  pltpu.SemaphoreType.DMA((4,)), pltpu.SemaphoreType.DMA((4 * n_kc,)),
                  pltpu.SemaphoreType.DMA((1,)))

    def main(w1_v, w3_v, w2_v, wm_v, att_v, h2_v, y_v, sem_f, sem_y):
        cp_f = [pltpu.make_async_copy(s, d, sem_f.at[i]) for i, (s, d) in enumerate((
            (wm_src.at[:, pl.ds(2 * D, 4 * D)], wm_v), (w1_hbm, w1_v), (w3_hbm, w3_v), (w2_hbm, w2_v)))]
        cp_x.wait()
        cp_x2.start()
        hs_v[0:M, :] = mem0_ref[...].astype(F32)
        hs_v[M:L, :] = ada1(x_v[0])
        scale = Dh ** -0.5
        n_g = H // G

        def step(s, carry):
            @pl.when(s == XA - 1)
            def _():
                cp_x2.wait()
                for cp in cp_f:
                    cp.start()

            ri = lax.broadcasted_iota(jnp.int32, (2 * L, 2 * L), 0)
            ci = lax.broadcasted_iota(jnp.int32, (2 * L, 2 * L), 1)
            same = (ri >= L) == (ci >= L)
            rl = jnp.where(ri >= L, ri - L, ri)
            cl = jnp.where(ci >= L, ci - L, ci)
            keep = same & ((rl < M) | (rl >= cl))
            fill = jnp.where(same, -1e9, -jnp.inf).astype(F32)

            def stack(a, p):
                return jnp.concatenate([a[:, (2 * p) * Dh:(2 * p + 1) * Dh],
                                        a[:, (2 * p + 1) * Dh:(2 * p + 2) * Dh]], axis=0)

            early = pl.ds(pl.multiple_of(s * P, P), P)

            def proj(g):
                cols = slice(g * G * Dh, (g + 1) * G * Dh)
                q, k = [jnp.concatenate([_dot(hs_v[0:L - P, :], pltpu.bitcast(w[:, cols], BF16)),
                                         pre[early, cols]], axis=0)
                        for w, pre in ((wq32, pq_v), (wk32, pk_v))]
                return q, k, _dot(hs_v[...], pltpu.bitcast(wv32[:, cols], BF16))

            def scores(qkv):
                q, k, v = qkv
                res = []
                for p in range(G // 2):
                    sc = _dot(stack(q, p), stack(k, p).astype(BF16), _NT) * scale
                    sc = jnp.where(keep, sc, fill)
                    e = jnp.exp(sc - jnp.max(sc, axis=-1, keepdims=True))
                    res.append((e, 1.0 / jnp.sum(e, axis=-1, keepdims=True), stack(v, p).astype(BF16)))
                return res

            def values(g, res):
                for p, (e, inv, v) in enumerate(res):
                    o = _dot(e, v) * inv
                    h0 = g * G + 2 * p
                    o_v[:, h0 * Dh:(h0 + 1) * Dh] = o[0:L]
                    o_v[:, (h0 + 1) * Dh:(h0 + 2) * Dh] = o[L:2 * L]

            def outp(g0, g1):
                return _dot(o_v[:, g0 * G * Dh:g1 * G * Dh],
                            pltpu.bitcast(wo32[g0 * G * Dh // 2:g1 * G * Dh // 2, :], BF16))

            h_next = ada1(x_v[jnp.minimum(s + 1, n_seg - 1)])
            qkv, sm = {}, {}
            for g in range(n_g):
                qkv[g] = proj(g)
                if g >= 1:
                    sm[g - 1] = scores(qkv.pop(g - 1))
                if g >= 2:
                    values(g - 2, sm.pop(g - 2))
            half = (n_g - 2) // 2
            acc = outp(0, half)
            sm[n_g - 1] = scores(qkv.pop(n_g - 1))
            values(n_g - 2, sm.pop(n_g - 2))
            acc = acc + outp(half, n_g - 2)
            values(n_g - 1, sm.pop(n_g - 1))
            acc = acc + outp(n_g - 2, n_g - 1)
            acc = acc + outp(n_g - 1, n_g)
            hs_v[0:M, :] = acc[0:M]
            hs_v[M:L, :] = h_next
            att_v[pl.ds(pl.multiple_of(s * T, T), T), :] = acc[M:L]
            return carry

        lax.fori_loop(0, n_seg, step, 0)

        for cp in cp_f:
            cp.wait()
        mod_v[:, 2 * D:6 * D] = _dot(silu_c(), pltpu.bitcast(wm_v[...], BF16))

        def resid(i):
            x = x_v[pl.ds(i * (BM // T), BM // T)].astype(F32).reshape(BM, D)
            return x + mod_v[0:1, 2 * D:3 * D] * att_v[pl.ds(pl.multiple_of(i * BM, BM), BM), :]

        def ada2(i):
            h2 = _layernorm(resid(i)) * (1.0 + mod_v[0:1, 4 * D:5 * D]) + mod_v[0:1, 3 * D:4 * D]
            return h2.astype(BF16)

        h2_v[...] = ada2(0)

        def out_copy(i):
            r = pl.ds(pl.multiple_of(i * BM, BM), BM)
            return pltpu.make_async_copy(y_v.at[r], out_hbm.at[r], sem_y.at[i])

        def ffn(i, carry):
            r = pl.ds(pl.multiple_of(i * BM, BM), BM)
            h2 = h2_v[...]
            h2_next = ada2(jnp.minimum(i + 1, S // BM - 1))
            acc = None
            for f in range(F // FC):
                cols = slice(f * FC, (f + 1) * FC)
                a = (_silu(_dot(h2, w1_v[:, cols])) * _dot(h2, w3_v[:, cols])).astype(BF16)
                d = _dot(a, w2_v[cols, :])
                acc = d if acc is None else acc + d
            y_v[r, :] = (resid(i) + mod_v[0:1, 5 * D:6 * D] * acc).astype(y_v.dtype)
            h2_v[...] = h2_next
            out_copy(i).start()
            return carry

        lax.fori_loop(0, S // BM, ffn, 0)
        for i in range(S // BM):
            out_copy(i).wait()

    pl.run_scoped(main,
                  pltpu.VMEM((D, F), BF16), pltpu.VMEM((D, F), BF16), pltpu.VMEM((F, D), BF16),
                  pltpu.VMEM((D // 2, 4 * D), U32), pltpu.VMEM((S, D), F32), pltpu.VMEM((BM, D), BF16),
                  pltpu.VMEM((S, D), out_hbm.dtype),
                  pltpu.SemaphoreType.DMA((4,)), pltpu.SemaphoreType.DMA((S // BM,)))


@functools.partial(jax.jit, static_argnames=("A_seg_len",))
def pallas_adaLN_cond__memory_aug_recurrent_mem_tr__glu_gated_swiglu__prompt_kernel(
    A_x, A_mem0, A_Wq, A_Wk, A_Wv, A_Wo, A_seg_len, B_x, B_w1, B_w3, B_w2, c, w_mod,
):
    del B_x
    B, S, D = A_x.shape
    _, H, Dh = A_Wq.shape
    M, T, F = A_mem0.shape[1], int(A_seg_len), B_w1.shape[1]
    assert B == 1 and S % T == 0
    L, HD = M + T, H * Dh
    hbm = pl.BlockSpec(memory_space=pl.ANY)
    vmem = pl.BlockSpec(memory_space=pltpu.VMEM)
    body = functools.partial(_body, S=S, D=D, H=H, Dh=Dh, M=M, T=T, F=F, G=8, BM=256, FC=512)
    out = pl.pallas_call(
        body,
        out_shape=jax.ShapeDtypeStruct((S, D), A_x.dtype),
        in_specs=[hbm, vmem, hbm, hbm, hbm, hbm, hbm, hbm, hbm, vmem, hbm],
        out_specs=hbm,
        scratch_shapes=[
            pltpu.VMEM((D // 2, HD), U32), pltpu.VMEM((D // 2, HD), U32), pltpu.VMEM((D // 2, HD), U32),
            pltpu.VMEM((HD // 2, D), U32),
            pltpu.VMEM((S // T * 8, HD), F32), pltpu.VMEM((S // T * 8, HD), F32),
            pltpu.VMEM((S // T, T, D), A_x.dtype), pltpu.VMEM((8, 6 * D), F32),
            pltpu.VMEM((L, D), F32), pltpu.VMEM((L, HD), F32),
            pltpu.SemaphoreType.DMA((2,)),
        ],
        compiler_params=pltpu.CompilerParams(vmem_limit_bytes=120 * 2**20),
    )(A_x.reshape(S // T, T, D), A_mem0.reshape(M, D),
      A_Wq.reshape(D // 2, 2 * H, Dh), A_Wk.reshape(D // 2, 2 * H, Dh), A_Wv.reshape(D // 2, 2 * H, Dh), A_Wo.reshape(HD, D),
      B_w1, B_w3, B_w2, c, w_mod)
    return out.reshape(B, S, D)
```

```python
import functools

import jax
import jax.numpy as jnp
from jax import lax
import jax.experimental.pallas as pl
import jax.experimental.pallas.tpu as pltpu

F32, BF16, U32 = jnp.float32, jnp.bfloat16, jnp.uint32
_LOG2E = 1.4426950408889634
_NN = (((1,), (0,)), ((), ()))
_NT = (((1,), (1,)), ((), ()))


def _dot(a, b, dims=_NN):
    return lax.dot_general(a, b, dims, preferred_element_type=F32)


def _layernorm(x, eps=1e-5):
    m = jnp.mean(x, axis=-1, keepdims=True)
    d = x - m
    v = jnp.mean(d * d, axis=-1, keepdims=True)
    return d * lax.rsqrt(v + eps)


def _silu(x):
    return x / (1.0 + jnp.exp(-x))


def _body(x_hbm, mem0_ref, wq_hbm, wk_hbm, wv_hbm, wo_hbm, w1_hbm, w3_hbm, w2_hbm,
          c_ref, wm_hbm, out_hbm,
          wq32, wk32, wv32, wo32, pq_v, pk_v, x_v, mod_v, hs_v, o_v, sems,
          *, S, D, H, Dh, M, T, F, G, BM, FC):
    n_seg = S // T
    L = M + T
    HD = H * Dh
    UN = 2
    P = 8
    KC = 128
    n_kc = D // KC
    OC = HD // 2 // n_kc
    wo_src = wo_hbm.bitcast(U32)
    wm_src = wm_hbm.bitcast(U32)
    HP = H + 8
    XA = 9
    cp_x = pltpu.make_async_copy(x_hbm.at[pl.ds(0, XA)], x_v.at[pl.ds(0, XA)], sems.at[0])
    cp_x2 = pltpu.make_async_copy(x_hbm.at[pl.ds(XA, n_seg - XA)], x_v.at[pl.ds(XA, n_seg - XA)], sems.at[1])

    def silu_c():
        return jnp.broadcast_to(_silu(c_ref[...].astype(F32)), (8, D)).astype(BF16)

    def ada1(x):
        return _layernorm(x.astype(F32)) * (1.0 + mod_v[0:1, D:2 * D]) + mod_v[0:1, 0:D]

    def startup(wm_v, raw, xp_v, hp_v, sem_m, sem_w, sem_p):
        srcs = [w.bitcast(U32) for w in (wq_hbm, wk_hbm, wv_hbm)]

        def cp_w(t, c):
            if t == 3:
                r = pl.ds(pl.multiple_of(c * OC, OC), OC)
                return pltpu.make_async_copy(wo_src.at[r], wo32.at[r], sem_w.at[3 * n_kc + c])
            j = t * n_kc + c
            return pltpu.make_async_copy(srcs[t].at[pl.ds(c * (KC // 2), KC // 2)],
                                         raw.at[pl.ds(j * (KC // 2), KC // 2), pl.ds(0, H)], sem_w.at[j])

        n_m = 4
        mr = D // n_m
        cp_m = [pltpu.make_async_copy(wm_src.at[pl.ds(j * mr // 2, mr // 2), pl.ds(0, 2 * D)], wm_v.at[j], sem_m.at[j])
                for j in range(n_m)]
        cp_p = pltpu.make_async_copy(x_hbm.at[:, pl.ds(T - P, P), :], xp_v, sem_p.at[0])
        cp_p.start()
        for cp in cp_m:
            cp.start()
        cp_w(0, 0).start()

        def zero(i, carry):
            r = pl.ds(pl.multiple_of(i * 32, 32), 32)
            pq_v[r, :] = jnp.zeros((32, HD), F32)
            pk_v[r, :] = jnp.zeros((32, HD), F32)
            return carry
        lax.fori_loop(0, n_seg * P // 32, zero, 0)

        sc = silu_c()
        cp_p.wait()
        xn = _layernorm(xp_v[...].astype(F32).reshape(n_seg * P, D))
        mod = None
        for j in range(n_m):
            cp_m[j].wait()
            if j < 2:
                cp_w(0, j + 1).start()
            d = _dot(sc[:, j * mr:(j + 1) * mr], pltpu.bitcast(wm_v[j], BF16))
            mod = d if mod is None else mod + d
        mod_v[:, 0:2 * D] = mod
        hp = (xn * (1.0 + mod[0:1, D:2 * D]) + mod[0:1, 0:D]).astype(BF16)
        for c in range(n_kc):
            hp_v[c] = hp[:, c * KC:(c + 1) * KC]

        raw2 = raw.reshape(3 * D // 2 * HP, Dh)

        def retile(c, jobs):
            rows = pl.ds(pl.multiple_of(c * (KC // 2), KC // 2), KC // 2)
            for h4 in range(H // 4):
                for t, dst, pre in jobs:
                    tiles = []
                    for hp2 in (2 * h4, 2 * h4 + 1):
                        base = (t * n_kc + c) * (KC // 2 * HP) + hp2
                        a = raw2[pl.ds(base, KC // 2, stride=HP), :]
                        b = raw2[pl.ds(base + H // 2, KC // 2, stride=HP), :]
                        tiles += [(a & 0xFFFF) | (b << 16), (a >> 16) | ((b >> 16) << 16)]
                    w = jnp.concatenate(tiles, axis=1)
                    cols = slice(4 * h4 * Dh, 4 * (h4 + 1) * Dh)
                    dst[rows, cols] = w
                    if pre is not None:
                        pre[:, cols] += _dot(hp_v[c], pltpu.bitcast(w, BF16))

        order = ([(0, c) for c in range(n_kc)] + [(t, c) for c in range(n_kc) for t in (1, 2)]
                 + [(3, c) for c in range(n_kc)])

        def issue(i, base):
            for it in range(n_kc):
                todo = order[3 + 2 * (base + it):5 + 2 * (base + it)]
                if todo:
                    @pl.when(i == it)
                    def _(todo=todo):
                        for t, c in todo:
                            cp_w(t, c).start()

        def q_phase(c, carry):
            cp_w(0, c).wait()
            issue(c, 0)
            retile(c, [(0, wq32, pq_v)])
            return carry
        lax.fori_loop(0, n_kc, q_phase, 0)

        def k_phase(c, carry):
            cp_w(1, c).wait()
            cp_w(2, c).wait()
            issue(c, n_kc)

            @pl.when(c == n_kc - 2)
            def _():
                cp_x.start()
            retile(c, [(1, wk32, pk_v), (2, wv32, None)])
            return carry
        lax.fori_loop(0, n_kc, k_phase, 0)
        for c in range(n_kc):
            cp_w(3, c).wait()

    pl.run_scoped(startup,
                  pltpu.VMEM((4, D // 8, 2 * D), U32), pltpu.VMEM((3 * D // 2, HP, Dh), U32),
                  pltpu.VMEM((n_seg, P, D), x_hbm.dtype), pltpu.VMEM((n_kc, n_seg * P, KC), BF16),
                  pltpu.SemaphoreType.DMA((4,)), pltpu.SemaphoreType.DMA((4 * n_kc,)),
                  pltpu.SemaphoreType.DMA((1,)))

    def main(w1_v, w3_v, w2_v, wm_v, att_v, h2_v, y_v, sem_f, sem_y):
        cp_f = [pltpu.make_async_copy(s, d, sem_f.at[i]) for i, (s, d) in enumerate((
            (wm_src.at[:, pl.ds(2 * D, 4 * D)], wm_v), (w1_hbm, w1_v), (w3_hbm, w3_v), (w2_hbm, w2_v)))]
        cp_x.wait()
        cp_x2.start()
        hs_v[0:M, :] = mem0_ref[...].astype(F32)
        hs_v[M:L, :] = ada1(x_v[0])
        scale = Dh ** -0.5
        n_g = H // G

        def step(s, carry):
            KP = 2 * L
            ri = lax.broadcasted_iota(jnp.int32, (2 * L, KP), 0)
            ci = lax.broadcasted_iota(jnp.int32, (2 * L, KP), 1)
            same = ((ri >= L) == (ci >= L)) & (ci < 2 * L)
            rl = jnp.where(ri >= L, ri - L, ri)
            cl = jnp.where(ci >= L, ci - L, ci)
            keep = same & ((rl < M) | (rl >= cl))
            fill = jnp.where(same, -1e9 / scale, -jnp.inf).astype(F32)
            early = pl.ds(pl.multiple_of(s * P, P), P)

            def stack(a, p, rows=2 * L):
                parts = [a[:, (2 * p) * Dh:(2 * p + 1) * Dh], a[:, (2 * p + 1) * Dh:(2 * p + 2) * Dh]]
                if rows > 2 * L:
                    parts.append(jnp.zeros((rows - 2 * L, Dh), a.dtype))
                return jnp.concatenate(parts, axis=0)

            def gcols(g):
                return slice(g * G * Dh, (g + 1) * G * Dh)

            def proj_qk(g):
                return [jnp.concatenate([_dot(hs_v[0:L - P, :], pltpu.bitcast(w[:, gcols(g)], BF16)),
                                         pre[early, gcols(g)]], axis=0)
                        for w, pre in ((wq32, pq_v), (wk32, pk_v))]

            def proj_v(g):
                return _dot(hs_v[...], pltpu.bitcast(wv32[:, gcols(g)], BF16))

            def scores(q, k):
                res = []
                for p in range(G // 2):
                    sc = jnp.where(keep, _dot(stack(q, p), stack(k, p, KP).astype(BF16), _NT), fill)
                    e = jnp.exp2((sc - jnp.max(sc, axis=-1, keepdims=True)) * (scale * _LOG2E))
                    den = jnp.sum(e, axis=-1, keepdims=True)
                    r = pl.reciprocal(den, approx=True)
                    res.append((e, r * (2.0 - den * r)))
                return res

            def values(g, res, v):
                for p, (e, inv) in enumerate(res):
                    o = _dot(e, stack(v, p, KP).astype(BF16)) * inv
                    h0 = g * G + 2 * p
                    o_v[:, h0 * Dh:(h0 + 1) * Dh] = o[0:L]
                    o_v[:, (h0 + 1) * Dh:(h0 + 2) * Dh] = o[L:2 * L]

            def outp(g):
                return _dot(o_v[:, gcols(g)],
                            pltpu.bitcast(wo32[g * G * Dh // 2:(g + 1) * G * Dh // 2, :], BF16))

            h_next = ada1(x_v[jnp.minimum(s + 1, n_seg - 1)])
            qk, sm, vv = {}, {}, {}
            for g in range(n_g):
                qk[g] = proj_qk(g)
                if g >= 1:
                    sm[g - 1] = scores(*qk.pop(g - 1))
            for g in range(n_g):
                vv[g] = proj_v(g)
                if g == 0:
                    sm[n_g - 1] = scores(*qk.pop(n_g - 1))
                else:
                    values(g - 1, sm.pop(g - 1), vv.pop(g - 1))
            acc = outp(0)
            values(n_g - 1, sm.pop(n_g - 1), vv.pop(n_g - 1))
            for g in range(1, n_g):
                acc = acc + outp(g)
            hs_v[0:M, :] = acc[0:M]
            hs_v[M:L, :] = h_next
            att_v[pl.ds(pl.multiple_of(s * T, T), T), :] = acc[M:L]
            return carry

        def steps(i, carry):
            @pl.when(i == (XA - 1) // UN)
            def _():
                cp_x2.wait()
                for cp in cp_f:
                    cp.start()
            for j in range(UN):
                step(i * UN + j, carry)
            return carry

        lax.fori_loop(0, n_seg // UN, steps, 0)

        for cp in cp_f:
            cp.wait()
        mod_v[:, 2 * D:6 * D] = _dot(silu_c(), pltpu.bitcast(wm_v[...], BF16))

        def resid(i):
            x = x_v[pl.ds(i * (BM // T), BM // T)].astype(F32).reshape(BM, D)
            return x + mod_v[0:1, 2 * D:3 * D] * att_v[pl.ds(pl.multiple_of(i * BM, BM), BM), :]

        def ada2(i):
            h2 = _layernorm(resid(i)) * (1.0 + mod_v[0:1, 4 * D:5 * D]) + mod_v[0:1, 3 * D:4 * D]
            return h2.astype(BF16)

        h2_v[...] = ada2(0)

        def out_copy(i):
            r = pl.ds(pl.multiple_of(i * BM, BM), BM)
            return pltpu.make_async_copy(y_v.at[r], out_hbm.at[r], sem_y.at[i])

        def ffn(i, carry):
            r = pl.ds(pl.multiple_of(i * BM, BM), BM)
            h2 = h2_v[...]
            h2_next = ada2(jnp.minimum(i + 1, S // BM - 1))
            acc = None
            for f in range(F // FC):
                cols = slice(f * FC, (f + 1) * FC)
                a = (_silu(_dot(h2, w1_v[:, cols])) * _dot(h2, w3_v[:, cols])).astype(BF16)
                d = _dot(a, w2_v[cols, :])
                acc = d if acc is None else acc + d
            y_v[r, :] = (resid(i) + mod_v[0:1, 5 * D:6 * D] * acc).astype(y_v.dtype)
            h2_v[...] = h2_next
            out_copy(i).start()
            return carry

        lax.fori_loop(0, S // BM, ffn, 0)
        for i in range(S // BM):
            out_copy(i).wait()

    pl.run_scoped(main,
                  pltpu.VMEM((D, F), BF16), pltpu.VMEM((D, F), BF16), pltpu.VMEM((F, D), BF16),
                  pltpu.VMEM((D // 2, 4 * D), U32), pltpu.VMEM((S, D), F32), pltpu.VMEM((BM, D), BF16),
                  pltpu.VMEM((S, D), out_hbm.dtype),
                  pltpu.SemaphoreType.DMA((4,)), pltpu.SemaphoreType.DMA((S // BM,)))


@functools.partial(jax.jit, static_argnames=("A_seg_len",))
def pallas_adaLN_cond__memory_aug_recurrent_mem_tr__glu_gated_swiglu__prompt_kernel(
    A_x, A_mem0, A_Wq, A_Wk, A_Wv, A_Wo, A_seg_len, B_x, B_w1, B_w3, B_w2, c, w_mod,
):
    del B_x
    B, S, D = A_x.shape
    _, H, Dh = A_Wq.shape
    M, T, F = A_mem0.shape[1], int(A_seg_len), B_w1.shape[1]
    assert B == 1 and S % T == 0
    L, HD = M + T, H * Dh
    hbm = pl.BlockSpec(memory_space=pl.ANY)
    vmem = pl.BlockSpec(memory_space=pltpu.VMEM)
    body = functools.partial(_body, S=S, D=D, H=H, Dh=Dh, M=M, T=T, F=F, G=8, BM=128, FC=1792)
    out = pl.pallas_call(
        body,
        out_shape=jax.ShapeDtypeStruct((S, D), A_x.dtype),
        in_specs=[hbm, vmem, hbm, hbm, hbm, hbm, hbm, hbm, hbm, vmem, hbm],
        out_specs=hbm,
        scratch_shapes=[
            pltpu.VMEM((D // 2, HD), U32), pltpu.VMEM((D // 2, HD), U32), pltpu.VMEM((D // 2, HD), U32),
            pltpu.VMEM((HD // 2, D), U32),
            pltpu.VMEM((S // T * 8, HD), F32), pltpu.VMEM((S // T * 8, HD), F32),
            pltpu.VMEM((S // T, T, D), A_x.dtype), pltpu.VMEM((8, 6 * D), F32),
            pltpu.VMEM((L, D), F32), pltpu.VMEM((L, HD), F32),
            pltpu.SemaphoreType.DMA((2,)),
        ],
        compiler_params=pltpu.CompilerParams(vmem_limit_bytes=120 * 2**20),
    )(A_x.reshape(S // T, T, D), A_mem0.reshape(M, D),
      A_Wq.reshape(D // 2, 2 * H, Dh), A_Wk.reshape(D // 2, 2 * H, Dh), A_Wv.reshape(D // 2, 2 * H, Dh), A_Wo.reshape(HD, D),
      B_w1, B_w3, B_w2, c, w_mod)
    return out.reshape(B, S, D)
```

```python
import functools

import jax
import jax.numpy as jnp
from jax import lax
import jax.experimental.pallas as pl
import jax.experimental.pallas.tpu as pltpu

F32, BF16, U32 = jnp.float32, jnp.bfloat16, jnp.uint32
_LOG2E = 1.4426950408889634
_NN = (((1,), (0,)), ((), ()))
_NT = (((1,), (1,)), ((), ()))


def _dot(a, b, dims=_NN):
    return lax.dot_general(a, b, dims, preferred_element_type=F32)


def _layernorm(x, eps=1e-5):
    m = jnp.mean(x, axis=-1, keepdims=True)
    d = x - m
    v = jnp.mean(d * d, axis=-1, keepdims=True)
    return d * lax.rsqrt(v + eps)


def _silu(x):
    return x / (1.0 + jnp.exp(-x))


def _unpack(w):
    return jnp.stack([pltpu.unpack_elementwise(w, index=i, packed_dtype=BF16, unpacked_dtype=F32)
                      for i in range(2)])


def _pack(x):
    return pltpu.bitcast(pltpu.pack_elementwise([x[0], x[1]], packed_dtype=BF16), U32)


def _strassen_lhs(a11, a12, a21, a22):
    return [v.astype(BF16) for v in (a11 + a22, a21 + a22, a11, a22, a11 + a12, a21 - a11, a12 - a22)]


def _strassen_products(lhs, w, e, rows, c0, width):
    n = w.shape[2] // 2
    lo, hi = slice(c0, c0 + width), slice(n + c0, n + c0 + width)
    rhs = (e.at[0, rows, lo], w.at[0, rows, lo], w.at[0, rows, hi], w.at[1, rows, lo],
           w.at[1, rows, hi], e.at[1, rows, lo], e.at[2, rows, lo])
    return [_dot(a, pltpu.bitcast(b[...], BF16)) for a, b in zip(lhs, rhs)]


def _strassen_combine(m):
    m1, m2, m3, m4, m5, m6, m7 = m
    return m1 + m4 - m5 + m7, m3 + m5, m2 + m4, m1 - m2 + m3 + m6


def _body(x_hbm, mem0_ref, wq_hbm, wk_hbm, wv_hbm, wo_hbm, w1_hbm, w3_hbm, w2_hbm,
          c_ref, wm_hbm, out_hbm,
          wq32, wk32, wv32, wo32, pq_v, pk_v, x_v, mod_v, hs_v, o_v, zero_v, sems,
          *, S, D, H, Dh, M, T, F, G, BM, FC):
    n_seg = S // T
    L = M + T
    HD = H * Dh
    UN = 2
    P = 8
    KC = 128
    n_kc = D // KC
    OC = HD // 2 // n_kc
    wo_src = wo_hbm.bitcast(U32)
    wm_src = wm_hbm.bitcast(U32)
    HP = H + 8
    XA = 9
    cp_x = pltpu.make_async_copy(x_hbm.at[pl.ds(0, XA)], x_v.at[pl.ds(0, XA)], sems.at[0])
    cp_x2 = pltpu.make_async_copy(x_hbm.at[pl.ds(XA, n_seg - XA)], x_v.at[pl.ds(XA, n_seg - XA)], sems.at[1])

    zero_v[...] = jnp.zeros(zero_v.shape, U32)

    def after(anchor):
        return pltpu.bitcast(anchor[0:8, 0:128], U32) & zero_v[...]

    def silu_c():
        return jnp.broadcast_to(_silu(c_ref[...].astype(F32)), (8, D)).astype(BF16)

    def ada1(x):
        return _layernorm(x.astype(F32)) * (1.0 + mod_v[0:1, D:2 * D]) + mod_v[0:1, 0:D]

    def startup(wm_v, raw, xp_v, hp_v, sem_m, sem_w, sem_p):
        srcs = [w.bitcast(U32) for w in (wq_hbm, wk_hbm, wv_hbm)]

        def cp_w(t, c):
            if t == 3:
                r = pl.ds(pl.multiple_of(c * OC, OC), OC)
                return pltpu.make_async_copy(wo_src.at[r], wo32.at[r], sem_w.at[3 * n_kc + c])
            j = t * n_kc + c
            return pltpu.make_async_copy(srcs[t].at[pl.ds(c * (KC // 2), KC // 2)],
                                         raw.at[pl.ds(j * (KC // 2), KC // 2), pl.ds(0, H)], sem_w.at[j])

        n_m = 4
        mr = D // n_m
        cp_m = [pltpu.make_async_copy(wm_src.at[pl.ds(j * mr // 2, mr // 2), pl.ds(0, 2 * D)], wm_v.at[j], sem_m.at[j])
                for j in range(n_m)]
        cp_p = pltpu.make_async_copy(x_hbm.at[:, pl.ds(T - P, P), :], xp_v, sem_p.at[0])
        cp_p.start()
        for cp in cp_m:
            cp.start()
        cp_w(0, 0).start()

        def zero(i, carry):
            r = pl.ds(pl.multiple_of(i * 32, 32), 32)
            pq_v[r, :] = jnp.zeros((32, HD), F32)
            pk_v[r, :] = jnp.zeros((32, HD), F32)
            return carry
        lax.fori_loop(0, n_seg * P // 32, zero, 0)

        sc = silu_c()
        cp_p.wait()
        xn = _layernorm(xp_v[...].astype(F32).reshape(n_seg * P, D))
        mod = None
        for j in range(n_m):
            cp_m[j].wait()
            if j < 2:
                cp_w(0, j + 1).start()
            d = _dot(sc[:, j * mr:(j + 1) * mr], pltpu.bitcast(wm_v[j], BF16))
            mod = d if mod is None else mod + d
        mod_v[:, 0:2 * D] = mod
        hp = (xn * (1.0 + mod[0:1, D:2 * D]) + mod[0:1, 0:D]).astype(BF16)
        for c in range(n_kc):
            hp_v[c] = hp[:, c * KC:(c + 1) * KC]

        raw2 = raw.reshape(3 * D // 2 * HP, Dh)

        def retile(c, jobs):
            rows = pl.ds(pl.multiple_of(c * (KC // 2), KC // 2), KC // 2)
            for h4 in range(H // 4):
                tie = None
                for t, dst, pre in jobs:
                    tiles = []
                    for hp2 in (2 * h4, 2 * h4 + 1):
                        base = (t * n_kc + c) * (KC // 2 * HP) + hp2
                        a = raw2[pl.ds(base, KC // 2, stride=HP), :]
                        b = raw2[pl.ds(base + H // 2, KC // 2, stride=HP), :]
                        if tie is not None:
                            a, b = a | tie, b | tie
                        tiles += [(a & 0xFFFF) | (b << 16), (a >> 16) | ((b >> 16) << 16)]
                    w = jnp.concatenate(tiles, axis=1)
                    cols = slice(4 * h4 * Dh, 4 * (h4 + 1) * Dh)
                    dst[rows, cols] = w
                    if pre is not None:
                        d = _dot(hp_v[c], pltpu.bitcast(w, BF16))
                        pre[:, cols] += d
                        tie = jnp.tile(after(d), (KC // 16, 1))

        order = ([(0, c) for c in range(n_kc)] + [(t, c) for c in range(n_kc) for t in (1, 2)]
                 + [(3, c) for c in range(n_kc)])

        def issue(i, base):
            for it in range(n_kc):
                todo = order[3 + 2 * (base + it):5 + 2 * (base + it)]
                if todo:
                    @pl.when(i == it)
                    def _(todo=todo):
                        for t, c in todo:
                            cp_w(t, c).start()

        def q_phase(c, carry):
            cp_w(0, c).wait()
            issue(c, 0)
            retile(c, [(0, wq32, pq_v)])
            return carry
        lax.fori_loop(0, n_kc, q_phase, 0)

        def k_phase(c, carry):
            cp_w(1, c).wait()
            cp_w(2, c).wait()
            issue(c, n_kc)

            @pl.when(c == n_kc - 2)
            def _():
                cp_x.start()
            retile(c, [(1, wk32, pk_v), (2, wv32, None)])
            return carry
        lax.fori_loop(0, n_kc, k_phase, 0)
        for c in range(n_kc):
            cp_w(3, c).wait()

    pl.run_scoped(startup,
                  pltpu.VMEM((4, D // 8, 2 * D), U32), pltpu.VMEM((3 * D // 2, HP, Dh), U32),
                  pltpu.VMEM((n_seg, P, D), x_hbm.dtype), pltpu.VMEM((n_kc, n_seg * P, KC), BF16),
                  pltpu.SemaphoreType.DMA((4,)), pltpu.SemaphoreType.DMA((4 * n_kc,)),
                  pltpu.SemaphoreType.DMA((1,)))

    n_it = n_seg // UN
    n_prep = n_it // 2
    R1, R2 = D // 4, F // 4
    r1, r2 = R1 // n_prep, R2 // n_prep

    def main(w1_v, w3_v, w2_v, e1_v, e3_v, e2_v, wm_v, att_v, h2_v, sem_f, sem_y):
        ffn_w = ((w1_hbm, w1_v, e1_v, R1, r1), (w3_hbm, w3_v, e3_v, R1, r1), (w2_hbm, w2_v, e2_v, R2, r2))
        cp_f = [pltpu.make_async_copy(src.bitcast(U32).at[pl.ds(i * R, R)], w.at[i, pl.ds(0, R)],
                                      sem_f.at[2 * j + i])
                for j, (src, w, _, R, _) in enumerate(ffn_w) for i in range(2)]
        cp_m = pltpu.make_async_copy(wm_src.at[:, pl.ds(2 * D, 4 * D)], wm_v, sem_f.at[6])
        for _, w, _, R, r in ffn_w:
            w[:, R:R + r, :] = jnp.zeros((2, r, w.shape[2]), U32)

        pieces = [(j, r0, c0) for j, (_, w, _, _, r) in enumerate(ffn_w)
                  for r0 in range(0, r, 8) for c0 in range(0, w.shape[2] // 2, 128)]

        def prep_ffn(i, site, n_sites, anchor):
            tie = after(anchor)
            for j, r0, c0 in pieces[site::n_sites]:
                _, w, e, R, r = ffn_w[j]
                n = w.shape[2] // 2
                base = jnp.where(i >= n_it - n_prep, (i - (n_it - n_prep)) * r, R)
                rows = pl.ds(pl.multiple_of(base + r0, 8), 8)
                lo, hi = slice(c0, c0 + 128), slice(n + c0, n + c0 + 128)
                b11, b12 = _unpack(w[0, rows, lo] | tie), _unpack(w[0, rows, hi] | tie)
                b21, b22 = _unpack(w[1, rows, lo] | tie), _unpack(w[1, rows, hi] | tie)
                e[0, rows, lo] = _pack(b11 + b22)
                e[1, rows, lo] = _pack(b11 + b12)
                e[2, rows, lo] = _pack(b21 + b22)
                w[0, rows, hi] = _pack(b12 - b22)
                w[1, rows, lo] = _pack(b21 - b11)

        cp_x.wait()
        cp_x2.start()
        hs_v[0:M, :] = mem0_ref[...].astype(F32)
        hs_v[M:L, :] = ada1(x_v[0])
        scale = Dh ** -0.5
        n_g = H // G

        def step(s, side):
            KP = 2 * L
            ri = lax.broadcasted_iota(jnp.int32, (2 * L, KP), 0)
            ci = lax.broadcasted_iota(jnp.int32, (2 * L, KP), 1)
            same = ((ri >= L) == (ci >= L)) & (ci < 2 * L)
            rl = jnp.where(ri >= L, ri - L, ri)
            cl = jnp.where(ci >= L, ci - L, ci)
            keep = same & ((rl < M) | (rl >= cl))
            fill = jnp.where(same, -1e9 / scale, -jnp.inf).astype(F32)
            early = pl.ds(pl.multiple_of(s * P, P), P)

            def stack(a, p, rows=2 * L):
                parts = [a[:, (2 * p) * Dh:(2 * p + 1) * Dh], a[:, (2 * p + 1) * Dh:(2 * p + 2) * Dh]]
                if rows > 2 * L:
                    parts.append(jnp.zeros((rows - 2 * L, Dh), a.dtype))
                return jnp.concatenate(parts, axis=0)

            def gcols(g):
                return slice(g * G * Dh, (g + 1) * G * Dh)

            def proj_qk(g):
                return [jnp.concatenate([_dot(hs_v[0:L - P, :], pltpu.bitcast(w[:, gcols(g)], BF16)),
                                         pre[early, gcols(g)]], axis=0)
                        for w, pre in ((wq32, pq_v), (wk32, pk_v))]

            def proj_v(g):
                return _dot(hs_v[...], pltpu.bitcast(wv32[:, gcols(g)], BF16))

            def scores(q, k):
                res = []
                for p in range(G // 2):
                    sc = jnp.where(keep, _dot(stack(q, p), stack(k, p, KP).astype(BF16), _NT), fill)
                    e = jnp.exp2((sc - jnp.max(sc, axis=-1, keepdims=True)) * (scale * _LOG2E))
                    den = jnp.sum(e, axis=-1, keepdims=True)
                    r = pl.reciprocal(den, approx=True)
                    res.append((e, r * (2.0 - den * r)))
                return res

            def values(g, res, v):
                for p, (e, inv) in enumerate(res):
                    o = _dot(e, stack(v, p, KP).astype(BF16)) * inv
                    h0 = g * G + 2 * p
                    o_v[:, h0 * Dh:(h0 + 1) * Dh] = o[0:L]
                    o_v[:, (h0 + 1) * Dh:(h0 + 2) * Dh] = o[L:2 * L]

            def outp(g):
                return _dot(o_v[:, gcols(g)],
                            pltpu.bitcast(wo32[g * G * Dh // 2:(g + 1) * G * Dh // 2, :], BF16))

            h_next = ada1(x_v[jnp.minimum(s + 1, n_seg - 1)])
            qk, sm, vv = {}, {}, {}
            for g in range(n_g):
                qk[g] = proj_qk(g)
                if g >= 1:
                    sm[g - 1] = scores(*qk.pop(g - 1))
                    side(g - 1, qk[g][0])
            for g in range(n_g):
                vv[g] = proj_v(g)
                side(n_g - 1 + g, vv[g])
                if g == 0:
                    sm[n_g - 1] = scores(*qk.pop(n_g - 1))
                else:
                    values(g - 1, sm.pop(g - 1), vv.pop(g - 1))
            acc = outp(0)
            values(n_g - 1, sm.pop(n_g - 1), vv.pop(n_g - 1))
            for g in range(1, n_g):
                acc = acc + outp(g)
            hs_v[0:M, :] = acc[0:M]
            hs_v[M:L, :] = h_next
            att_v[pl.ds(pl.multiple_of(s * T, T), T), :] = acc[M:L]

        def steps(i, carry):
            @pl.when(i == (XA - 1) // UN)
            def _():
                cp_x2.wait()
                for cp in cp_f:
                    cp.start()
                cp_m.start()

            @pl.when(i == n_it - n_prep)
            def _():
                for cp in cp_f:
                    cp.wait()
            for j in range(UN):
                per = 2 * n_g - 1
                step(i * UN + j, lambda k, anchor, j=j: prep_ffn(i, j * per + k, UN * per, anchor))
            return carry

        lax.fori_loop(0, n_seg // UN, steps, 0)

        cp_m.wait()
        mod_v[:, 2 * D:6 * D] = _dot(silu_c(), pltpu.bitcast(wm_v[...], BF16))

        def resid(i):
            x = x_v[pl.ds(i * (BM // T), BM // T)].astype(F32).reshape(BM, D)
            return x + mod_v[0:1, 2 * D:3 * D] * att_v[pl.ds(pl.multiple_of(i * BM, BM), BM), :]

        def ada2(i):
            h2 = _layernorm(resid(i)) * (1.0 + mod_v[0:1, 4 * D:5 * D]) + mod_v[0:1, 3 * D:4 * D]
            hm, hd = BM // 2, D // 2
            return _strassen_lhs(h2[:hm, :hd], h2[:hm, hd:], h2[hm:, :hd], h2[hm:, hd:])

        def put_h2(parts):
            for j, part in enumerate(parts):
                h2_v[j] = part

        put_h2(ada2(0))

        def out_copy(i):
            r = pl.ds(i * (BM // T), BM // T)
            return pltpu.make_async_copy(x_v.at[r], out_hbm.at[r], sem_y.at[i])

        def ffn(i, carry):
            lhs = [h2_v[j] for j in range(7)]
            h2_next = ada2(jnp.minimum(i + 1, S // BM - 1))
            acc = None
            for c0 in range(0, F // 2, FC):
                gate = _strassen_combine(_strassen_products(lhs, w1_v, e1_v, slice(0, R1), c0, FC))
                up = _strassen_combine(_strassen_products(lhs, w3_v, e3_v, slice(0, R1), c0, FC))
                act = _strassen_lhs(*[_silu(g) * u for g, u in zip(gate, up)])
                m = _strassen_products(act, w2_v, e2_v, slice(c0 // 2, (c0 + FC) // 2), 0, D // 2)
                acc = m if acc is None else [x + y for x, y in zip(acc, m)]
            c11, c12, c21, c22 = _strassen_combine(acc)
            ffn_out = jnp.concatenate([jnp.concatenate([c11, c12], axis=1),
                                       jnp.concatenate([c21, c22], axis=1)], axis=0)
            y = resid(i) + mod_v[0:1, 5 * D:6 * D] * ffn_out
            x_v[pl.ds(i * (BM // T), BM // T)] = y.reshape(BM // T, T, D).astype(x_v.dtype)
            put_h2(h2_next)
            out_copy(i).start()
            return carry

        lax.fori_loop(0, S // BM, ffn, 0)
        for i in range(S // BM):
            out_copy(i).wait()

    pl.run_scoped(main,
                  pltpu.VMEM((2, R1 + r1, F), U32), pltpu.VMEM((2, R1 + r1, F), U32),
                  pltpu.VMEM((2, R2 + r2, D), U32),
                  pltpu.VMEM((3, R1 + r1, F // 2), U32), pltpu.VMEM((3, R1 + r1, F // 2), U32),
                  pltpu.VMEM((3, R2 + r2, D // 2), U32),
                  pltpu.VMEM((D // 2, 4 * D), U32), pltpu.VMEM((S, D), F32),
                  pltpu.VMEM((7, BM // 2, D // 2), BF16),
                  pltpu.SemaphoreType.DMA((7,)), pltpu.SemaphoreType.DMA((S // BM,)))


@functools.partial(jax.jit, static_argnames=("A_seg_len",))
def pallas_adaLN_cond__memory_aug_recurrent_mem_tr__glu_gated_swiglu__prompt_kernel(
    A_x, A_mem0, A_Wq, A_Wk, A_Wv, A_Wo, A_seg_len, B_x, B_w1, B_w3, B_w2, c, w_mod,
):
    del B_x
    B, S, D = A_x.shape
    _, H, Dh = A_Wq.shape
    M, T, F = A_mem0.shape[1], int(A_seg_len), B_w1.shape[1]
    assert B == 1 and S % T == 0
    L, HD = M + T, H * Dh
    hbm = pl.BlockSpec(memory_space=pl.ANY)
    vmem = pl.BlockSpec(memory_space=pltpu.VMEM)
    body = functools.partial(_body, S=S, D=D, H=H, Dh=Dh, M=M, T=T, F=F, G=8, BM=128, FC=1792)
    out = pl.pallas_call(
        body,
        out_shape=jax.ShapeDtypeStruct((S // T, T, D), A_x.dtype),
        in_specs=[hbm, vmem, hbm, hbm, hbm, hbm, hbm, hbm, hbm, vmem, hbm],
        out_specs=hbm,
        scratch_shapes=[
            pltpu.VMEM((D // 2, HD), U32), pltpu.VMEM((D // 2, HD), U32), pltpu.VMEM((D // 2, HD), U32),
            pltpu.VMEM((HD // 2, D), U32),
            pltpu.VMEM((S // T * 8, HD), F32), pltpu.VMEM((S // T * 8, HD), F32),
            pltpu.VMEM((S // T, T, D), A_x.dtype), pltpu.VMEM((8, 6 * D), F32),
            pltpu.VMEM((L, D), F32), pltpu.VMEM((L, HD), F32), pltpu.VMEM((8, 128), U32),
            pltpu.SemaphoreType.DMA((2,)),
        ],
        compiler_params=pltpu.CompilerParams(vmem_limit_bytes=126 * 2**20, flags={'XLA_TPU_EVENLY_DISTRIBUTE_CRITICAL_NODES': True}),
    )(A_x.reshape(S // T, T, D), A_mem0.reshape(M, D),
      A_Wq.reshape(D // 2, 2 * H, Dh), A_Wk.reshape(D // 2, 2 * H, Dh), A_Wv.reshape(D // 2, 2 * H, Dh), A_Wo.reshape(HD, D),
      B_w1, B_w3, B_w2, c, w_mod)
    return out.reshape(B, S, D)
```

```python
import functools

import jax
import jax.numpy as jnp
from jax import lax
import jax.experimental.pallas as pl
import jax.experimental.pallas.tpu as pltpu

F32, BF16, U32 = jnp.float32, jnp.bfloat16, jnp.uint32
_LOG2E = 1.4426950408889634
_NN = (((1,), (0,)), ((), ()))
_NT = (((1,), (1,)), ((), ()))


def _dot(a, b, dims=_NN):
    return lax.dot_general(a, b, dims, preferred_element_type=F32)


def _layernorm(x, eps=1e-5):
    m = jnp.mean(x, axis=-1, keepdims=True)
    d = x - m
    v = jnp.mean(d * d, axis=-1, keepdims=True)
    return d * lax.rsqrt(v + eps)


def _silu(x):
    return x / (1.0 + jnp.exp(-x))


def _unpack(w):
    return jnp.stack([pltpu.unpack_elementwise(w, index=i, packed_dtype=BF16, unpacked_dtype=F32)
                      for i in range(2)])


def _pack(x):
    return pltpu.bitcast(pltpu.pack_elementwise([x[0], x[1]], packed_dtype=BF16), U32)


def _strassen_lhs(a11, a12, a21, a22):
    return [v.astype(BF16) for v in (a11 + a22, a21 + a22, a11, a22, a11 + a12, a21 - a11, a12 - a22)]


def _strassen_products(lhs, w, e, rows, c0, width):
    n = w.shape[2] // 2
    lo, hi = slice(c0, c0 + width), slice(n + c0, n + c0 + width)
    rhs = (e.at[0, rows, lo], w.at[0, rows, lo], w.at[0, rows, hi], w.at[1, rows, lo],
           w.at[1, rows, hi], e.at[1, rows, lo], e.at[2, rows, lo])
    return [_dot(a, pltpu.bitcast(b[...], BF16)) for a, b in zip(lhs, rhs)]


def _strassen_combine(m):
    m1, m2, m3, m4, m5, m6, m7 = m
    return m1 + m4 - m5 + m7, m3 + m5, m2 + m4, m1 - m2 + m3 + m6


def _body(x_hbm, mem0_ref, wq_hbm, wk_hbm, wv_hbm, wo_hbm, w1_hbm, w3_hbm, w2_hbm,
          c_ref, wm_hbm, out_hbm,
          wq32, wk32, wv32, wo32, pq_v, pk_v, x_v, mod_v, hs_v, o_v, zero_v, sems,
          *, S, D, H, Dh, M, T, F, G, BM, FC):
    n_seg = S // T
    L = M + T
    HD = H * Dh
    UN = 2
    P = 8
    KC = 128
    n_kc = D // KC
    OC = HD // 2 // n_kc
    wo_src = wo_hbm.bitcast(U32)
    wm_src = wm_hbm.bitcast(U32)
    HP = H + 8
    XA = 9
    cp_x = pltpu.make_async_copy(x_hbm.at[pl.ds(0, XA)], x_v.at[pl.ds(0, XA)], sems.at[0])
    cp_x2 = pltpu.make_async_copy(x_hbm.at[pl.ds(XA, n_seg - XA)], x_v.at[pl.ds(XA, n_seg - XA)], sems.at[1])

    zero_v[...] = jnp.zeros(zero_v.shape, U32)

    def after(anchor):
        return pltpu.bitcast(anchor[0:8, 0:128], U32) & zero_v[...]

    def silu_c():
        return jnp.broadcast_to(_silu(c_ref[...].astype(F32)), (8, D)).astype(BF16)

    def ada1(x):
        return _layernorm(x.astype(F32)) * (1.0 + mod_v[0:1, D:2 * D]) + mod_v[0:1, 0:D]

    def startup(wm_v, raw, xp_v, hp_v, sem_m, sem_w, sem_p):
        srcs = [w.bitcast(U32) for w in (wq_hbm, wk_hbm, wv_hbm)]

        def cp_w(t, c):
            if t == 3:
                r = pl.ds(pl.multiple_of(c * OC, OC), OC)
                return pltpu.make_async_copy(wo_src.at[r], wo32.at[r], sem_w.at[3 * n_kc + c])
            j = t * n_kc + c
            return pltpu.make_async_copy(srcs[t].at[pl.ds(c * (KC // 2), KC // 2)],
                                         raw.at[pl.ds(j * (KC // 2), KC // 2), pl.ds(0, H)], sem_w.at[j])

        n_m = 4
        mr = D // n_m
        cp_m = [pltpu.make_async_copy(wm_src.at[pl.ds(j * mr // 2, mr // 2), pl.ds(0, 2 * D)], wm_v.at[j], sem_m.at[j])
                for j in range(n_m)]
        cp_p = pltpu.make_async_copy(x_hbm.at[:, pl.ds(T - P, P), :], xp_v, sem_p.at[0])
        cp_p.start()
        for cp in cp_m:
            cp.start()
        cp_w(0, 0).start()

        def zero(i, carry):
            r = pl.ds(pl.multiple_of(i * 32, 32), 32)
            pq_v[r, :] = jnp.zeros((32, HD), F32)
            pk_v[r, :] = jnp.zeros((32, HD), F32)
            return carry
        lax.fori_loop(0, n_seg * P // 32, zero, 0)

        sc = silu_c()
        cp_p.wait()
        xn = _layernorm(xp_v[...].astype(F32).reshape(n_seg * P, D))
        mod = None
        for j in range(n_m):
            cp_m[j].wait()
            if j < 2:
                cp_w(0, j + 1).start()
            d = _dot(sc[:, j * mr:(j + 1) * mr], pltpu.bitcast(wm_v[j], BF16))
            mod = d if mod is None else mod + d
        mod_v[:, 0:2 * D] = mod
        hp = (xn * (1.0 + mod[0:1, D:2 * D]) + mod[0:1, 0:D]).astype(BF16)
        for c in range(n_kc):
            hp_v[c] = hp[:, c * KC:(c + 1) * KC]

        raw2 = raw.reshape(3 * D // 2 * HP, Dh)

        def retile(c, jobs):
            rows = pl.ds(pl.multiple_of(c * (KC // 2), KC // 2), KC // 2)
            for h4 in range(H // 4):
                tie = None
                for t, dst, pre in jobs:
                    tiles = []
                    for hp2 in (2 * h4, 2 * h4 + 1):
                        base = (t * n_kc + c) * (KC // 2 * HP) + hp2
                        a = raw2[pl.ds(base, KC // 2, stride=HP), :]
                        b = raw2[pl.ds(base + H // 2, KC // 2, stride=HP), :]
                        if tie is not None:
                            a, b = a | tie, b | tie
                        tiles += [(a & 0xFFFF) | (b << 16), (a >> 16) | ((b >> 16) << 16)]
                    w = jnp.concatenate(tiles, axis=1)
                    cols = slice(4 * h4 * Dh, 4 * (h4 + 1) * Dh)
                    dst[rows, cols] = w
                    if pre is not None:
                        d = _dot(hp_v[c], pltpu.bitcast(w, BF16))
                        pre[:, cols] += d
                        tie = jnp.tile(after(d), (KC // 16, 1))

        order = ([(0, c) for c in range(n_kc)] + [(t, c) for c in range(n_kc) for t in (1, 2)]
                 + [(3, c) for c in range(n_kc)])

        def issue(i, base):
            for it in range(n_kc):
                todo = order[3 + 2 * (base + it):5 + 2 * (base + it)]
                if todo:
                    @pl.when(i == it)
                    def _(todo=todo):
                        for t, c in todo:
                            cp_w(t, c).start()

        def q_phase(c, carry):
            cp_w(0, c).wait()
            issue(c, 0)
            retile(c, [(0, wq32, pq_v)])
            return carry
        lax.fori_loop(0, n_kc, q_phase, 0)

        def k_phase(c, carry):
            cp_w(1, c).wait()
            cp_w(2, c).wait()
            issue(c, n_kc)

            @pl.when(c == n_kc - 2)
            def _():
                cp_x.start()
            retile(c, [(1, wk32, pk_v), (2, wv32, None)])
            return carry
        lax.fori_loop(0, n_kc, k_phase, 0)
        for c in range(n_kc):
            cp_w(3, c).wait()

    pl.run_scoped(startup,
                  pltpu.VMEM((4, D // 8, 2 * D), U32), pltpu.VMEM((3 * D // 2, HP, Dh), U32),
                  pltpu.VMEM((n_seg, P, D), x_hbm.dtype), pltpu.VMEM((n_kc, n_seg * P, KC), BF16),
                  pltpu.SemaphoreType.DMA((4,)), pltpu.SemaphoreType.DMA((4 * n_kc,)),
                  pltpu.SemaphoreType.DMA((1,)))

    n_it = n_seg // UN
    n_prep = n_it // 2
    R1, R2 = D // 4, F // 4
    r1, r2 = R1 // n_prep, R2 // n_prep

    def main(w1_v, w3_v, w2_v, e1_v, e3_v, e2_v, wm_v, att_v, h2_v, sem_f, sem_y):
        ffn_w = ((w1_hbm, w1_v, e1_v, R1, r1), (w3_hbm, w3_v, e3_v, R1, r1), (w2_hbm, w2_v, e2_v, R2, r2))
        cp_f = [pltpu.make_async_copy(src.bitcast(U32).at[pl.ds(i * R, R)], w.at[i, pl.ds(0, R)],
                                      sem_f.at[2 * j + i])
                for j, (src, w, _, R, _) in enumerate(ffn_w) for i in range(2)]
        cp_m = pltpu.make_async_copy(wm_src.at[:, pl.ds(2 * D, 4 * D)], wm_v, sem_f.at[6])
        for _, w, _, R, r in ffn_w:
            w[:, R:R + r, :] = jnp.zeros((2, r, w.shape[2]), U32)

        pieces = [(j, r0, c0) for j, (_, w, _, _, r) in enumerate(ffn_w)
                  for r0 in range(0, r, 8) for c0 in range(0, w.shape[2] // 2, 128)]

        def prep_ffn(i, site, n_sites, anchor):
            for k, (j, r0, c0) in enumerate(pieces[site::n_sites]):
                tie = after(anchor[:, (k * 128) % anchor.shape[1]:])
                _, w, e, R, r = ffn_w[j]
                n = w.shape[2] // 2
                base = jnp.where(i >= n_it - n_prep, (i - (n_it - n_prep)) * r, R)
                rows = pl.ds(pl.multiple_of(base + r0, 8), 8)
                lo, hi = slice(c0, c0 + 128), slice(n + c0, n + c0 + 128)
                b11, b12 = _unpack(w[0, rows, lo] | tie), _unpack(w[0, rows, hi] | tie)
                b21, b22 = _unpack(w[1, rows, lo] | tie), _unpack(w[1, rows, hi] | tie)
                e[0, rows, lo] = _pack(b11 + b22)
                e[1, rows, lo] = _pack(b11 + b12)
                e[2, rows, lo] = _pack(b21 + b22)
                w[0, rows, hi] = _pack(b12 - b22)
                w[1, rows, lo] = _pack(b21 - b11)

        cp_x.wait()
        cp_x2.start()
        for cp in cp_f:
            cp.start()
        cp_m.start()
        hs_v[0:M, :] = mem0_ref[...].astype(F32)
        hs_v[M:L, :] = ada1(x_v[0])
        scale = Dh ** -0.5
        n_g = H // G

        def step(s, side):
            KP = 2 * L
            ri = lax.broadcasted_iota(jnp.int32, (2 * L, KP), 0)
            ci = lax.broadcasted_iota(jnp.int32, (2 * L, KP), 1)
            same = ((ri >= L) == (ci >= L)) & (ci < 2 * L)
            rl = jnp.where(ri >= L, ri - L, ri)
            cl = jnp.where(ci >= L, ci - L, ci)
            keep = same & ((rl < M) | (rl >= cl))
            fill = jnp.where(same, -1e9 / scale, -jnp.inf).astype(F32)
            early = pl.ds(pl.multiple_of(s * P, P), P)

            def stack(a, p, rows=2 * L):
                parts = [a[:, (2 * p) * Dh:(2 * p + 1) * Dh], a[:, (2 * p + 1) * Dh:(2 * p + 2) * Dh]]
                if rows > 2 * L:
                    parts.append(jnp.zeros((rows - 2 * L, Dh), a.dtype))
                return jnp.concatenate(parts, axis=0)

            def gcols(g):
                return slice(g * G * Dh, (g + 1) * G * Dh)

            def proj_qk(g):
                return [jnp.concatenate([_dot(hs_v[0:L - P, :], pltpu.bitcast(w[:, gcols(g)], BF16)),
                                         pre[early, gcols(g)]], axis=0)
                        for w, pre in ((wq32, pq_v), (wk32, pk_v))]

            def proj_v(g):
                return _dot(hs_v[...], pltpu.bitcast(wv32[:, gcols(g)], BF16))

            def scores(q, k):
                res = []
                for p in range(G // 2):
                    sc = jnp.where(keep, _dot(stack(q, p), stack(k, p, KP).astype(BF16), _NT), fill)
                    e = jnp.exp2((sc - jnp.max(sc, axis=-1, keepdims=True)) * (scale * _LOG2E))
                    den = jnp.sum(e, axis=-1, keepdims=True)
                    r = pl.reciprocal(den, approx=True)
                    res.append((e, r * (2.0 - den * r)))
                return res

            def values(g, res, v):
                for p, (e, inv) in enumerate(res):
                    o = _dot(e, stack(v, p, KP).astype(BF16)) * inv
                    h0 = g * G + 2 * p
                    o_v[:, h0 * Dh:(h0 + 1) * Dh] = o[0:L]
                    o_v[:, (h0 + 1) * Dh:(h0 + 2) * Dh] = o[L:2 * L]

            def outp(g):
                return _dot(o_v[:, gcols(g)],
                            pltpu.bitcast(wo32[g * G * Dh // 2:(g + 1) * G * Dh // 2, :], BF16))

            h_next = ada1(x_v[jnp.minimum(s + 1, n_seg - 1)])
            qk, sm, vv = {}, {}, {}
            for g in range(n_g):
                qk[g] = proj_qk(g)
                if g >= 1:
                    sm[g - 1] = scores(*qk.pop(g - 1))
            for g in range(n_g):
                vv[g] = proj_v(g)
                side(g, vv[g])
                if g == 0:
                    sm[n_g - 1] = scores(*qk.pop(n_g - 1))
                else:
                    values(g - 1, sm.pop(g - 1), vv.pop(g - 1))
            acc = outp(0)
            values(n_g - 1, sm.pop(n_g - 1), vv.pop(n_g - 1))
            for g in range(1, n_g):
                side(n_g - 1 + g, acc)
                acc = acc + outp(g)
            hs_v[0:M, :] = acc[0:M]
            hs_v[M:L, :] = h_next
            att_v[pl.ds(pl.multiple_of(s * T, T), T), :] = acc[M:L]

        def steps(i, carry):
            @pl.when(i == (XA - 1) // UN)
            def _():
                cp_x2.wait()

            @pl.when(i == n_it - n_prep)
            def _():
                for cp in cp_f:
                    cp.wait()
            for j in range(UN):
                per = 2 * n_g - 1
                step(i * UN + j, lambda k, anchor, j=j: prep_ffn(i, j * per + k, UN * per, anchor))
            return carry

        lax.fori_loop(0, n_seg // UN, steps, 0)

        cp_m.wait()
        mod_v[:, 2 * D:6 * D] = _dot(silu_c(), pltpu.bitcast(wm_v[...], BF16))

        def resid(i):
            x = x_v[pl.ds(i * (BM // T), BM // T)].astype(F32).reshape(BM, D)
            return x + mod_v[0:1, 2 * D:3 * D] * att_v[pl.ds(pl.multiple_of(i * BM, BM), BM), :]

        def ada2(i):
            h2 = _layernorm(resid(i)) * (1.0 + mod_v[0:1, 4 * D:5 * D]) + mod_v[0:1, 3 * D:4 * D]
            hm, hd = BM // 2, D // 2
            return _strassen_lhs(h2[:hm, :hd], h2[:hm, hd:], h2[hm:, :hd], h2[hm:, hd:])

        def put_h2(parts):
            for j, part in enumerate(parts):
                h2_v[j] = part

        put_h2(ada2(0))

        def out_copy(i):
            r = pl.ds(i * (BM // T), BM // T)
            return pltpu.make_async_copy(x_v.at[r], out_hbm.at[r], sem_y.at[i])

        def ffn(i, carry):
            lhs = [h2_v[j] for j in range(7)]
            h2_next = ada2(jnp.minimum(i + 1, S // BM - 1))
            acc = None
            for c0 in range(0, F // 2, FC):
                gate = _strassen_combine(_strassen_products(lhs, w1_v, e1_v, slice(0, R1), c0, FC))
                up = _strassen_combine(_strassen_products(lhs, w3_v, e3_v, slice(0, R1), c0, FC))
                act = _strassen_lhs(*[_silu(g) * u for g, u in zip(gate, up)])
                m = _strassen_products(act, w2_v, e2_v, slice(c0 // 2, (c0 + FC) // 2), 0, D // 2)
                acc = m if acc is None else [x + y for x, y in zip(acc, m)]
            c11, c12, c21, c22 = _strassen_combine(acc)
            ffn_out = jnp.concatenate([jnp.concatenate([c11, c12], axis=1),
                                       jnp.concatenate([c21, c22], axis=1)], axis=0)
            y = resid(i) + mod_v[0:1, 5 * D:6 * D] * ffn_out
            x_v[pl.ds(i * (BM // T), BM // T)] = y.reshape(BM // T, T, D).astype(x_v.dtype)
            put_h2(h2_next)
            out_copy(i).start()
            return carry

        lax.fori_loop(0, S // BM, ffn, 0)
        for i in range(S // BM):
            out_copy(i).wait()

    pl.run_scoped(main,
                  pltpu.VMEM((2, R1 + r1, F), U32), pltpu.VMEM((2, R1 + r1, F), U32),
                  pltpu.VMEM((2, R2 + r2, D), U32),
                  pltpu.VMEM((3, R1 + r1, F // 2), U32), pltpu.VMEM((3, R1 + r1, F // 2), U32),
                  pltpu.VMEM((3, R2 + r2, D // 2), U32),
                  pltpu.VMEM((D // 2, 4 * D), U32), pltpu.VMEM((S, D), F32),
                  pltpu.VMEM((7, BM // 2, D // 2), BF16),
                  pltpu.SemaphoreType.DMA((7,)), pltpu.SemaphoreType.DMA((S // BM,)))


@functools.partial(jax.jit, static_argnames=("A_seg_len",))
def pallas_adaLN_cond__memory_aug_recurrent_mem_tr__glu_gated_swiglu__prompt_kernel(
    A_x, A_mem0, A_Wq, A_Wk, A_Wv, A_Wo, A_seg_len, B_x, B_w1, B_w3, B_w2, c, w_mod,
):
    del B_x
    B, S, D = A_x.shape
    _, H, Dh = A_Wq.shape
    M, T, F = A_mem0.shape[1], int(A_seg_len), B_w1.shape[1]
    assert B == 1 and S % T == 0
    L, HD = M + T, H * Dh
    hbm = pl.BlockSpec(memory_space=pl.ANY)
    vmem = pl.BlockSpec(memory_space=pltpu.VMEM)
    body = functools.partial(_body, S=S, D=D, H=H, Dh=Dh, M=M, T=T, F=F, G=8, BM=128, FC=1792)
    out = pl.pallas_call(
        body,
        out_shape=jax.ShapeDtypeStruct((S // T, T, D), A_x.dtype),
        in_specs=[hbm, vmem, hbm, hbm, hbm, hbm, hbm, hbm, hbm, vmem, hbm],
        out_specs=hbm,
        scratch_shapes=[
            pltpu.VMEM((D // 2, HD), U32), pltpu.VMEM((D // 2, HD), U32), pltpu.VMEM((D // 2, HD), U32),
            pltpu.VMEM((HD // 2, D), U32),
            pltpu.VMEM((S // T * 8, HD), F32), pltpu.VMEM((S // T * 8, HD), F32),
            pltpu.VMEM((S // T, T, D), A_x.dtype), pltpu.VMEM((8, 6 * D), F32),
            pltpu.VMEM((L, D), F32), pltpu.VMEM((L, HD), F32), pltpu.VMEM((8, 128), U32),
            pltpu.SemaphoreType.DMA((2,)),
        ],
        compiler_params=pltpu.CompilerParams(vmem_limit_bytes=126 * 2**20, flags={'XLA_TPU_EVENLY_DISTRIBUTE_CRITICAL_NODES': True}),
    )(A_x.reshape(S // T, T, D), A_mem0.reshape(M, D),
      A_Wq.reshape(D // 2, 2 * H, Dh), A_Wk.reshape(D // 2, 2 * H, Dh), A_Wv.reshape(D // 2, 2 * H, Dh), A_Wo.reshape(HD, D),
      B_w1, B_w3, B_w2, c, w_mod)
    return out.reshape(B, S, D)
```

```python
import functools

import jax
import jax.numpy as jnp
from jax import lax
import jax.experimental.pallas as pl
import jax.experimental.pallas.tpu as pltpu

F32, BF16, U32 = jnp.float32, jnp.bfloat16, jnp.uint32
_LOG2E = 1.4426950408889634
_NN = (((1,), (0,)), ((), ()))
_NT = (((1,), (1,)), ((), ()))


def _dot(a, b, dims=_NN):
    return lax.dot_general(a, b, dims, preferred_element_type=F32)


def _layernorm(x, eps=1e-5):
    m = jnp.mean(x, axis=-1, keepdims=True)
    d = x - m
    v = jnp.mean(d * d, axis=-1, keepdims=True)
    return d * lax.rsqrt(v + eps)


def _silu(x):
    return x / (1.0 + jnp.exp(-x))


def _unpack(w):
    return jnp.stack([pltpu.unpack_elementwise(w, index=i, packed_dtype=BF16, unpacked_dtype=F32)
                      for i in range(2)])


def _pack(x):
    return pltpu.bitcast(pltpu.pack_elementwise([x[0], x[1]], packed_dtype=BF16), U32)


def _strassen_lhs(a11, a12, a21, a22):
    return [v.astype(BF16) for v in (a11 + a22, a21 + a22, a11, a22, a11 + a12, a21 - a11, a12 - a22)]


def _strassen_products(lhs, w, e, rows, c0, width):
    n = w.shape[2] // 2
    lo, hi = slice(c0, c0 + width), slice(n + c0, n + c0 + width)
    rhs = (e.at[0, rows, lo], w.at[0, rows, lo], w.at[0, rows, hi], w.at[1, rows, lo],
           w.at[1, rows, hi], e.at[1, rows, lo], e.at[2, rows, lo])
    return [_dot(a, pltpu.bitcast(b[...], BF16)) for a, b in zip(lhs, rhs)]


def _strassen_combine(m):
    m1, m2, m3, m4, m5, m6, m7 = m
    return m1 + m4 - m5 + m7, m3 + m5, m2 + m4, m1 - m2 + m3 + m6


def _body(x_hbm, mem0_ref, wq_hbm, wk_hbm, wv_hbm, wo_hbm, w1_hbm, w3_hbm, w2_hbm,
          c_ref, wm_hbm, out_hbm,
          wqkv, wo32, pre_v, x_v, mod_v, mod1_v, hs_v, o_v, zero_v, sems,
          *, S, D, H, Dh, M, T, F, G, BM, FC):
    n_seg = S // T
    L = M + T
    HD = H * Dh
    UN = 2
    P = 8
    KC = 256
    n_kc = D // KC
    wo_src = wo_hbm.bitcast(U32)
    wm_src = wm_hbm.bitcast(U32)
    HP = H + 8
    XA = 9
    cp_x = pltpu.make_async_copy(x_hbm.at[pl.ds(0, XA)], x_v.at[pl.ds(0, XA)], sems.at[0])
    cp_x2 = pltpu.make_async_copy(x_hbm.at[pl.ds(XA, n_seg - XA)], x_v.at[pl.ds(XA, n_seg - XA)], sems.at[1])

    zero_v[...] = jnp.zeros(zero_v.shape, U32)

    def after(anchor):
        return pltpu.bitcast(anchor[0:8, 0:128], U32) & zero_v[...]

    def silu_c():
        return jnp.broadcast_to(_silu(c_ref[...].astype(F32)), (8, D)).astype(BF16)

    def ada1(x):
        return _layernorm(x.astype(F32)[:T - P]) * (1.0 + mod_v[0:1, D:2 * D]) + mod_v[0:1, 0:D]

    def startup(wm_v, raw, xp_v, xn_v, hp_v, sem_m, sem_w, sem_p):
        srcs = [w.bitcast(U32) for w in (wq_hbm, wk_hbm, wv_hbm)]
        n_j = 3 * n_kc
        R = n_seg * P

        def cp_w(j, t=0):
            return pltpu.make_async_copy(srcs[t].at[pl.ds((j % n_kc) * (KC // 2), KC // 2)],
                                         raw.at[pl.ds(j * (KC // 2), KC // 2), pl.ds(0, H)], sem_w.at[j])

        def cp_m(c, i):
            return pltpu.make_async_copy(wm_src.at[:, pl.ds(pl.multiple_of(i * D + c * KC, KC), KC)],
                                         wm_v.at[c, :, pl.ds(i * KC, KC)], sem_m.at[2 * c + i])

        def start(j):
            cp_m(j, 0).start()
            cp_m(j, 1).start()
            cp_w(j).start()

        def cp_o(i):
            r = pl.ds(pl.multiple_of(i * (HD // 16), HD // 16), HD // 16)
            return pltpu.make_async_copy(wo_src.at[r], wo32.at[r], sem_p.at[1 + i])

        cp_p = pltpu.make_async_copy(x_hbm.at[:, pl.ds(T - P, P), :], xp_v, sem_p.at[0])
        cp_p.start()
        start(0)

        cp_p.wait()

        def norm(i, carry):
            xn = _layernorm(xp_v[pl.ds(i * 8, 8)].astype(F32).reshape(8 * P, D))
            for c in range(n_kc):
                xn_v[c, pl.ds(pl.multiple_of(i * 8 * P, 8 * P), 8 * P), :] = xn[:, c * KC:(c + 1) * KC]
            return carry
        lax.fori_loop(0, n_seg // 8, norm, 0)
        start(1)
        raw2 = raw.reshape(3 * D // 2 * HP, Dh)

        def chunk(j, carry):
            t, c = j // n_kc, j % n_kc

            @pl.when(j < n_kc)
            def _():
                cp_m(c, 0).wait()
                cp_m(c, 1).wait()

                @pl.when(j + 2 < n_kc)
                def _():
                    start(j + 2)
                mod = _dot(silu_c(), pltpu.bitcast(wm_v[c], BF16))
                mod1_v[c] = mod
                h = xn_v[c] * (1.0 + mod[0:1, KC:]) + mod[0:1, :KC]
                parts = _strassen_lhs(h[:R // 2, :KC // 2], h[:R // 2, KC // 2:],
                                      h[R // 2:, :KC // 2], h[R // 2:, KC // 2:])
                for i, part in enumerate(parts):
                    hp_v[c, i] = pltpu.bitcast(part, U32)

            cp_w(j).wait()
            for src in (1, 2):
                @pl.when((j + 2) // n_kc == src)
                def _(src=src):
                    cp_w(j + 2, src).start()

            @pl.when(j >= n_j - 8)
            def _():
                cp_o(j - (n_j - 8)).start()

            @pl.when(j == n_j - 2)
            def _():
                cp_x.start()

            q4 = KC // 4
            for hp in range(H // 2):
                blk = []
                for half in range(2):
                    base = (j * 2 + half) * (q4 * HP) + hp
                    a = _unpack(raw2[pl.ds(base, q4, stride=HP), :])
                    b = _unpack(raw2[pl.ds(base + H // 2, q4, stride=HP), :])
                    blk += [jnp.stack([a[0], b[0]]), jnp.stack([a[1], b[1]])]
                b11, b12, b21, b22 = blk
                tiles = [_pack(v) for v in blk]
                cols = [slice((2 * hp + i) * Dh, (2 * hp + i + 1) * Dh) for i in range(2)]
                for i, tile in enumerate(tiles):
                    wqkv[t, pl.ds(pl.multiple_of((2 * c + i // 2) * q4, q4), q4), cols[i % 2]] = tile
                rhs = (_pack(b11 + b22), tiles[0], _pack(b12 - b22), _pack(b21 - b11), tiles[3],
                       _pack(b11 + b12), _pack(b21 + b22))
                cs = _strassen_combine([_dot(pltpu.bitcast(hp_v[c, i], BF16), pltpu.bitcast(rhs[i], BF16))
                                        for i in range(7)])
                for i, part in enumerate(cs):
                    dst = pre_v.at[t, (i // 2) * (R // 2):(i // 2 + 1) * (R // 2), cols[i % 2]]
                    dst[...] = jnp.where(c > 0, dst[...], 0.0) + part
            return carry

        lax.fori_loop(0, n_j, chunk, 0)
        for c in range(n_kc):
            mod_v[:, c * KC:(c + 1) * KC] = mod1_v[c, :, :KC]
            mod_v[:, D + c * KC:D + (c + 1) * KC] = mod1_v[c, :, KC:]
        for i in range(8):
            cp_o(i).wait()

    pl.run_scoped(startup,
                  pltpu.VMEM((n_kc, D // 2, 2 * KC), U32), pltpu.VMEM((3 * D // 2, HP, Dh), U32),
                  pltpu.VMEM((n_seg, P, D), x_hbm.dtype), pltpu.VMEM((n_kc, n_seg * P, KC), F32),
                  pltpu.VMEM((n_kc, 7, n_seg * P // 4, KC // 2), U32),
                  pltpu.SemaphoreType.DMA((2 * n_kc,)), pltpu.SemaphoreType.DMA((3 * n_kc,)),
                  pltpu.SemaphoreType.DMA((9,)))

    n_it = n_seg // UN
    n_prep = n_it // 2
    R1, R2 = D // 4, F // 4
    r1, r2 = R1 // n_prep, R2 // n_prep

    def main(w1_v, w3_v, w2_v, e1_v, e3_v, e2_v, wm_v, att_v, h2_v, sem_f, sem_y):
        ffn_w = ((w1_hbm, w1_v, e1_v, R1, r1), (w3_hbm, w3_v, e3_v, R1, r1), (w2_hbm, w2_v, e2_v, R2, r2))
        cp_f = [pltpu.make_async_copy(src.bitcast(U32).at[pl.ds(i * R, R)], w.at[i, pl.ds(0, R)],
                                      sem_f.at[2 * j + i])
                for j, (src, w, _, R, _) in enumerate(ffn_w) for i in range(2)]
        cp_m = pltpu.make_async_copy(wm_src.at[:, pl.ds(2 * D, 4 * D)], wm_v, sem_f.at[6])
        for _, w, _, R, r in ffn_w:
            w[:, R:R + r, :] = jnp.zeros((2, r, w.shape[2]), U32)

        pieces = [(j, r0, c0) for j, (_, w, _, _, r) in enumerate(ffn_w)
                  for r0 in range(0, r, 8) for c0 in range(0, w.shape[2] // 2, 128)]

        def prep_ffn(i, site, n_sites, anchor):
            for k, (j, r0, c0) in enumerate(pieces[site::n_sites]):
                tie = after(anchor[:, (k * 128) % anchor.shape[1]:])
                _, w, e, R, r = ffn_w[j]
                n = w.shape[2] // 2
                base = jnp.where(i >= n_it - n_prep, (i - (n_it - n_prep)) * r, R)
                rows = pl.ds(pl.multiple_of(base + r0, 8), 8)
                lo, hi = slice(c0, c0 + 128), slice(n + c0, n + c0 + 128)
                b11, b12 = _unpack(w[0, rows, lo] | tie), _unpack(w[0, rows, hi] | tie)
                b21, b22 = _unpack(w[1, rows, lo] | tie), _unpack(w[1, rows, hi] | tie)
                e[0, rows, lo] = _pack(b11 + b22)
                e[1, rows, lo] = _pack(b11 + b12)
                e[2, rows, lo] = _pack(b21 + b22)
                w[0, rows, hi] = _pack(b12 - b22)
                w[1, rows, lo] = _pack(b21 - b11)

        cp_x.wait()
        cp_x2.start()
        for cp in cp_f:
            cp.start()
        cp_m.start()
        hs_v[...] = pltpu.bitcast(
            jnp.concatenate([mem0_ref[...].astype(F32), ada1(x_v[0])], axis=0).astype(BF16), U32)
        scale = Dh ** -0.5
        n_g = H // G

        def step(s, side):
            KP = 2 * L
            ri = lax.broadcasted_iota(jnp.int32, (2 * L, KP), 0)
            ci = lax.broadcasted_iota(jnp.int32, (2 * L, KP), 1)
            same = ((ri >= L) == (ci >= L)) & (ci < 2 * L)
            rl = jnp.where(ri >= L, ri - L, ri)
            cl = jnp.where(ci >= L, ci - L, ci)
            keep = same & ((rl < M) | (rl >= cl))
            fill = jnp.where(same, -1e9 / scale, -jnp.inf).astype(F32)
            early = pl.ds(pl.multiple_of(s * P, P), P)

            def stack(a, p, rows=2 * L):
                parts = [a[:, (2 * p) * Dh:(2 * p + 1) * Dh], a[:, (2 * p + 1) * Dh:(2 * p + 2) * Dh]]
                if rows > 2 * L:
                    parts.append(jnp.zeros((rows - 2 * L, Dh), a.dtype))
                return jnp.concatenate(parts, axis=0)

            def gcols(g):
                return slice(g * G * Dh, (g + 1) * G * Dh)

            def proj(t, g):
                return jnp.concatenate([_dot(pltpu.bitcast(hs_v[...], BF16), pltpu.bitcast(wqkv[t, :, gcols(g)], BF16)),
                                        pre_v[t, early, gcols(g)]], axis=0)

            def scores(q, k):
                res = []
                for p in range(G // 2):
                    sc = jnp.where(keep, _dot(stack(q, p), stack(k, p, KP).astype(BF16), _NT), fill)
                    e = jnp.exp2((sc - jnp.max(sc, axis=-1, keepdims=True)) * (scale * _LOG2E))
                    den = jnp.sum(e, axis=-1, keepdims=True)
                    r = pl.reciprocal(den, approx=True)
                    res.append((e, r * (2.0 - den * r)))
                return res

            def values(g, res, v):
                for p, (e, inv) in enumerate(res):
                    o = _dot(e, stack(v, p, KP).astype(BF16)) * inv
                    h0 = g * G + 2 * p
                    o_v[:, h0 * Dh:(h0 + 1) * Dh] = o[0:L]
                    o_v[:, (h0 + 1) * Dh:(h0 + 2) * Dh] = o[L:2 * L]

            def outp(g):
                return _dot(o_v[:, gcols(g)],
                            pltpu.bitcast(wo32[g * G * Dh // 2:(g + 1) * G * Dh // 2, :], BF16))

            h_next = ada1(x_v[jnp.minimum(s + 1, n_seg - 1)])
            qk, sm, vv = {}, {}, {}
            for g in range(n_g):
                qk[g] = proj(0, g), proj(1, g)
                if g >= 1:
                    sm[g - 1] = scores(*qk.pop(g - 1))
            for g in range(n_g):
                vv[g] = proj(2, g)
                side(g, vv[g])
                if g == 0:
                    sm[n_g - 1] = scores(*qk.pop(n_g - 1))
                else:
                    values(g - 1, sm.pop(g - 1), vv.pop(g - 1))
            acc = outp(0)
            values(n_g - 1, sm.pop(n_g - 1), vv.pop(n_g - 1))
            for g in range(1, n_g):
                side(n_g - 1 + g, acc)
                acc = acc + outp(g)
            hs_v[...] = pltpu.bitcast(jnp.concatenate([acc[0:M], h_next], axis=0).astype(BF16), U32)
            att_v[pl.ds(pl.multiple_of(s * T, T), T), :] = acc[M:L]

        def steps(i, carry):
            @pl.when(i == (XA - 1) // UN)
            def _():
                cp_x2.wait()

            @pl.when(i == n_it - n_prep)
            def _():
                for cp in cp_f:
                    cp.wait()
            for j in range(UN):
                per = 2 * n_g - 1
                step(i * UN + j, lambda k, anchor, j=j: prep_ffn(i, j * per + k, UN * per, anchor))
            return carry

        lax.fori_loop(0, n_seg // UN, steps, 0)

        cp_m.wait()
        mod_v[:, 2 * D:6 * D] = _dot(silu_c(), pltpu.bitcast(wm_v[...], BF16))

        def resid(i):
            x = x_v[pl.ds(i * (BM // T), BM // T)].astype(F32).reshape(BM, D)
            return x + mod_v[0:1, 2 * D:3 * D] * att_v[pl.ds(pl.multiple_of(i * BM, BM), BM), :]

        def ada2(i):
            h2 = _layernorm(resid(i)) * (1.0 + mod_v[0:1, 4 * D:5 * D]) + mod_v[0:1, 3 * D:4 * D]
            hm, hd = BM // 2, D // 2
            return _strassen_lhs(h2[:hm, :hd], h2[:hm, hd:], h2[hm:, :hd], h2[hm:, hd:])

        def put_h2(parts):
            for j, part in enumerate(parts):
                h2_v[j] = pltpu.bitcast(part, U32)

        put_h2(ada2(0))

        def out_copy(i):
            r = pl.ds(i * (BM // T), BM // T)
            return pltpu.make_async_copy(x_v.at[r], out_hbm.at[r], sem_y.at[i])

        def ffn(i, carry):
            lhs = [pltpu.bitcast(h2_v[j], BF16) for j in range(7)]
            h2_next = ada2(jnp.minimum(i + 1, S // BM - 1))
            acc = None
            for c0 in range(0, F // 2, FC):
                gate = _strassen_combine(_strassen_products(lhs, w1_v, e1_v, slice(0, R1), c0, FC))
                up = _strassen_combine(_strassen_products(lhs, w3_v, e3_v, slice(0, R1), c0, FC))
                act = _strassen_lhs(*[_silu(g) * u for g, u in zip(gate, up)])
                m = _strassen_products(act, w2_v, e2_v, slice(c0 // 2, (c0 + FC) // 2), 0, D // 2)
                acc = m if acc is None else [x + y for x, y in zip(acc, m)]
            c11, c12, c21, c22 = _strassen_combine(acc)
            ffn_out = jnp.concatenate([jnp.concatenate([c11, c12], axis=1),
                                       jnp.concatenate([c21, c22], axis=1)], axis=0)
            y = resid(i) + mod_v[0:1, 5 * D:6 * D] * ffn_out
            x_v[pl.ds(i * (BM // T), BM // T)] = y.reshape(BM // T, T, D).astype(x_v.dtype)
            put_h2(h2_next)
            out_copy(i).start()
            return carry

        lax.fori_loop(0, S // BM, ffn, 0)
        for i in range(S // BM):
            out_copy(i).wait()

    pl.run_scoped(main,
                  pltpu.VMEM((2, R1 + r1, F), U32), pltpu.VMEM((2, R1 + r1, F), U32),
                  pltpu.VMEM((2, R2 + r2, D), U32),
                  pltpu.VMEM((3, R1 + r1, F // 2), U32), pltpu.VMEM((3, R1 + r1, F // 2), U32),
                  pltpu.VMEM((3, R2 + r2, D // 2), U32),
                  pltpu.VMEM((D // 2, 4 * D), U32), pltpu.VMEM((S, D), F32),
                  pltpu.VMEM((7, BM // 4, D // 2), U32),
                  pltpu.SemaphoreType.DMA((7,)), pltpu.SemaphoreType.DMA((S // BM,)))


@functools.partial(jax.jit, static_argnames=("A_seg_len",))
def pallas_adaLN_cond__memory_aug_recurrent_mem_tr__glu_gated_swiglu__prompt_kernel(
    A_x, A_mem0, A_Wq, A_Wk, A_Wv, A_Wo, A_seg_len, B_x, B_w1, B_w3, B_w2, c, w_mod,
):
    del B_x
    B, S, D = A_x.shape
    _, H, Dh = A_Wq.shape
    M, T, F = A_mem0.shape[1], int(A_seg_len), B_w1.shape[1]
    assert B == 1 and S % T == 0
    L, HD = M + T, H * Dh
    hbm = pl.BlockSpec(memory_space=pl.ANY)
    vmem = pl.BlockSpec(memory_space=pltpu.VMEM)
    body = functools.partial(_body, S=S, D=D, H=H, Dh=Dh, M=M, T=T, F=F, G=8, BM=128, FC=1792)
    out = pl.pallas_call(
        body,
        out_shape=jax.ShapeDtypeStruct((S // T, T, D), A_x.dtype),
        in_specs=[hbm, vmem, hbm, hbm, hbm, hbm, hbm, hbm, hbm, vmem, hbm],
        out_specs=hbm,
        scratch_shapes=[
            pltpu.VMEM((3, D // 2, HD), U32), pltpu.VMEM((HD // 2, D), U32),
            pltpu.VMEM((3, S // T * 8, HD), F32),
            pltpu.VMEM((S // T, T, D), A_x.dtype), pltpu.VMEM((8, 6 * D), F32),
            pltpu.VMEM((D // 256, 8, 512), F32),
            pltpu.VMEM(((L - 8) // 2, D), U32), pltpu.VMEM((L, HD), F32), pltpu.VMEM((8, 128), U32),
            pltpu.SemaphoreType.DMA((2,)),
        ],
        compiler_params=pltpu.CompilerParams(vmem_limit_bytes=126 * 2**20, flags={'XLA_TPU_EVENLY_DISTRIBUTE_CRITICAL_NODES': True}),
    )(A_x.reshape(S // T, T, D), A_mem0.reshape(M, D),
      A_Wq.reshape(D // 2, 2 * H, Dh), A_Wk.reshape(D // 2, 2 * H, Dh), A_Wv.reshape(D // 2, 2 * H, Dh), A_Wo.reshape(HD, D),
      B_w1, B_w3, B_w2, c, w_mod)
    return out.reshape(B, S, D)
```

```python
import functools

import jax
import jax.numpy as jnp
from jax import lax
import jax.experimental.pallas as pl
import jax.experimental.pallas.tpu as pltpu

F32, BF16, U32 = jnp.float32, jnp.bfloat16, jnp.uint32
_LOG2E = 1.4426950408889634
_NN = (((1,), (0,)), ((), ()))
_NT = (((1,), (1,)), ((), ()))


def _dot(a, b, dims=_NN):
    return lax.dot_general(a, b, dims, preferred_element_type=F32)


def _layernorm(x, eps=1e-5):
    m = jnp.mean(x, axis=-1, keepdims=True)
    d = x - m
    v = jnp.mean(d * d, axis=-1, keepdims=True)
    return d * lax.rsqrt(v + eps)


def _silu(x):
    h = 0.5 * x
    return h + h * jnp.tanh(h)


def _unpack(w):
    return jnp.stack([pltpu.unpack_elementwise(w, index=i, packed_dtype=BF16, unpacked_dtype=F32)
                      for i in range(2)])


def _pack(x):
    return pltpu.bitcast(pltpu.pack_elementwise([x[0], x[1]], packed_dtype=BF16), U32)


def _strassen_lhs(a, levels):
    if levels == 0:
        return [a.astype(BF16)]
    m, k = a.shape[0] // 2, a.shape[1] // 2
    a11, a12, a21, a22 = a[:m, :k], a[:m, k:], a[m:, :k], a[m:, k:]
    return [x for v in (a11 + a22, a21 + a22, a11, a22, a11 + a12, a21 - a11, a12 - a22)
            for x in _strassen_lhs(v, levels - 1)]


def _strassen_rhs(blocks):
    if len(blocks) == 1:
        return blocks
    n = len(blocks) // 4
    b11, b12, b21, b22 = (blocks[i * n:(i + 1) * n] for i in range(4))
    add = lambda x, y: [u + v for u, v in zip(x, y)]
    sub = lambda x, y: [u - v for u, v in zip(x, y)]
    return [x for v in (add(b11, b22), b11, sub(b12, b22), sub(b21, b11), b22, add(b11, b12), add(b21, b22))
            for x in _strassen_rhs(v)]


def _strassen_blocks(levels):
    out = [(0, 0, 0)]
    for _ in range(levels):
        out = [(2 * i + q // 2, 2 * j + q % 2, 7 * slot + 1 + q) for i, j, slot in out for q in range(4)]
    return out


def _strassen_out(m):
    if len(m) == 1:
        return m[0]
    n = len(m) // 7
    m1, m2, m3, m4, m5, m6, m7 = (_strassen_out(m[i * n:(i + 1) * n]) for i in range(7))
    return jnp.concatenate([jnp.concatenate([m1 + m4 - m5 + m7, m3 + m5], axis=1),
                            jnp.concatenate([m2 + m4, m1 - m2 + m3 + m6], axis=1)], axis=0)


def _body(x_hbm, mem0_ref, wq_hbm, wk_hbm, wv_hbm, wo_hbm, w1_hbm, w3_hbm, w2_hbm,
          c_ref, wm_hbm, out_hbm,
          wqkv, wo32, pre_v, x_v, mod_v, mod1_v, hs_v, o_v, zero_v, sems,
          *, S, D, H, Dh, M, T, F, G, BM, LV):
    n_seg = S // T
    L = M + T
    HD = H * Dh
    UN = 2
    P = 8
    KC = 256
    n_kc = D // KC
    wo_src = wo_hbm.bitcast(U32)
    wm_src = wm_hbm.bitcast(U32)
    HP = H + 8
    XA = 9
    cp_x = pltpu.make_async_copy(x_hbm.at[pl.ds(0, XA)], x_v.at[pl.ds(0, XA)], sems.at[0])
    cp_x2 = pltpu.make_async_copy(x_hbm.at[pl.ds(XA, n_seg - XA)], x_v.at[pl.ds(XA, n_seg - XA)], sems.at[1])

    zero_v[...] = jnp.zeros(zero_v.shape, U32)

    def after(anchor):
        return pltpu.bitcast(anchor[0:8, 0:128], U32) & zero_v[...]

    def silu_c():
        return jnp.broadcast_to(_silu(c_ref[...].astype(F32)), (8, D)).astype(BF16)

    def ada1(x):
        return _layernorm(x.astype(F32)[:T - P]) * (1.0 + mod_v[0:1, D:2 * D]) + mod_v[0:1, 0:D]

    def startup(wm_v, wr_v, raw, xp_v, xn_v, hp_v, sem_m, sem_w, sem_p):
        srcs = [w.bitcast(U32) for w in (wq_hbm, wk_hbm, wv_hbm)]
        n_j = 3 * n_kc
        R = n_seg * P

        def cp_w(j, t=0):
            return pltpu.make_async_copy(srcs[t].at[pl.ds((j % n_kc) * (KC // 2), KC // 2)],
                                         raw.at[pl.ds(j * (KC // 2), KC // 2), pl.ds(0, H)], sem_w.at[j])

        def cp_m(c, i):
            return pltpu.make_async_copy(wm_src.at[:, pl.ds(pl.multiple_of(i * D + c * KC, KC), KC)],
                                         wm_v.at[c, :, pl.ds(i * KC, KC)], sem_m.at[2 * c + i])

        def start(j):
            cp_m(j, 0).start()
            cp_m(j, 1).start()
            cp_w(j).start()

        def cp_o(i):
            r = pl.ds(pl.multiple_of(i * (HD // 16), HD // 16), HD // 16)
            return pltpu.make_async_copy(wo_src.at[r], wo32.at[r], sem_p.at[1 + i])

        def cp_r(i):
            r = pl.ds(pl.multiple_of(i * (D // 16), D // 16), D // 16)
            return pltpu.make_async_copy(wm_src.at[r, pl.ds(2 * D, 4 * D)], wr_v.at[r], sem_p.at[9 + i])

        cp_p = pltpu.make_async_copy(x_hbm.at[:, pl.ds(T - P, P), :], xp_v, sem_p.at[0])
        cp_p.start()
        start(0)

        cp_p.wait()

        def norm(i, carry):
            xn = _layernorm(xp_v[pl.ds(i * 8, 8)].astype(F32).reshape(8 * P, D))
            for c in range(n_kc):
                xn_v[c, pl.ds(pl.multiple_of(i * 8 * P, 8 * P), 8 * P), :] = xn[:, c * KC:(c + 1) * KC]
            return carry
        lax.fori_loop(0, n_seg // 8, norm, 0)
        start(1)
        raw2 = raw.reshape(3 * D // 2 * HP, Dh)

        def chunk(j, carry):
            t, c = j // n_kc, j % n_kc

            @pl.when(j < n_kc)
            def _():
                cp_m(c, 0).wait()
                cp_m(c, 1).wait()

                @pl.when(j + 2 < n_kc)
                def _():
                    start(j + 2)
                mod = _dot(silu_c(), pltpu.bitcast(wm_v[c], BF16))
                mod1_v[c] = mod
                h = xn_v[c] * (1.0 + mod[0:1, KC:]) + mod[0:1, :KC]
                for i, part in enumerate(_strassen_lhs(h, 1)):
                    hp_v[c, i] = pltpu.bitcast(part, U32)

            cp_w(j).wait()
            for src in (1, 2):
                @pl.when((j + 2) // n_kc == src)
                def _(src=src):
                    cp_w(j + 2, src).start()

            @pl.when(j >= n_j - 8)
            def _():
                cp_r(j - (n_j - 8)).start()
                cp_o(j - (n_j - 8)).start()

            @pl.when(j == n_j - 2)
            def _():
                cp_x.start()

            q4 = KC // 4
            for hp in range(H // 2):
                blk = []
                for half in range(2):
                    base = (j * 2 + half) * (q4 * HP) + hp
                    a = _unpack(raw2[pl.ds(base, q4, stride=HP), :])
                    b = _unpack(raw2[pl.ds(base + H // 2, q4, stride=HP), :])
                    blk += [jnp.stack([a[0], b[0]]), jnp.stack([a[1], b[1]])]
                tiles = [_pack(v) for v in blk]
                cols = [slice((2 * hp + i) * Dh, (2 * hp + i + 1) * Dh) for i in range(2)]
                for i, tile in enumerate(tiles):
                    wqkv[t, pl.ds(pl.multiple_of((2 * c + i // 2) * q4, q4), q4), cols[i % 2]] = tile
                part = _strassen_out([_dot(pltpu.bitcast(hp_v[c, i], BF16), pltpu.bitcast(_pack(w), BF16))
                                      for i, w in enumerate(_strassen_rhs(blk))])
                dst = pre_v.at[t, :, 2 * hp * Dh:(2 * hp + 2) * Dh]
                dst[...] = jnp.where(c > 0, dst[...], 0.0) + part
            return carry

        lax.fori_loop(0, n_j, chunk, 0)
        for c in range(n_kc):
            mod_v[:, c * KC:(c + 1) * KC] = mod1_v[c, :, :KC]
            mod_v[:, D + c * KC:D + (c + 1) * KC] = mod1_v[c, :, KC:]
        for i in range(8):
            cp_r(i).wait()
        mod_v[:, 2 * D:6 * D] = _dot(silu_c(), pltpu.bitcast(wr_v[...], BF16))
        for i in range(8):
            cp_o(i).wait()

    pl.run_scoped(startup,
                  pltpu.VMEM((n_kc, D // 2, 2 * KC), U32), pltpu.VMEM((D // 2, 4 * D), U32),
                  pltpu.VMEM((3 * D // 2, HP, Dh), U32),
                  pltpu.VMEM((n_seg, P, D), x_hbm.dtype), pltpu.VMEM((n_kc, n_seg * P, KC), F32),
                  pltpu.VMEM((n_kc, 7, n_seg * P // 4, KC // 2), U32),
                  pltpu.SemaphoreType.DMA((2 * n_kc,)), pltpu.SemaphoreType.DMA((3 * n_kc,)),
                  pltpu.SemaphoreType.DMA((17,)))

    n_it = n_seg // UN
    first_prep = n_it // 2
    ffn_cfg = ((w1_hbm, LV[0]), (w3_hbm, LV[0]), (w2_hbm, LV[1]))

    def main(e1_v, e3_v, e2_v, h2_v, sem_f, sem_y):
        cp_f, pieces = [], []
        for (src, lv), e in zip(ffn_cfg, (e1_v, e3_v, e2_v)):
            R, n = e.shape[1] - 8, e.shape[2]
            for bi, bj, slot in _strassen_blocks(lv):
                cp_f.append(pltpu.make_async_copy(src.bitcast(U32).at[pl.ds(bi * R, R), pl.ds(bj * n, n)],
                                                  e.at[slot, pl.ds(0, R)], sem_f.at[len(cp_f)]))
                e[slot, R:R + 8, :] = jnp.zeros((8, n), U32)
            r = 8 * pl.cdiv(R // 8, n_it - first_prep)
            groups = [range(7)] if lv == 1 else [range(7 * o, 7 * o + 7) for o in (0, 5, 6, 2, 3, 1, 4)]
            pieces += [(e, lv, r, r0, c0, grp) for r0 in range(0, r, 8) for c0 in range(0, n, 128)
                       for grp in groups]

        def prep_ffn(i, site, n_sites, anchor):
            per = pl.cdiv(len(pieces), n_sites)
            for k, (e, lv, r, r0, c0, grp) in enumerate(pieces[site * per:(site + 1) * per]):
                tie = after(anchor[:, (k * 128) % anchor.shape[1]:])
                R = e.shape[1] - 8
                row = jnp.where(i >= first_prep, jnp.minimum((i - first_prep) * r + r0, R), R)
                rows, cols = pl.ds(pl.multiple_of(row, 8), 8), slice(c0, c0 + 128)
                blocks = [_unpack(e[slot, rows, cols] | tie) for _, _, slot in _strassen_blocks(lv)]
                for slot, w in enumerate(_strassen_rhs(blocks)):
                    if slot in grp and not any(w is blk for blk in blocks):
                        e[slot, rows, cols] = _pack(w)

        cp_x.wait()
        cp_x2.start()
        for cp in cp_f:
            cp.start()
        hs_v[...] = pltpu.bitcast(
            jnp.concatenate([mem0_ref[...].astype(F32), ada1(x_v[0])], axis=0).astype(BF16), U32)
        scale = Dh ** -0.5
        n_g = H // G

        def step(s, side):
            KP = 2 * L
            ri = lax.broadcasted_iota(jnp.int32, (2 * L, KP), 0)
            ci = lax.broadcasted_iota(jnp.int32, (2 * L, KP), 1)
            same = ((ri >= L) == (ci >= L)) & (ci < 2 * L)
            rl = jnp.where(ri >= L, ri - L, ri)
            cl = jnp.where(ci >= L, ci - L, ci)
            keep = same & ((rl < M) | (rl >= cl))
            fill = jnp.where(same, -1e9 / scale, -jnp.inf).astype(F32)
            early = pl.ds(pl.multiple_of(s * P, P), P)

            def stack(a, p, rows=2 * L):
                parts = [a[:, (2 * p) * Dh:(2 * p + 1) * Dh], a[:, (2 * p + 1) * Dh:(2 * p + 2) * Dh]]
                if rows > 2 * L:
                    parts.append(jnp.zeros((rows - 2 * L, Dh), a.dtype))
                return jnp.concatenate(parts, axis=0)

            def gcols(g):
                return slice(g * G * Dh, (g + 1) * G * Dh)

            def proj(t, g):
                return jnp.concatenate([_dot(pltpu.bitcast(hs_v[...], BF16), pltpu.bitcast(wqkv[t, :, gcols(g)], BF16)),
                                        pre_v[t, early, gcols(g)]], axis=0)

            def scores(q, k):
                res = []
                for p in range(G // 2):
                    sc = jnp.where(keep, _dot(stack(q, p), stack(k, p, KP).astype(BF16), _NT), fill)
                    e = jnp.exp2((sc - jnp.max(sc, axis=-1, keepdims=True)) * (scale * _LOG2E))
                    den = jnp.sum(e, axis=-1, keepdims=True)
                    r = pl.reciprocal(den, approx=True)
                    res.append((e, r * (2.0 - den * r)))
                return res

            def values(g, res, v):
                for p, (e, inv) in enumerate(res):
                    o = _dot(e, stack(v, p, KP).astype(BF16)) * inv
                    h0 = g * G + 2 * p
                    o_v[:, h0 * Dh:(h0 + 1) * Dh] = o[0:L]
                    o_v[:, (h0 + 1) * Dh:(h0 + 2) * Dh] = o[L:2 * L]

            def outp(g):
                return _dot(o_v[:, gcols(g)],
                            pltpu.bitcast(wo32[g * G * Dh // 2:(g + 1) * G * Dh // 2, :], BF16))

            h_next = ada1(x_v[jnp.minimum(s + 1, n_seg - 1)])
            qk, sm, vv = {}, {}, {}
            for g in range(n_g):
                qk[g] = proj(0, g), proj(1, g)
                if g >= 1:
                    sm[g - 1] = scores(*qk.pop(g - 1))
                side(g, qk[g][1])
            for g in range(n_g):
                vv[g] = proj(2, g)
                side(n_g + g, vv[g])
                if g == 0:
                    sm[n_g - 1] = scores(*qk.pop(n_g - 1))
                else:
                    values(g - 1, sm.pop(g - 1), vv.pop(g - 1))
            acc = outp(0)
            values(n_g - 1, sm.pop(n_g - 1), vv.pop(n_g - 1))
            for g in range(1, n_g):
                side(2 * n_g - 1 + g, acc)
                acc = acc + outp(g)
            hs_v[...] = pltpu.bitcast(jnp.concatenate([acc[0:M], h_next], axis=0).astype(BF16), U32)
            x_v[s] = (x_v[s].astype(F32) + mod_v[0:1, 2 * D:3 * D] * acc[M:L]).astype(x_v.dtype)

        def steps(i, carry):
            @pl.when(i == (XA - 1) // UN)
            def _():
                cp_x2.wait()

            @pl.when(i == first_prep)
            def _():
                for cp in cp_f:
                    cp.wait()
            for j in range(UN):
                per = 3 * n_g - 1
                step(i * UN + j, lambda k, anchor, j=j: prep_ffn(i, j * per + k, UN * per, anchor))
            return carry

        lax.fori_loop(0, n_seg // UN, steps, 0)

        def resid(i):
            return x_v[pl.ds(i * (BM // T), BM // T)].astype(F32).reshape(BM, D)

        def ada2(i):
            h2 = _layernorm(resid(i)) * (1.0 + mod_v[0:1, 4 * D:5 * D]) + mod_v[0:1, 3 * D:4 * D]
            return _strassen_lhs(h2, LV[0])

        def matmul(lhs, e):
            return _strassen_out([_dot(a, pltpu.bitcast(e[k, 0:e.shape[1] - 8, :], BF16))
                                  for k, a in enumerate(lhs)])

        def put_h2(parts):
            for j, part in enumerate(parts):
                h2_v[j] = pltpu.bitcast(part, U32)

        put_h2(ada2(0))

        def out_copy(i):
            r = pl.ds(i * (BM // T), BM // T)
            return pltpu.make_async_copy(x_v.at[r], out_hbm.at[r], sem_y.at[i])

        def ffn(i, carry):
            lhs = [pltpu.bitcast(h2_v[j], BF16) for j in range(h2_v.shape[0])]
            h2_next = ada2(jnp.minimum(i + 1, S // BM - 1))
            act = _silu(matmul(lhs, e1_v)) * matmul(lhs, e3_v)
            ffn_out = matmul(_strassen_lhs(act, LV[1]), e2_v)
            y = resid(i) + mod_v[0:1, 5 * D:6 * D] * ffn_out
            x_v[pl.ds(i * (BM // T), BM // T)] = y.reshape(BM // T, T, D).astype(x_v.dtype)
            put_h2(h2_next)
            out_copy(i).start()
            return carry

        lax.fori_loop(0, S // BM, ffn, 0)
        for i in range(S // BM):
            out_copy(i).wait()

    pl.run_scoped(main,
                  *[pltpu.VMEM((7 ** lv, (w.shape[0] >> (lv + 1)) + 8, w.shape[1] >> lv), U32)
                    for w, lv in ffn_cfg],
                  pltpu.VMEM((7 ** LV[0], BM >> (LV[0] + 1), D >> LV[0]), U32),
                  pltpu.SemaphoreType.DMA((sum(4 ** lv for _, lv in ffn_cfg),)),
                  pltpu.SemaphoreType.DMA((S // BM,)))


@functools.partial(jax.jit, static_argnames=("A_seg_len",))
def pallas_adaLN_cond__memory_aug_recurrent_mem_tr__glu_gated_swiglu__prompt_kernel(
    A_x, A_mem0, A_Wq, A_Wk, A_Wv, A_Wo, A_seg_len, B_x, B_w1, B_w3, B_w2, c, w_mod,
):
    del B_x
    B, S, D = A_x.shape
    _, H, Dh = A_Wq.shape
    M, T, F = A_mem0.shape[1], int(A_seg_len), B_w1.shape[1]
    assert B == 1 and S % T == 0
    L, HD = M + T, H * Dh
    hbm = pl.BlockSpec(memory_space=pl.ANY)
    vmem = pl.BlockSpec(memory_space=pltpu.VMEM)
    body = functools.partial(_body, S=S, D=D, H=H, Dh=Dh, M=M, T=T, F=F, G=8, BM=128, LV=(2, 1))
    out = pl.pallas_call(
        body,
        out_shape=jax.ShapeDtypeStruct((S // T, T, D), A_x.dtype),
        in_specs=[hbm, vmem, hbm, hbm, hbm, hbm, hbm, hbm, hbm, vmem, hbm],
        out_specs=hbm,
        scratch_shapes=[
            pltpu.VMEM((3, D // 2, HD), U32), pltpu.VMEM((HD // 2, D), U32),
            pltpu.VMEM((3, S // T * 8, HD), F32),
            pltpu.VMEM((S // T, T, D), A_x.dtype), pltpu.VMEM((8, 6 * D), F32),
            pltpu.VMEM((D // 256, 8, 512), F32),
            pltpu.VMEM(((L - 8) // 2, D), U32), pltpu.VMEM((L, HD), F32), pltpu.VMEM((8, 128), U32),
            pltpu.SemaphoreType.DMA((2,)),
        ],
        compiler_params=pltpu.CompilerParams(vmem_limit_bytes=126 * 2**20, flags={'XLA_TPU_EVENLY_DISTRIBUTE_CRITICAL_NODES': True}),
    )(A_x.reshape(S // T, T, D), A_mem0.reshape(M, D),
      A_Wq.reshape(D // 2, 2 * H, Dh), A_Wk.reshape(D // 2, 2 * H, Dh), A_Wv.reshape(D // 2, 2 * H, Dh), A_Wo.reshape(HD, D),
      B_w1, B_w3, B_w2, c, w_mod)
    return out.reshape(B, S, D)
```

```python
import functools

import jax
import jax.numpy as jnp
from jax import lax
import jax.experimental.pallas as pl
import jax.experimental.pallas.tpu as pltpu

F32, BF16, U32 = jnp.float32, jnp.bfloat16, jnp.uint32
_LOG2E = 1.4426950408889634
_NN = (((1,), (0,)), ((), ()))
_NT = (((1,), (1,)), ((), ()))


def _dot(a, b, dims=_NN):
    return lax.dot_general(a, b, dims, preferred_element_type=F32)


def _layernorm(x, eps=1e-5):
    m = jnp.mean(x, axis=-1, keepdims=True)
    d = x - m
    v = jnp.mean(d * d, axis=-1, keepdims=True)
    return d * lax.rsqrt(v + eps)


def _silu(x):
    h = 0.5 * x
    return h + h * jnp.tanh(h)


def _unpack(w):
    return jnp.stack([pltpu.unpack_elementwise(w, index=i, packed_dtype=BF16, unpacked_dtype=F32)
                      for i in range(2)])


def _pack(x):
    return pltpu.bitcast(pltpu.pack_elementwise([x[0], x[1]], packed_dtype=BF16), U32)


def _strassen_lhs(a, levels):
    if levels == 0:
        return [a.astype(BF16)]
    m, k = a.shape[0] // 2, a.shape[1] // 2
    a11, a12, a21, a22 = a[:m, :k], a[:m, k:], a[m:, :k], a[m:, k:]
    return [x for v in (a11 + a22, a21 + a22, a11, a22, a11 + a12, a21 - a11, a12 - a22)
            for x in _strassen_lhs(v, levels - 1)]


def _strassen_rhs(blocks):
    if len(blocks) == 1:
        return blocks
    n = len(blocks) // 4
    b11, b12, b21, b22 = (blocks[i * n:(i + 1) * n] for i in range(4))
    add = lambda x, y: [u + v for u, v in zip(x, y)]
    sub = lambda x, y: [u - v for u, v in zip(x, y)]
    return [x for v in (add(b11, b22), b11, sub(b12, b22), sub(b21, b11), b22, add(b11, b12), add(b21, b22))
            for x in _strassen_rhs(v)]


def _strassen_blocks(levels):
    out = [(0, 0, 0)]
    for _ in range(levels):
        out = [(2 * i + q // 2, 2 * j + q % 2, 7 * slot + 1 + q) for i, j, slot in out for q in range(4)]
    return out


def _strassen_out(m):
    if len(m) == 1:
        return m[0]
    n = len(m) // 7
    m1, m2, m3, m4, m5, m6, m7 = (_strassen_out(m[i * n:(i + 1) * n]) for i in range(7))
    return jnp.concatenate([jnp.concatenate([m1 + m4 - m5 + m7, m3 + m5], axis=1),
                            jnp.concatenate([m2 + m4, m1 - m2 + m3 + m6], axis=1)], axis=0)


def _body(x_hbm, mem0_ref, wq_hbm, wk_hbm, wv_hbm, wo_hbm, w1_hbm, w3_hbm, w2_hbm,
          c_ref, wm_hbm, out_hbm,
          wqkv, wo32, pre_v, x_v, mod_v, mod1_v, hs_v, o_v, zero_v, sems,
          *, S, D, H, Dh, M, T, F, G, BM, FC, LV):
    n_seg = S // T
    L = M + T
    HD = H * Dh
    UN = 2
    P = 8
    KC = 256
    n_kc = D // KC
    wo_src = wo_hbm.bitcast(U32)
    wm_src = wm_hbm.bitcast(U32)
    HP = H + 8
    XA = 9
    cp_x = pltpu.make_async_copy(x_hbm.at[pl.ds(0, XA)], x_v.at[pl.ds(0, XA)], sems.at[0])
    cp_x2 = pltpu.make_async_copy(x_hbm.at[pl.ds(XA, n_seg - XA)], x_v.at[pl.ds(XA, n_seg - XA)], sems.at[1])

    zero_v[...] = jnp.zeros(zero_v.shape, U32)

    def after(anchor):
        return pltpu.bitcast(anchor[0:8, 0:128], U32) & zero_v[...]

    def silu_c():
        return jnp.broadcast_to(_silu(c_ref[...].astype(F32)), (8, D)).astype(BF16)

    def ada1(x):
        return _layernorm(x.astype(F32)[:T - P]) * (1.0 + mod_v[0:1, D:2 * D]) + mod_v[0:1, 0:D]

    def startup(wm_v, wr_v, raw, xp_v, xn_v, hp_v, sem_m, sem_w, sem_p):
        srcs = [w.bitcast(U32) for w in (wq_hbm, wk_hbm, wv_hbm)]
        n_j = 3 * n_kc
        R = n_seg * P

        def cp_w(j, t=0):
            return pltpu.make_async_copy(srcs[t].at[pl.ds((j % n_kc) * (KC // 2), KC // 2)],
                                         raw.at[pl.ds(j * (KC // 2), KC // 2), pl.ds(0, H)], sem_w.at[j])

        def cp_m(c, i):
            return pltpu.make_async_copy(wm_src.at[:, pl.ds(pl.multiple_of(i * D + c * KC, KC), KC)],
                                         wm_v.at[c, :, pl.ds(i * KC, KC)], sem_m.at[2 * c + i])

        def start(j):
            cp_m(j, 0).start()
            cp_m(j, 1).start()
            cp_w(j).start()

        def cp_o(i):
            r = pl.ds(pl.multiple_of(i * (HD // 16), HD // 16), HD // 16)
            return pltpu.make_async_copy(wo_src.at[r], wo32.at[r], sem_p.at[1 + i])

        def cp_r(i):
            r = pl.ds(pl.multiple_of(i * (D // 16), D // 16), D // 16)
            return pltpu.make_async_copy(wm_src.at[r, pl.ds(2 * D, 4 * D)], wr_v.at[r], sem_p.at[9 + i])

        cp_p = pltpu.make_async_copy(x_hbm.at[:, pl.ds(T - P, P), :], xp_v, sem_p.at[0])
        cp_p.start()
        start(0)

        cp_p.wait()

        def norm(i, carry):
            xn = _layernorm(xp_v[pl.ds(i * 8, 8)].astype(F32).reshape(8 * P, D))
            for c in range(n_kc):
                xn_v[c, pl.ds(pl.multiple_of(i * 8 * P, 8 * P), 8 * P), :] = xn[:, c * KC:(c + 1) * KC]
            return carry
        lax.fori_loop(0, n_seg // 8, norm, 0)
        start(1)
        raw2 = raw.reshape(3 * D // 2 * HP, Dh)

        def chunk(j, carry):
            t, c = j // n_kc, j % n_kc

            @pl.when(j < n_kc)
            def _():
                cp_m(c, 0).wait()
                cp_m(c, 1).wait()

                @pl.when(j + 2 < n_kc)
                def _():
                    start(j + 2)
                mod = _dot(silu_c(), pltpu.bitcast(wm_v[c], BF16))
                mod1_v[c] = mod
                h = xn_v[c] * (1.0 + mod[0:1, KC:]) + mod[0:1, :KC]
                for i, part in enumerate(_strassen_lhs(h, 1)):
                    hp_v[c, i] = pltpu.bitcast(part, U32)

            cp_w(j).wait()
            for src in (1, 2):
                @pl.when((j + 2) // n_kc == src)
                def _(src=src):
                    cp_w(j + 2, src).start()

            @pl.when(j >= n_j - 8)
            def _():
                cp_r(j - (n_j - 8)).start()
                cp_o(j - (n_j - 8)).start()

            @pl.when(j == n_j - 2)
            def _():
                cp_x.start()

            q4 = KC // 4
            for hp in range(H // 2):
                blk = []
                for half in range(2):
                    base = (j * 2 + half) * (q4 * HP) + hp
                    a = _unpack(raw2[pl.ds(base, q4, stride=HP), :])
                    b = _unpack(raw2[pl.ds(base + H // 2, q4, stride=HP), :])
                    blk += [jnp.stack([a[0], b[0]]), jnp.stack([a[1], b[1]])]
                tiles = [_pack(v) for v in blk]
                cols = [slice((2 * hp + i) * Dh, (2 * hp + i + 1) * Dh) for i in range(2)]
                for i, tile in enumerate(tiles):
                    wqkv[t, pl.ds(pl.multiple_of((2 * c + i // 2) * q4, q4), q4), cols[i % 2]] = tile
                part = _strassen_out([_dot(pltpu.bitcast(hp_v[c, i], BF16), pltpu.bitcast(_pack(w), BF16))
                                      for i, w in enumerate(_strassen_rhs(blk))])
                dst = pre_v.at[t, :, 2 * hp * Dh:(2 * hp + 2) * Dh]
                dst[...] = jnp.where(c > 0, dst[...], 0.0) + part
            return carry

        lax.fori_loop(0, n_j, chunk, 0)
        for c in range(n_kc):
            mod_v[:, c * KC:(c + 1) * KC] = mod1_v[c, :, :KC]
            mod_v[:, D + c * KC:D + (c + 1) * KC] = mod1_v[c, :, KC:]
        for i in range(8):
            cp_r(i).wait()
        mod_v[:, 2 * D:6 * D] = _dot(silu_c(), pltpu.bitcast(wr_v[...], BF16))
        for i in range(8):
            cp_o(i).wait()

    pl.run_scoped(startup,
                  pltpu.VMEM((n_kc, D // 2, 2 * KC), U32), pltpu.VMEM((D // 2, 4 * D), U32),
                  pltpu.VMEM((3 * D // 2, HP, Dh), U32),
                  pltpu.VMEM((n_seg, P, D), x_hbm.dtype), pltpu.VMEM((n_kc, n_seg * P, KC), F32),
                  pltpu.VMEM((n_kc, 7, n_seg * P // 4, KC // 2), U32),
                  pltpu.SemaphoreType.DMA((2 * n_kc,)), pltpu.SemaphoreType.DMA((3 * n_kc,)),
                  pltpu.SemaphoreType.DMA((17,)))

    n_it = n_seg // UN
    first_prep = n_it // 8
    ffn_cfg = ((w1_hbm, LV[0]), (w3_hbm, LV[0]), (w2_hbm, LV[1]))

    def main(e1_v, e3_v, e2_v, h2_v, sem_f, sem_y):
        cp_f, pieces = [], []
        for (src, lv), e in zip(ffn_cfg, (e1_v, e3_v, e2_v)):
            R, n = e.shape[1] - 8, e.shape[2]
            for bi, bj, slot in _strassen_blocks(lv):
                cp_f.append(pltpu.make_async_copy(src.bitcast(U32).at[pl.ds(bi * R, R), pl.ds(bj * n, n)],
                                                  e.at[slot, pl.ds(0, R)], sem_f.at[len(cp_f)]))
                e[slot, R:R + 8, 0:128] = jnp.zeros((8, 128), U32)
            per_it = pl.cdiv(R // 8 * (n // 128), n_it - first_prep)
            groups = [range(7)] if lv == 1 else [range(7 * o, 7 * o + 7) for o in (0, 5, 6, 2, 3, 1, 4)]
            pieces += [(e, lv, per_it, u, grp) for u in range(per_it) for grp in groups]

        def prep_ffn(i, site, n_sites, anchor):
            per = pl.cdiv(len(pieces), n_sites)
            for k, (e, lv, per_it, u, grp) in enumerate(pieces[site * per:(site + 1) * per]):
                tie = after(anchor[:, (k * 128) % anchor.shape[1]:])
                n_r, n_c = e.shape[1] // 8 - 1, e.shape[2] // 128
                pos = jnp.maximum(i - first_prep, 0) * per_it + u
                live = (i >= first_prep) & (pos < n_r * n_c)
                rows = pl.ds(pl.multiple_of(jnp.where(live, lax.rem(pos, n_r), n_r) * 8, 8), 8)
                cols = pl.ds(pl.multiple_of(jnp.where(live, lax.div(pos, n_r), 0) * 128, 128), 128)
                blocks = [_unpack(e[slot, rows, cols] | tie) for _, _, slot in _strassen_blocks(lv)]
                for slot, w in enumerate(_strassen_rhs(blocks)):
                    if slot in grp and not any(w is blk for blk in blocks):
                        e[slot, rows, cols] = _pack(w)

        cp_x.wait()
        cp_x2.start()
        for cp in cp_f:
            cp.start()
        hs_v[...] = pltpu.bitcast(
            jnp.concatenate([mem0_ref[...].astype(F32), ada1(x_v[0])], axis=0).astype(BF16), U32)
        scale = Dh ** -0.5
        n_g = H // G

        def step(s, side):
            KP = 2 * L
            ri = lax.broadcasted_iota(jnp.int32, (2 * L, KP), 0)
            ci = lax.broadcasted_iota(jnp.int32, (2 * L, KP), 1)
            same = ((ri >= L) == (ci >= L)) & (ci < 2 * L)
            rl = jnp.where(ri >= L, ri - L, ri)
            cl = jnp.where(ci >= L, ci - L, ci)
            keep = same & ((rl < M) | (rl >= cl))
            fill = jnp.where(same, -1e9 / scale, -jnp.inf).astype(F32)
            early = pl.ds(pl.multiple_of(s * P, P), P)

            def stack(a, p, rows=2 * L):
                parts = [a[:, (2 * p) * Dh:(2 * p + 1) * Dh], a[:, (2 * p + 1) * Dh:(2 * p + 2) * Dh]]
                if rows > 2 * L:
                    parts.append(jnp.zeros((rows - 2 * L, Dh), a.dtype))
                return jnp.concatenate(parts, axis=0)

            def gcols(g):
                return slice(g * G * Dh, (g + 1) * G * Dh)

            def proj(t, g):
                return jnp.concatenate([_dot(pltpu.bitcast(hs_v[...], BF16), pltpu.bitcast(wqkv[t, :, gcols(g)], BF16)),
                                        pre_v[t, early, gcols(g)]], axis=0)

            def scores(q, k):
                res = []
                for p in range(G // 2):
                    sc = jnp.where(keep, _dot(stack(q, p), stack(k, p, KP).astype(BF16), _NT), fill)
                    e = jnp.exp2((sc - jnp.max(sc, axis=-1, keepdims=True)) * (scale * _LOG2E))
                    den = jnp.sum(e, axis=-1, keepdims=True)
                    r = pl.reciprocal(den, approx=True)
                    res.append((e, r * (2.0 - den * r)))
                return res

            def values(g, res, v):
                for p, (e, inv) in enumerate(res):
                    o = _dot(e, stack(v, p, KP).astype(BF16)) * inv
                    h0 = g * G + 2 * p
                    o_v[:, h0 * Dh:(h0 + 1) * Dh] = o[0:L]
                    o_v[:, (h0 + 1) * Dh:(h0 + 2) * Dh] = o[L:2 * L]

            def outp(g):
                return _dot(o_v[:, gcols(g)],
                            pltpu.bitcast(wo32[g * G * Dh // 2:(g + 1) * G * Dh // 2, :], BF16))

            h_next = ada1(x_v[jnp.minimum(s + 1, n_seg - 1)])
            qk, sm, vv = {}, {}, {}
            for g in range(n_g):
                qk[g] = proj(0, g), proj(1, g)
                if g >= 1:
                    sm[g - 1] = scores(*qk.pop(g - 1))
                side(g, qk[g][1])
            for g in range(n_g):
                vv[g] = proj(2, g)
                side(n_g + g, vv[g])
                if g == 0:
                    sm[n_g - 1] = scores(*qk.pop(n_g - 1))
                else:
                    values(g - 1, sm.pop(g - 1), vv.pop(g - 1))
            acc = outp(0)
            values(n_g - 1, sm.pop(n_g - 1), vv.pop(n_g - 1))
            for g in range(1, n_g):
                side(2 * n_g - 1 + g, acc)
                acc = acc + outp(g)
            hs_v[...] = pltpu.bitcast(jnp.concatenate([acc[0:M], h_next], axis=0).astype(BF16), U32)
            x_v[s] = (x_v[s].astype(F32) + mod_v[0:1, 2 * D:3 * D] * acc[M:L]).astype(x_v.dtype)

        def steps(i, carry):
            @pl.when(i == (XA - 1) // UN)
            def _():
                cp_x2.wait()

            @pl.when(i == first_prep)
            def _():
                for cp in cp_f:
                    cp.wait()
            for j in range(UN):
                per = 3 * n_g - 1
                step(i * UN + j, lambda k, anchor, j=j: prep_ffn(i, j * per + k, UN * per, anchor))
            return carry

        lax.fori_loop(0, n_seg // UN, steps, 0)

        def resid(i):
            return x_v[pl.ds(i * (BM // T), BM // T)].astype(F32).reshape(BM, D)

        def ada2(i):
            h2 = _layernorm(resid(i)) * (1.0 + mod_v[0:1, 4 * D:5 * D]) + mod_v[0:1, 3 * D:4 * D]
            return _strassen_lhs(h2, LV[0])

        def matmul(lhs, e, cols=slice(None)):
            return _strassen_out([_dot(a, pltpu.bitcast(e[k, 0:e.shape[1] - 8, cols], BF16))
                                  for k, a in enumerate(lhs)])

        def put_h2(parts):
            for j, part in enumerate(parts):
                h2_v[j] = pltpu.bitcast(part, U32)

        put_h2(ada2(0))

        def out_copy(i):
            r = pl.ds(i * (BM // T), BM // T)
            return pltpu.make_async_copy(x_v.at[r], out_hbm.at[r], sem_y.at[i])

        def ffn(i, carry):
            lhs = [pltpu.bitcast(h2_v[j], BF16) for j in range(h2_v.shape[0])]
            h2_next = ada2(jnp.minimum(i + 1, S // BM - 1))
            n, parts = e1_v.shape[2], []
            for c0 in range(0, n, FC):
                cols = slice(c0, min(c0 + FC, n))
                a = _silu(matmul(lhs, e1_v, cols)) * matmul(lhs, e3_v, cols)
                parts.append(jnp.split(a, F // n, axis=1))
            act = jnp.concatenate([part[j] for j in range(F // n) for part in parts], axis=1)
            ffn_out = matmul(_strassen_lhs(act, LV[1]), e2_v)
            y = resid(i) + mod_v[0:1, 5 * D:6 * D] * ffn_out
            x_v[pl.ds(i * (BM // T), BM // T)] = y.reshape(BM // T, T, D).astype(x_v.dtype)
            put_h2(h2_next)
            out_copy(i).start()
            return carry

        lax.fori_loop(0, S // BM, ffn, 0)
        for i in range(S // BM):
            out_copy(i).wait()

    pl.run_scoped(main,
                  *[pltpu.VMEM((7 ** lv, (w.shape[0] >> (lv + 1)) + 8, w.shape[1] >> lv), U32)
                    for w, lv in ffn_cfg],
                  pltpu.VMEM((7 ** LV[0], BM >> (LV[0] + 1), D >> LV[0]), U32),
                  pltpu.SemaphoreType.DMA((sum(4 ** lv for _, lv in ffn_cfg),)),
                  pltpu.SemaphoreType.DMA((S // BM,)))


@functools.partial(jax.jit, static_argnames=("A_seg_len",))
def pallas_adaLN_cond__memory_aug_recurrent_mem_tr__glu_gated_swiglu__prompt_kernel(
    A_x, A_mem0, A_Wq, A_Wk, A_Wv, A_Wo, A_seg_len, B_x, B_w1, B_w3, B_w2, c, w_mod,
):
    del B_x
    B, S, D = A_x.shape
    _, H, Dh = A_Wq.shape
    M, T, F = A_mem0.shape[1], int(A_seg_len), B_w1.shape[1]
    assert B == 1 and S % T == 0
    L, HD = M + T, H * Dh
    hbm = pl.BlockSpec(memory_space=pl.ANY)
    vmem = pl.BlockSpec(memory_space=pltpu.VMEM)
    body = functools.partial(_body, S=S, D=D, H=H, Dh=Dh, M=M, T=T, F=F, G=8, BM=128, FC=128, LV=(2, 1))
    out = pl.pallas_call(
        body,
        out_shape=jax.ShapeDtypeStruct((S // T, T, D), A_x.dtype),
        in_specs=[hbm, vmem, hbm, hbm, hbm, hbm, hbm, hbm, hbm, vmem, hbm],
        out_specs=hbm,
        scratch_shapes=[
            pltpu.VMEM((3, D // 2, HD), U32), pltpu.VMEM((HD // 2, D), U32),
            pltpu.VMEM((3, S // T * 8, HD), F32),
            pltpu.VMEM((S // T, T, D), A_x.dtype), pltpu.VMEM((8, 6 * D), F32),
            pltpu.VMEM((D // 256, 8, 512), F32),
            pltpu.VMEM(((L - 8) // 2, D), U32), pltpu.VMEM((L, HD), F32), pltpu.VMEM((8, 128), U32),
            pltpu.SemaphoreType.DMA((2,)),
        ],
        compiler_params=pltpu.CompilerParams(vmem_limit_bytes=126 * 2**20, flags={'XLA_TPU_EVENLY_DISTRIBUTE_CRITICAL_NODES': True}),
    )(A_x.reshape(S // T, T, D), A_mem0.reshape(M, D),
      A_Wq.reshape(D // 2, 2 * H, Dh), A_Wk.reshape(D // 2, 2 * H, Dh), A_Wv.reshape(D // 2, 2 * H, Dh), A_Wo.reshape(HD, D),
      B_w1, B_w3, B_w2, c, w_mod)
    return out.reshape(B, S, D)
```

```python
import functools

import jax
import jax.numpy as jnp
from jax import lax
import jax.experimental.pallas as pl
import jax.experimental.pallas.tpu as pltpu

F32, BF16, U32 = jnp.float32, jnp.bfloat16, jnp.uint32
_LOG2E = 1.4426950408889634
_NN = (((1,), (0,)), ((), ()))
_NT = (((1,), (1,)), ((), ()))


def _dot(a, b, dims=_NN):
    return lax.dot_general(a, b, dims, preferred_element_type=F32)


def _layernorm(x, eps=1e-5):
    m = jnp.mean(x, axis=-1, keepdims=True)
    d = x - m
    v = jnp.mean(d * d, axis=-1, keepdims=True)
    return d * lax.rsqrt(v + eps)


def _silu(x):
    h = 0.5 * x
    return h + h * jnp.tanh(h)


def _unpack(w):
    return jnp.stack([pltpu.unpack_elementwise(w, index=i, packed_dtype=BF16, unpacked_dtype=F32)
                      for i in range(2)])


def _pack(x):
    return pltpu.bitcast(pltpu.pack_elementwise([x[0], x[1]], packed_dtype=BF16), U32)


def _strassen_lhs(a, levels):
    if levels == 0:
        return [a.astype(BF16)]
    m, k = a.shape[0] // 2, a.shape[1] // 2
    a11, a12, a21, a22 = a[:m, :k], a[:m, k:], a[m:, :k], a[m:, k:]
    return [x for v in (a11 + a22, a21 + a22, a11, a22, a11 + a12, a21 - a11, a12 - a22)
            for x in _strassen_lhs(v, levels - 1)]


def _strassen_rhs(blocks):
    if len(blocks) == 1:
        return blocks
    n = len(blocks) // 4
    b11, b12, b21, b22 = (blocks[i * n:(i + 1) * n] for i in range(4))
    add = lambda x, y: [u + v for u, v in zip(x, y)]
    sub = lambda x, y: [u - v for u, v in zip(x, y)]
    return [x for v in (add(b11, b22), b11, sub(b12, b22), sub(b21, b11), b22, add(b11, b12), add(b21, b22))
            for x in _strassen_rhs(v)]


def _strassen_blocks(levels):
    out = [(0, 0, 0)]
    for _ in range(levels):
        out = [(2 * i + q // 2, 2 * j + q % 2, 7 * slot + 1 + q) for i, j, slot in out for q in range(4)]
    return out


def _strassen_out(m):
    if len(m) == 1:
        return m[0]
    n = len(m) // 7
    m1, m2, m3, m4, m5, m6, m7 = (_strassen_out(m[i * n:(i + 1) * n]) for i in range(7))
    return jnp.concatenate([jnp.concatenate([m1 + m4 - m5 + m7, m3 + m5], axis=1),
                            jnp.concatenate([m2 + m4, m1 - m2 + m3 + m6], axis=1)], axis=0)


def _body(x_hbm, mem0_ref, wq_hbm, wk_hbm, wv_hbm, wo_hbm, w1_hbm, w3_hbm, w2_hbm,
          c_ref, wm_hbm, out_hbm,
          wqkv, wo32, pre_v, x_v, mod_v, mod1_v, hs_v, o_v, zero_v, sems,
          *, S, D, H, Dh, M, T, F, G, BM, FC, LV):
    n_seg = S // T
    L = M + T
    HD = H * Dh
    UN = 2
    P = 8
    KC = 256
    n_kc = D // KC
    wo_src = wo_hbm.bitcast(U32)
    wm_src = wm_hbm.bitcast(U32)
    HP = H + 8
    XA = 9
    cp_x = pltpu.make_async_copy(x_hbm.at[pl.ds(0, XA)], x_v.at[pl.ds(0, XA)], sems.at[0])
    cp_x2 = pltpu.make_async_copy(x_hbm.at[pl.ds(XA, n_seg - XA)], x_v.at[pl.ds(XA, n_seg - XA)], sems.at[1])

    zero_v[...] = jnp.zeros(zero_v.shape, U32)

    def after(anchor):
        return pltpu.bitcast(anchor[0:8, 0:128], U32) & zero_v[...]

    def silu_c():
        return jnp.broadcast_to(_silu(c_ref[...].astype(F32)), (8, D)).astype(BF16)

    def ada1(x):
        return _layernorm(x.astype(F32)[:T - P]) * (1.0 + mod_v[0:1, D:2 * D]) + mod_v[0:1, 0:D]

    def startup(wm_v, wr_v, raw, xp_v, xn_v, hp_v, acc_v, sem_m, sem_w, sem_p):
        srcs = [w.bitcast(U32) for w in (wq_hbm, wk_hbm, wv_hbm)]
        n_j = 3 * n_kc
        R = n_seg * P

        def cp_w(j, t=0):
            return pltpu.make_async_copy(srcs[t].at[pl.ds((j % n_kc) * (KC // 2), KC // 2)],
                                         raw.at[pl.ds(j * (KC // 2), KC // 2), pl.ds(0, H)], sem_w.at[j])

        def cp_m(c, i):
            return pltpu.make_async_copy(wm_src.at[:, pl.ds(pl.multiple_of(i * D + c * KC, KC), KC)],
                                         wm_v.at[c, :, pl.ds(i * KC, KC)], sem_m.at[2 * c + i])

        def start(j):
            cp_m(j, 0).start()
            cp_m(j, 1).start()
            cp_w(j).start()

        def cp_o(i):
            r = pl.ds(pl.multiple_of(i * (HD // 16), HD // 16), HD // 16)
            return pltpu.make_async_copy(wo_src.at[r], wo32.at[r], sem_p.at[1 + i])

        def cp_r(i):
            r = pl.ds(pl.multiple_of(i * (D // 16), D // 16), D // 16)
            return pltpu.make_async_copy(wm_src.at[r, pl.ds(2 * D, 4 * D)], wr_v.at[r], sem_p.at[9 + i])

        cp_p = pltpu.make_async_copy(x_hbm.at[:, pl.ds(T - P, P), :], xp_v, sem_p.at[0])
        cp_p.start()
        start(0)

        cp_p.wait()

        def norm(i, carry):
            xn = _layernorm(xp_v[pl.ds(i * 8, 8)].astype(F32).reshape(8 * P, D))
            for c in range(n_kc):
                xn_v[c, pl.ds(pl.multiple_of(i * 8 * P, 8 * P), 8 * P), :] = xn[:, c * KC:(c + 1) * KC]
            return carry
        lax.fori_loop(0, n_seg // 8, norm, 0)
        start(1)
        raw2 = raw.reshape(3 * D // 2 * HP, Dh)

        def chunk(j, carry):
            t, c = j // n_kc, j % n_kc

            @pl.when(j < n_kc)
            def _():
                cp_m(c, 0).wait()
                cp_m(c, 1).wait()

                @pl.when(j + 2 < n_kc)
                def _():
                    start(j + 2)
                mod = _dot(silu_c(), pltpu.bitcast(wm_v[c], BF16))
                mod1_v[c] = mod
                h = xn_v[c] * (1.0 + mod[0:1, KC:]) + mod[0:1, :KC]
                for i, part in enumerate(_strassen_lhs(h, 1)):
                    hp_v[c, i] = pltpu.bitcast(part, U32)

            cp_w(j).wait()
            for src in (1, 2):
                @pl.when((j + 2) // n_kc == src)
                def _(src=src):
                    cp_w(j + 2, src).start()

            @pl.when(j >= n_j - 8)
            def _():
                cp_r(j - (n_j - 8)).start()
                cp_o(j - (n_j - 8)).start()

            @pl.when(j == n_j - 2)
            def _():
                cp_x.start()

            q4 = KC // 4
            for hp in range(H // 2):
                blk = []
                for half in range(2):
                    base = (j * 2 + half) * (q4 * HP) + hp
                    a = _unpack(raw2[pl.ds(base, q4, stride=HP), :])
                    b = _unpack(raw2[pl.ds(base + H // 2, q4, stride=HP), :])
                    blk += [jnp.stack([a[0], b[0]]), jnp.stack([a[1], b[1]])]
                tiles = [_pack(v) for v in blk]
                cols = [slice((2 * hp + i) * Dh, (2 * hp + i + 1) * Dh) for i in range(2)]
                for i, tile in enumerate(tiles):
                    wqkv[t, pl.ds(pl.multiple_of((2 * c + i // 2) * q4, q4), q4), cols[i % 2]] = tile
                part = _strassen_out([_dot(pltpu.bitcast(hp_v[c, i], BF16), pltpu.bitcast(_pack(w), BF16))
                                      for i, w in enumerate(_strassen_rhs(blk))])
                pair = slice(2 * hp * Dh, (2 * hp + 2) * Dh)
                part = jnp.where(c > 0, acc_v[:, pair], 0.0) + part
                acc_v[:, pair] = part
                pre_v[t, :, hp * Dh:(hp + 1) * Dh] = _pack((part[:, :Dh], part[:, Dh:]))
            return carry

        lax.fori_loop(0, n_j, chunk, 0)
        for c in range(n_kc):
            mod_v[:, c * KC:(c + 1) * KC] = mod1_v[c, :, :KC]
            mod_v[:, D + c * KC:D + (c + 1) * KC] = mod1_v[c, :, KC:]
        for i in range(8):
            cp_r(i).wait()
        mod_v[:, 2 * D:6 * D] = _dot(silu_c(), pltpu.bitcast(wr_v[...], BF16))
        for i in range(8):
            cp_o(i).wait()

    pl.run_scoped(startup,
                  pltpu.VMEM((n_kc, D // 2, 2 * KC), U32), pltpu.VMEM((D // 2, 4 * D), U32),
                  pltpu.VMEM((3 * D // 2, HP, Dh), U32),
                  pltpu.VMEM((n_seg, P, D), x_hbm.dtype), pltpu.VMEM((n_kc, n_seg * P, KC), F32),
                  pltpu.VMEM((n_kc, 7, n_seg * P // 4, KC // 2), U32), pltpu.VMEM((n_seg * P, HD), F32),
                  pltpu.SemaphoreType.DMA((2 * n_kc,)), pltpu.SemaphoreType.DMA((3 * n_kc,)),
                  pltpu.SemaphoreType.DMA((17,)))

    n_it = n_seg // UN
    first_prep = n_it // 8
    ffn_cfg = ((w1_hbm, LV[0]), (w3_hbm, LV[0]), (w2_hbm, LV[1]))

    def main(e1_v, e3_v, e2_v, h2_v, sem_f, sem_y):
        cp_f, pieces = [], []
        for (src, lv), e in zip(ffn_cfg, (e1_v, e3_v, e2_v)):
            R, n = e.shape[1] - 8, e.shape[2]
            for bi, bj, slot in _strassen_blocks(lv):
                cp_f.append(pltpu.make_async_copy(src.bitcast(U32).at[pl.ds(bi * R, R), pl.ds(bj * n, n)],
                                                  e.at[slot, pl.ds(0, R)], sem_f.at[len(cp_f)]))
                e[slot, R:R + 8, 0:128] = jnp.zeros((8, 128), U32)
            per_it = pl.cdiv(R // 8 * (n // 128), n_it - first_prep)
            groups = [range(7)] if lv == 1 else [range(7 * o, 7 * o + 7) for o in (0, 5, 6, 2, 3, 1, 4)]
            pieces += [(e, lv, per_it, u, grp) for u in range(per_it) for grp in groups]

        def prep_ffn(i, site, n_sites, anchor):
            per = pl.cdiv(len(pieces), n_sites)
            for k, (e, lv, per_it, u, grp) in enumerate(pieces[site * per:(site + 1) * per]):
                tie = after(anchor[:, (k * 128) % anchor.shape[1]:])
                n_r, n_c = e.shape[1] // 8 - 1, e.shape[2] // 128
                pos = jnp.maximum(i - first_prep, 0) * per_it + u
                live = (i >= first_prep) & (pos < n_r * n_c)
                rows = pl.ds(pl.multiple_of(jnp.where(live, lax.rem(pos, n_r), n_r) * 8, 8), 8)
                cols = pl.ds(pl.multiple_of(jnp.where(live, lax.div(pos, n_r), 0) * 128, 128), 128)
                blocks = [_unpack(e[slot, rows, cols] | tie) for _, _, slot in _strassen_blocks(lv)]
                for slot, w in enumerate(_strassen_rhs(blocks)):
                    if slot in grp and not any(w is blk for blk in blocks):
                        e[slot, rows, cols] = _pack(w)

        cp_x.wait()
        cp_x2.start()
        for cp in cp_f:
            cp.start()
        hs_v[...] = pltpu.bitcast(
            jnp.concatenate([mem0_ref[...].astype(F32), ada1(x_v[0])], axis=0).astype(BF16), U32)
        scale = Dh ** -0.5
        n_g = H // G

        def step(s, side):
            ri = lax.broadcasted_iota(jnp.int32, (2 * L, 2 * L), 0)
            ci = lax.broadcasted_iota(jnp.int32, (2 * L, 2 * L), 1)
            same = (ri >= L) == (ci >= L)
            rl = jnp.where(ri >= L, ri - L, ri)
            cl = jnp.where(ci >= L, ci - L, ci)
            keep = same & ((rl < M) | (rl >= cl))
            fill = jnp.where(same, -1e9 / scale, -jnp.inf).astype(F32)
            early = pl.ds(pl.multiple_of(s * P, P), P)

            def gcols(g):
                return slice(g * G * Dh, (g + 1) * G * Dh)

            def proj(t, g):
                return _dot(pltpu.bitcast(hs_v[...], BF16), pltpu.bitcast(wqkv[t, :, gcols(g)], BF16))

            def stack(a, t, g, p):
                hp = g * G // 2 + p
                pre = _unpack(pre_v[t, early, hp * Dh:(hp + 1) * Dh])
                return jnp.concatenate([a[:, (2 * p) * Dh:(2 * p + 1) * Dh], pre[0],
                                        a[:, (2 * p + 1) * Dh:(2 * p + 2) * Dh], pre[1]], axis=0).astype(BF16)

            def scores(g, q, k):
                res = []
                for p in range(G // 2):
                    sc = jnp.where(keep, _dot(stack(q, 0, g, p), stack(k, 1, g, p), _NT), fill)
                    e = jnp.exp2((sc - jnp.max(sc, axis=-1, keepdims=True)) * (scale * _LOG2E))
                    den = jnp.sum(e, axis=-1, keepdims=True)
                    r = pl.reciprocal(den, approx=True)
                    res.append((e.astype(BF16), r * (2.0 - den * r)))
                return res

            def values(g, res, v):
                for p, (e, inv) in enumerate(res):
                    o = _dot(e, stack(v, 2, g, p)) * inv
                    h0 = g * G + 2 * p
                    o_v[:, h0 * Dh:(h0 + 1) * Dh] = o[0:L]
                    o_v[:, (h0 + 1) * Dh:(h0 + 2) * Dh] = o[L:2 * L]

            def outp(g):
                return _dot(o_v[:, gcols(g)],
                            pltpu.bitcast(wo32[g * G * Dh // 2:(g + 1) * G * Dh // 2, :], BF16))

            h_next = ada1(x_v[jnp.minimum(s + 1, n_seg - 1)])
            qk, sm, vv = {}, {}, {}
            for g in range(n_g):
                qk[g] = proj(0, g), proj(1, g)
                if g >= 1:
                    sm[g - 1] = scores(g - 1, *qk.pop(g - 1))
                side(g, qk[g][1])
            for g in range(n_g):
                vv[g] = proj(2, g)
                side(n_g + g, vv[g])
                if g == 0:
                    sm[n_g - 1] = scores(n_g - 1, *qk.pop(n_g - 1))
                else:
                    values(g - 1, sm.pop(g - 1), vv.pop(g - 1))
            acc = outp(0)
            values(n_g - 1, sm.pop(n_g - 1), vv.pop(n_g - 1))
            for g in range(1, n_g):
                side(2 * n_g - 1 + g, acc)
                acc = acc + outp(g)
            hs_v[...] = pltpu.bitcast(jnp.concatenate([acc[0:M], h_next], axis=0).astype(BF16), U32)
            x_v[s] = (x_v[s].astype(F32) + mod_v[0:1, 2 * D:3 * D] * acc[M:L]).astype(x_v.dtype)

        def steps(i, carry):
            @pl.when(i == (XA - 1) // UN)
            def _():
                cp_x2.wait()

            @pl.when(i == first_prep)
            def _():
                for cp in cp_f:
                    cp.wait()
            for j in range(UN):
                per = 3 * n_g - 1
                step(i * UN + j, lambda k, anchor, j=j: prep_ffn(i, j * per + k, UN * per, anchor))
            return carry

        lax.fori_loop(0, n_seg // UN, steps, 0)

        def resid(i):
            return x_v[pl.ds(i * (BM // T), BM // T)].astype(F32).reshape(BM, D)

        def ada2(i):
            h2 = _layernorm(resid(i)) * (1.0 + mod_v[0:1, 4 * D:5 * D]) + mod_v[0:1, 3 * D:4 * D]
            return _strassen_lhs(h2, LV[0])

        def matmul(lhs, e, cols=slice(None)):
            return _strassen_out([_dot(a, pltpu.bitcast(e[k, 0:e.shape[1] - 8, cols], BF16))
                                  for k, a in enumerate(lhs)])

        def put_h2(parts):
            for j, part in enumerate(parts):
                h2_v[j] = pltpu.bitcast(part, U32)

        put_h2(ada2(0))

        def out_copy(i):
            r = pl.ds(i * (BM // T), BM // T)
            return pltpu.make_async_copy(x_v.at[r], out_hbm.at[r], sem_y.at[i])

        def ffn(i, carry):
            lhs = [pltpu.bitcast(h2_v[j], BF16) for j in range(h2_v.shape[0])]
            h2_next = ada2(jnp.minimum(i + 1, S // BM - 1))
            n, parts = e1_v.shape[2], []
            for c0 in range(0, n, FC):
                cols = slice(c0, min(c0 + FC, n))
                a = _silu(matmul(lhs, e1_v, cols)) * matmul(lhs, e3_v, cols)
                parts.append(jnp.split(a, F // n, axis=1))
            act = jnp.concatenate([part[j] for j in range(F // n) for part in parts], axis=1)
            ffn_out = matmul(_strassen_lhs(act, LV[1]), e2_v)
            y = resid(i) + mod_v[0:1, 5 * D:6 * D] * ffn_out
            x_v[pl.ds(i * (BM // T), BM // T)] = y.reshape(BM // T, T, D).astype(x_v.dtype)
            put_h2(h2_next)
            out_copy(i).start()
            return carry

        lax.fori_loop(0, S // BM, ffn, 0)
        for i in range(S // BM):
            out_copy(i).wait()

    pl.run_scoped(main,
                  *[pltpu.VMEM((7 ** lv, (w.shape[0] >> (lv + 1)) + 8, w.shape[1] >> lv), U32)
                    for w, lv in ffn_cfg],
                  pltpu.VMEM((7 ** LV[0], BM >> (LV[0] + 1), D >> LV[0]), U32),
                  pltpu.SemaphoreType.DMA((sum(4 ** lv for _, lv in ffn_cfg),)),
                  pltpu.SemaphoreType.DMA((S // BM,)))


@functools.partial(jax.jit, static_argnames=("A_seg_len",))
def pallas_adaLN_cond__memory_aug_recurrent_mem_tr__glu_gated_swiglu__prompt_kernel(
    A_x, A_mem0, A_Wq, A_Wk, A_Wv, A_Wo, A_seg_len, B_x, B_w1, B_w3, B_w2, c, w_mod,
):
    del B_x
    B, S, D = A_x.shape
    _, H, Dh = A_Wq.shape
    M, T, F = A_mem0.shape[1], int(A_seg_len), B_w1.shape[1]
    assert B == 1 and S % T == 0
    L, HD = M + T, H * Dh
    hbm = pl.BlockSpec(memory_space=pl.ANY)
    vmem = pl.BlockSpec(memory_space=pltpu.VMEM)
    body = functools.partial(_body, S=S, D=D, H=H, Dh=Dh, M=M, T=T, F=F, G=8, BM=128, FC=128, LV=(2, 2))
    out = pl.pallas_call(
        body,
        out_shape=jax.ShapeDtypeStruct((S // T, T, D), A_x.dtype),
        in_specs=[hbm, vmem, hbm, hbm, hbm, hbm, hbm, hbm, hbm, vmem, hbm],
        out_specs=hbm,
        scratch_shapes=[
            pltpu.VMEM((3, D // 2, HD), U32), pltpu.VMEM((HD // 2, D), U32),
            pltpu.VMEM((3, S // T * 8, HD // 2), U32),
            pltpu.VMEM((S // T, T, D), A_x.dtype), pltpu.VMEM((8, 6 * D), F32),
            pltpu.VMEM((D // 256, 8, 512), F32),
            pltpu.VMEM(((L - 8) // 2, D), U32), pltpu.VMEM((L, HD), F32), pltpu.VMEM((8, 128), U32),
            pltpu.SemaphoreType.DMA((2,)),
        ],
        compiler_params=pltpu.CompilerParams(vmem_limit_bytes=126 * 2**20, flags={'XLA_TPU_EVENLY_DISTRIBUTE_CRITICAL_NODES': True}),
    )(A_x.reshape(S // T, T, D), A_mem0.reshape(M, D),
      A_Wq.reshape(D // 2, 2 * H, Dh), A_Wk.reshape(D // 2, 2 * H, Dh), A_Wv.reshape(D // 2, 2 * H, Dh), A_Wo.reshape(HD, D),
      B_w1, B_w3, B_w2, c, w_mod)
    return out.reshape(B, S, D)
```

```python
import functools

import jax
import jax.numpy as jnp
from jax import lax
import jax.experimental.pallas as pl
import jax.experimental.pallas.tpu as pltpu

F32, BF16, U32 = jnp.float32, jnp.bfloat16, jnp.uint32
_LOG2E = 1.4426950408889634
_NN = (((1,), (0,)), ((), ()))
_NT = (((1,), (1,)), ((), ()))


def _dot(a, b, dims=_NN):
    return lax.dot_general(a, b, dims, preferred_element_type=F32)


def _layernorm(x, eps=1e-5):
    m = jnp.mean(x, axis=-1, keepdims=True)
    d = x - m
    v = jnp.mean(d * d, axis=-1, keepdims=True)
    return d * lax.rsqrt(v + eps)


def _silu(x):
    h = 0.5 * x
    return h + h * jnp.tanh(h)


def _unpack(w):
    return jnp.stack([pltpu.unpack_elementwise(w, index=i, packed_dtype=BF16, unpacked_dtype=F32)
                      for i in range(2)])


def _pack(x):
    return pltpu.bitcast(pltpu.pack_elementwise([x[0], x[1]], packed_dtype=BF16), U32)


def _strassen_lhs(a, levels):
    if levels == 0:
        return [a.astype(BF16)]
    m, k = a.shape[0] // 2, a.shape[1] // 2
    a11, a12, a21, a22 = a[:m, :k], a[:m, k:], a[m:, :k], a[m:, k:]
    return [x for v in (a11 + a22, a21 + a22, a11, a22, a11 + a12, a21 - a11, a12 - a22)
            for x in _strassen_lhs(v, levels - 1)]


def _strassen_rhs(blocks):
    if len(blocks) == 1:
        return blocks
    n = len(blocks) // 4
    b11, b12, b21, b22 = (blocks[i * n:(i + 1) * n] for i in range(4))
    add = lambda x, y: [u + v for u, v in zip(x, y)]
    sub = lambda x, y: [u - v for u, v in zip(x, y)]
    return [x for v in (add(b11, b22), b11, sub(b12, b22), sub(b21, b11), b22, add(b11, b12), add(b21, b22))
            for x in _strassen_rhs(v)]


def _strassen_blocks(levels):
    out = [(0, 0, 0)]
    for _ in range(levels):
        out = [(2 * i + q // 2, 2 * j + q % 2, 7 * slot + 1 + q) for i, j, slot in out for q in range(4)]
    return out


def _strassen_out(m):
    if len(m) == 1:
        return m[0]
    n = len(m) // 7
    m1, m2, m3, m4, m5, m6, m7 = (_strassen_out(m[i * n:(i + 1) * n]) for i in range(7))
    return jnp.concatenate([jnp.concatenate([m1 + m4 - m5 + m7, m3 + m5], axis=1),
                            jnp.concatenate([m2 + m4, m1 - m2 + m3 + m6], axis=1)], axis=0)


def _body(x_hbm, mem0_ref, wq_hbm, wk_hbm, wv_hbm, wo_hbm, w1_hbm, w3_hbm, w2_hbm,
          c_ref, wm_hbm, out_hbm,
          wqkv, wo32, pre_v, x_v, mod_v, mod1_v, hs_v, o_v, zero_v, sems,
          *, S, D, H, Dh, M, T, F, G, BM, FC, LV):
    n_seg = S // T
    L = M + T
    HD = H * Dh
    UN = 2
    P = 8
    KC = 256
    n_kc = D // KC
    wo_src = wo_hbm.bitcast(U32)
    wm_src = wm_hbm.bitcast(U32)
    HP = H + 8
    n_it = n_seg // UN
    first_prep = n_it // 8
    XA = first_prep * UN + 1
    cp_x = pltpu.make_async_copy(x_hbm.at[pl.ds(0, XA)], x_v.at[pl.ds(0, XA)], sems.at[0])
    cp_x2 = pltpu.make_async_copy(x_hbm.at[pl.ds(XA, n_seg - XA)], x_v.at[pl.ds(XA, n_seg - XA)], sems.at[1])

    zero_v[...] = jnp.zeros(zero_v.shape, U32)

    def after(anchor):
        return pltpu.bitcast(anchor[0:8, 0:128], U32) & zero_v[...]

    def silu_c():
        return jnp.broadcast_to(_silu(c_ref[...].astype(F32)), (8, D)).astype(BF16)

    def ada1(x):
        return _layernorm(x.astype(F32)[:T - P]) * (1.0 + mod_v[0:1, D:2 * D]) + mod_v[0:1, 0:D]

    def startup(wm_v, wr_v, raw, xp_v, xn_v, hp_v, acc_v, sem_m, sem_w, sem_p):
        srcs = [w.bitcast(U32) for w in (wq_hbm, wk_hbm, wv_hbm)]
        n_j = 3 * n_kc
        R = n_seg * P

        def cp_w(j, t=0):
            return pltpu.make_async_copy(srcs[t].at[pl.ds((j % n_kc) * (KC // 2), KC // 2)],
                                         raw.at[pl.ds(j * (KC // 2), KC // 2), pl.ds(0, H)], sem_w.at[j])

        def cp_m(c, i):
            return pltpu.make_async_copy(wm_src.at[:, pl.ds(pl.multiple_of(i * D + c * KC, KC), KC)],
                                         wm_v.at[c, :, pl.ds(i * KC, KC)], sem_m.at[2 * c + i])

        def start(j):
            cp_m(j, 0).start()
            cp_m(j, 1).start()
            cp_w(j).start()

        def cp_o(i):
            r = pl.ds(pl.multiple_of(i * (HD // 16), HD // 16), HD // 16)
            return pltpu.make_async_copy(wo_src.at[r], wo32.at[r], sem_p.at[1 + i])

        def cp_r(i):
            r = pl.ds(pl.multiple_of(i * (D // 16), D // 16), D // 16)
            return pltpu.make_async_copy(wm_src.at[r, pl.ds(2 * D, 4 * D)], wr_v.at[r], sem_p.at[9 + i])

        cp_p = pltpu.make_async_copy(x_hbm.at[:, pl.ds(T - P, P), :], xp_v, sem_p.at[0])
        cp_p.start()
        start(0)

        cp_p.wait()

        def norm(i, carry):
            xn = _layernorm(xp_v[pl.ds(i * 8, 8)].astype(F32).reshape(8 * P, D))
            for c in range(n_kc):
                xn_v[c, pl.ds(pl.multiple_of(i * 8 * P, 8 * P), 8 * P), :] = xn[:, c * KC:(c + 1) * KC]
            return carry
        lax.fori_loop(0, n_seg // 8, norm, 0)
        start(1)
        raw2 = raw.reshape(3 * D // 2 * HP, Dh)

        def chunk(j, carry):
            t, c = j // n_kc, j % n_kc

            @pl.when(j < n_kc)
            def _():
                cp_m(c, 0).wait()
                cp_m(c, 1).wait()

                @pl.when(j + 2 < n_kc)
                def _():
                    start(j + 2)
                mod = _dot(silu_c(), pltpu.bitcast(wm_v[c], BF16))
                mod1_v[c] = mod
                h = xn_v[c] * (1.0 + mod[0:1, KC:]) + mod[0:1, :KC]
                for i, part in enumerate(_strassen_lhs(h, 1)):
                    hp_v[c, i] = pltpu.bitcast(part, U32)

            cp_w(j).wait()
            for src in (1, 2):
                @pl.when((j + 2) // n_kc == src)
                def _(src=src):
                    cp_w(j + 2, src).start()

            @pl.when(j >= n_j - 8)
            def _():
                cp_r(j - (n_j - 8)).start()
                cp_o(j - (n_j - 8)).start()

            @pl.when(j == n_j - 2)
            def _():
                cp_x.start()

            q4 = KC // 4
            for hp in range(H // 2):
                blk = []
                for half in range(2):
                    base = (j * 2 + half) * (q4 * HP) + hp
                    a = _unpack(raw2[pl.ds(base, q4, stride=HP), :])
                    b = _unpack(raw2[pl.ds(base + H // 2, q4, stride=HP), :])
                    blk += [jnp.stack([a[0], b[0]]), jnp.stack([a[1], b[1]])]
                tiles = [_pack(v) for v in blk]
                cols = [slice((2 * hp + i) * Dh, (2 * hp + i + 1) * Dh) for i in range(2)]
                for i, tile in enumerate(tiles):
                    wqkv[t, pl.ds(pl.multiple_of((2 * c + i // 2) * q4, q4), q4), cols[i % 2]] = tile
                part = _strassen_out([_dot(pltpu.bitcast(hp_v[c, i], BF16), pltpu.bitcast(_pack(w), BF16))
                                      for i, w in enumerate(_strassen_rhs(blk))])
                pair = slice(2 * hp * Dh, (2 * hp + 2) * Dh)
                part = jnp.where(c > 0, acc_v[:, pair], 0.0) + part
                acc_v[:, pair] = part
                pre_v[t, :, hp * Dh:(hp + 1) * Dh] = _pack((part[:, :Dh], part[:, Dh:]))
            return carry

        lax.fori_loop(0, n_j, chunk, 0)
        for c in range(n_kc):
            mod_v[:, c * KC:(c + 1) * KC] = mod1_v[c, :, :KC]
            mod_v[:, D + c * KC:D + (c + 1) * KC] = mod1_v[c, :, KC:]
        for i in range(8):
            cp_r(i).wait()
        mod_v[:, 2 * D:6 * D] = _dot(silu_c(), pltpu.bitcast(wr_v[...], BF16))
        for i in range(8):
            cp_o(i).wait()

    pl.run_scoped(startup,
                  pltpu.VMEM((n_kc, D // 2, 2 * KC), U32), pltpu.VMEM((D // 2, 4 * D), U32),
                  pltpu.VMEM((3 * D // 2, HP, Dh), U32),
                  pltpu.VMEM((n_seg, P, D), x_hbm.dtype), pltpu.VMEM((n_kc, n_seg * P, KC), F32),
                  pltpu.VMEM((n_kc, 7, n_seg * P // 4, KC // 2), U32), pltpu.VMEM((n_seg * P, HD), F32),
                  pltpu.SemaphoreType.DMA((2 * n_kc,)), pltpu.SemaphoreType.DMA((3 * n_kc,)),
                  pltpu.SemaphoreType.DMA((17,)))

    ffn_cfg = ((w1_hbm, LV), (w3_hbm, LV), (w2_hbm, LV))

    def main(e1_v, e3_v, e2_v, h2_v, act_v, sem_f, sem_y):
        cp_f, pieces = [], []
        for (src, lv), e in zip(ffn_cfg, (e1_v, e3_v, e2_v)):
            R, n = e.shape[1] - 8, e.shape[2]
            for bi, bj, slot in _strassen_blocks(lv):
                cp_f.append(pltpu.make_async_copy(src.bitcast(U32).at[pl.ds(bi * R, R), pl.ds(bj * n, n)],
                                                  e.at[slot, pl.ds(0, R)], sem_f.at[len(cp_f)]))
                e[slot, R:R + 8, 0:128] = jnp.zeros((8, 128), U32)
            per_it = pl.cdiv(R // 8 * (n // 128), n_it - first_prep)
            groups = [range(7)] if lv == 1 else [range(7 * o, 7 * o + 7) for o in (0, 5, 6, 2, 3, 1, 4)]
            pieces += [(e, lv, per_it, u, grp) for u in range(per_it) for grp in groups]

        def prep_ffn(i, site, n_sites, anchor):
            per = pl.cdiv(len(pieces), n_sites)
            for k, (e, lv, per_it, u, grp) in enumerate(pieces[site * per:(site + 1) * per]):
                tie = after(anchor[:, (k * 128) % anchor.shape[1]:])
                n_r, n_c = e.shape[1] // 8 - 1, e.shape[2] // 128
                pos = jnp.maximum(i - first_prep, 0) * per_it + u
                live = (i >= first_prep) & (pos < n_r * n_c)
                rows = pl.ds(pl.multiple_of(jnp.where(live, lax.rem(pos, n_r), n_r) * 8, 8), 8)
                cols = pl.ds(pl.multiple_of(jnp.where(live, lax.div(pos, n_r), 0) * 128, 128), 128)
                blocks = [_unpack(e[slot, rows, cols] | tie) for _, _, slot in _strassen_blocks(lv)]
                for slot, w in enumerate(_strassen_rhs(blocks)):
                    if slot in grp and not any(w is blk for blk in blocks):
                        e[slot, rows, cols] = _pack(w)

        cp_x.wait()
        cp_x2.start()
        for cp in cp_f:
            cp.start()
        hs_v[...] = pltpu.bitcast(
            jnp.concatenate([mem0_ref[...].astype(F32), ada1(x_v[0])], axis=0).astype(BF16), U32)
        scale = Dh ** -0.5
        n_g = H // G

        def step(s, side):
            ri = lax.broadcasted_iota(jnp.int32, (2 * L, 2 * L), 0)
            ci = lax.broadcasted_iota(jnp.int32, (2 * L, 2 * L), 1)
            same = (ri >= L) == (ci >= L)
            rl = jnp.where(ri >= L, ri - L, ri)
            cl = jnp.where(ci >= L, ci - L, ci)
            keep = same & ((rl < M) | (rl >= cl))
            fill = jnp.where(same, -1e9 / scale, -jnp.inf).astype(F32)
            early = pl.ds(pl.multiple_of(s * P, P), P)

            def gcols(g):
                return slice(g * G * Dh, (g + 1) * G * Dh)

            def proj(t, g):
                return _dot(pltpu.bitcast(hs_v[...], BF16), pltpu.bitcast(wqkv[t, :, gcols(g)], BF16))

            def stack(a, t, g, p):
                hp = g * G // 2 + p
                pre = _unpack(pre_v[t, early, hp * Dh:(hp + 1) * Dh])
                return jnp.concatenate([a[:, (2 * p) * Dh:(2 * p + 1) * Dh], pre[0],
                                        a[:, (2 * p + 1) * Dh:(2 * p + 2) * Dh], pre[1]], axis=0).astype(BF16)

            def scores(g, q, k):
                res = []
                for p in range(G // 2):
                    sc = jnp.where(keep, _dot(stack(q, 0, g, p), stack(k, 1, g, p), _NT), fill)
                    e = jnp.exp2((sc - jnp.max(sc, axis=-1, keepdims=True)) * (scale * _LOG2E))
                    den = jnp.sum(e, axis=-1, keepdims=True)
                    r = pl.reciprocal(den, approx=True)
                    res.append((e.astype(BF16), r * (2.0 - den * r)))
                return res

            def values(g, res, v):
                for p, (e, inv) in enumerate(res):
                    o = _dot(e, stack(v, 2, g, p)) * inv
                    h0 = g * G + 2 * p
                    o_v[:, h0 * Dh:(h0 + 1) * Dh] = o[0:L]
                    o_v[:, (h0 + 1) * Dh:(h0 + 2) * Dh] = o[L:2 * L]

            def outp(g):
                return _dot(o_v[:, gcols(g)],
                            pltpu.bitcast(wo32[g * G * Dh // 2:(g + 1) * G * Dh // 2, :], BF16))

            h_next = ada1(x_v[jnp.minimum(s + 1, n_seg - 1)])
            qk, sm, vv = {}, {}, {}
            for g in range(n_g):
                qk[g] = proj(0, g), proj(1, g)
                if g >= 1:
                    sm[g - 1] = scores(g - 1, *qk.pop(g - 1))
                side(g, qk[g][1])
            for g in range(n_g):
                vv[g] = proj(2, g)
                side(n_g + g, vv[g])
                if g == 0:
                    sm[n_g - 1] = scores(n_g - 1, *qk.pop(n_g - 1))
                else:
                    values(g - 1, sm.pop(g - 1), vv.pop(g - 1))
            acc = outp(0)
            values(n_g - 1, sm.pop(n_g - 1), vv.pop(n_g - 1))
            for g in range(1, n_g):
                side(2 * n_g - 1 + g, acc)
                acc = acc + outp(g)
            hs_v[...] = pltpu.bitcast(jnp.concatenate([acc[0:M], h_next], axis=0).astype(BF16), U32)
            x_v[s] = (x_v[s].astype(F32) + mod_v[0:1, 2 * D:3 * D] * acc[M:L]).astype(x_v.dtype)

        def steps(i, carry):
            for j in range(UN):
                per = 3 * n_g - 1
                step(i * UN + j, lambda k, anchor, j=j: prep_ffn(i, j * per + k, UN * per, anchor))
            return carry

        def phase(ph, carry):
            @pl.when(ph == 1)
            def _():
                cp_x2.wait()
                for cp in cp_f:
                    cp.wait()
            return lax.fori_loop(ph * first_prep, jnp.where(ph == 0, first_prep, n_it), steps, carry)

        lax.fori_loop(0, 2, phase, 0)

        def resid(i):
            return x_v[pl.ds(i * (BM // T), BM // T)].astype(F32).reshape(BM, D)

        def ada2(i):
            h2 = _layernorm(resid(i)) * (1.0 + mod_v[0:1, 4 * D:5 * D]) + mod_v[0:1, 3 * D:4 * D]
            return _strassen_lhs(h2, LV)

        def matmul(lhs, e, cols=slice(None)):
            return _strassen_out([_dot(a, pltpu.bitcast(e[k, 0:e.shape[1] - 8, cols], BF16))
                                  for k, a in enumerate(lhs)])

        def put_h2(parts):
            for j, part in enumerate(parts):
                h2_v[j] = pltpu.bitcast(part, U32)

        put_h2(ada2(0))

        def out_copy(i):
            r = pl.ds(i * (BM // T), BM // T)
            return pltpu.make_async_copy(x_v.at[r], out_hbm.at[r], sem_y.at[i])

        def ffn(i, carry):
            lhs = [pltpu.bitcast(h2_v[j], BF16) for j in range(h2_v.shape[0])]
            h2_next = ada2(jnp.minimum(i + 1, S // BM - 1))
            for c0 in range(0, e1_v.shape[2], FC):
                cols = slice(c0, c0 + FC)
                act = _silu(matmul(lhs, e1_v, cols)) * matmul(lhs, e3_v, cols)
                for j, part in enumerate(_strassen_lhs(act, LV)):
                    act_v[j, :, cols] = pltpu.bitcast(part, U32)
            ffn_out = matmul([pltpu.bitcast(act_v[j], BF16) for j in range(7 ** LV)], e2_v)
            y = resid(i) + mod_v[0:1, 5 * D:6 * D] * ffn_out
            x_v[pl.ds(i * (BM // T), BM // T)] = y.reshape(BM // T, T, D).astype(x_v.dtype)
            put_h2(h2_next)
            out_copy(i).start()
            return carry

        lax.fori_loop(0, S // BM, ffn, 0)
        for i in range(S // BM):
            out_copy(i).wait()

    pl.run_scoped(main,
                  *[pltpu.VMEM((7 ** lv, (w.shape[0] >> (lv + 1)) + 8, w.shape[1] >> lv), U32)
                    for w, lv in ffn_cfg],
                  pltpu.VMEM((7 ** LV, BM >> (LV + 1), D >> LV), U32),
                  pltpu.VMEM((7 ** LV, BM >> (LV + 1), F >> LV), U32),
                  pltpu.SemaphoreType.DMA((sum(4 ** lv for _, lv in ffn_cfg),)),
                  pltpu.SemaphoreType.DMA((S // BM,)))


@functools.partial(jax.jit, static_argnames=("A_seg_len",))
def pallas_adaLN_cond__memory_aug_recurrent_mem_tr__glu_gated_swiglu__prompt_kernel(
    A_x, A_mem0, A_Wq, A_Wk, A_Wv, A_Wo, A_seg_len, B_x, B_w1, B_w3, B_w2, c, w_mod,
):
    del B_x
    B, S, D = A_x.shape
    _, H, Dh = A_Wq.shape
    M, T, F = A_mem0.shape[1], int(A_seg_len), B_w1.shape[1]
    assert B == 1 and S % T == 0
    L, HD = M + T, H * Dh
    hbm = pl.BlockSpec(memory_space=pl.ANY)
    vmem = pl.BlockSpec(memory_space=pltpu.VMEM)
    body = functools.partial(_body, S=S, D=D, H=H, Dh=Dh, M=M, T=T, F=F, G=8, BM=128, FC=128, LV=2)
    out = pl.pallas_call(
        body,
        out_shape=jax.ShapeDtypeStruct((S // T, T, D), A_x.dtype),
        in_specs=[hbm, vmem, hbm, hbm, hbm, hbm, hbm, hbm, hbm, vmem, hbm],
        out_specs=hbm,
        scratch_shapes=[
            pltpu.VMEM((3, D // 2, HD), U32), pltpu.VMEM((HD // 2, D), U32),
            pltpu.VMEM((3, S // T * 8, HD // 2), U32),
            pltpu.VMEM((S // T, T, D), A_x.dtype), pltpu.VMEM((8, 6 * D), F32),
            pltpu.VMEM((D // 256, 8, 512), F32),
            pltpu.VMEM(((L - 8) // 2, D), U32), pltpu.VMEM((L, HD), F32), pltpu.VMEM((8, 128), U32),
            pltpu.SemaphoreType.DMA((2,)),
        ],
        compiler_params=pltpu.CompilerParams(vmem_limit_bytes=126 * 2**20, flags={'XLA_TPU_EVENLY_DISTRIBUTE_CRITICAL_NODES': True}),
    )(A_x.reshape(S // T, T, D), A_mem0.reshape(M, D),
      A_Wq.reshape(D // 2, 2 * H, Dh), A_Wk.reshape(D // 2, 2 * H, Dh), A_Wv.reshape(D // 2, 2 * H, Dh), A_Wo.reshape(HD, D),
      B_w1, B_w3, B_w2, c, w_mod)
    return out.reshape(B, S, D)
```

```python
import functools

import jax
import jax.numpy as jnp
from jax import lax
import jax.experimental.pallas as pl
import jax.experimental.pallas.tpu as pltpu

F32, BF16, U32 = jnp.float32, jnp.bfloat16, jnp.uint32
_LOG2E = 1.4426950408889634
_NN = (((1,), (0,)), ((), ()))
_NT = (((1,), (1,)), ((), ()))


def _dot(a, b, dims=_NN):
    return lax.dot_general(a, b, dims, preferred_element_type=F32)


def _layernorm(x, eps=1e-5):
    m = jnp.mean(x, axis=-1, keepdims=True)
    d = x - m
    v = jnp.mean(d * d, axis=-1, keepdims=True)
    return d * lax.rsqrt(v + eps)


def _silu(x):
    h = 0.5 * x
    return h + h * jnp.tanh(h)


def _unpack(w):
    return jnp.stack([pltpu.unpack_elementwise(w, index=i, packed_dtype=BF16, unpacked_dtype=F32)
                      for i in range(2)])


def _pack(x):
    return pltpu.bitcast(pltpu.pack_elementwise([x[0], x[1]], packed_dtype=BF16), U32)


def _strassen_lhs(a, levels):
    if levels == 0:
        return [a.astype(BF16)]
    m, k = a.shape[0] // 2, a.shape[1] // 2
    a11, a12, a21, a22 = a[:m, :k], a[:m, k:], a[m:, :k], a[m:, k:]
    return [x for v in (a11 + a22, a21 + a22, a11, a22, a11 + a12, a21 - a11, a12 - a22)
            for x in _strassen_lhs(v, levels - 1)]


def _strassen_rhs(blocks):
    if len(blocks) == 1:
        return blocks
    n = len(blocks) // 4
    b11, b12, b21, b22 = (blocks[i * n:(i + 1) * n] for i in range(4))
    add = lambda x, y: [u + v for u, v in zip(x, y)]
    sub = lambda x, y: [u - v for u, v in zip(x, y)]
    return [x for v in (add(b11, b22), b11, sub(b12, b22), sub(b21, b11), b22, add(b11, b12), add(b21, b22))
            for x in _strassen_rhs(v)]


def _strassen_blocks(levels):
    out = [(0, 0, 0)]
    for _ in range(levels):
        out = [(2 * i + q // 2, 2 * j + q % 2, 7 * slot + 1 + q) for i, j, slot in out for q in range(4)]
    return out


def _strassen_out(m):
    if len(m) == 1:
        return m[0]
    n = len(m) // 7
    m1, m2, m3, m4, m5, m6, m7 = (_strassen_out(m[i * n:(i + 1) * n]) for i in range(7))
    return jnp.concatenate([jnp.concatenate([m1 + m4 - m5 + m7, m3 + m5], axis=1),
                            jnp.concatenate([m2 + m4, m1 - m2 + m3 + m6], axis=1)], axis=0)


def _body(x_hbm, mem0_ref, wq_hbm, wk_hbm, wv_hbm, wo_hbm, w1_hbm, w3_hbm, w2_hbm,
          c_ref, wm_hbm, out_hbm,
          wqkv, wo32, pre_v, x_v, mod_v, mod1_v, hs_v, o_v, zero_v, sems,
          *, S, D, H, Dh, M, T, F, G, BM, FC, LV):
    n_seg = S // T
    L = M + T
    HD = H * Dh
    UN = 2
    P = 8
    KC = 256
    n_kc = D // KC
    wo_src = wo_hbm.bitcast(U32)
    wm_src = wm_hbm.bitcast(U32)
    HP = H + 8
    n_it = n_seg // UN
    first_prep = n_it // 8
    XA = first_prep * UN + 1
    cp_x = pltpu.make_async_copy(x_hbm.at[pl.ds(0, XA)], x_v.at[pl.ds(0, XA)], sems.at[0])
    cp_x2 = pltpu.make_async_copy(x_hbm.at[pl.ds(XA, n_seg - XA)], x_v.at[pl.ds(XA, n_seg - XA)], sems.at[1])

    zero_v[...] = jnp.zeros(zero_v.shape, U32)

    def after(anchor):
        return pltpu.bitcast(anchor[0:8, 0:128], U32) & zero_v[...]

    def silu_c():
        return jnp.broadcast_to(_silu(c_ref[...].astype(F32)), (8, D)).astype(BF16)

    def ada1(x):
        return _layernorm(x.astype(F32)[:T - P]) * (1.0 + mod_v[0:1, D:2 * D]) + mod_v[0:1, 0:D]

    def startup(wm_v, wr_v, raw, xp_v, xn_v, hp_v, acc_v, sem_m, sem_w, sem_p):
        srcs = [w.bitcast(U32) for w in (wq_hbm, wk_hbm, wv_hbm)]
        n_j = 3 * n_kc
        R = n_seg * P

        def cp_w(j, t=0):
            return pltpu.make_async_copy(srcs[t].at[pl.ds((j % n_kc) * (KC // 2), KC // 2)],
                                         raw.at[pl.ds(j * (KC // 2), KC // 2), pl.ds(0, H)], sem_w.at[j])

        def cp_m(c, i):
            return pltpu.make_async_copy(wm_src.at[:, pl.ds(pl.multiple_of(i * D + c * KC, KC), KC)],
                                         wm_v.at[c, :, pl.ds(i * KC, KC)], sem_m.at[2 * c + i])

        def start(j):
            cp_m(j, 0).start()
            cp_m(j, 1).start()
            cp_w(j).start()

        def cp_o(i):
            r = pl.ds(pl.multiple_of(i * (HD // 16), HD // 16), HD // 16)
            return pltpu.make_async_copy(wo_src.at[r], wo32.at[r], sem_p.at[1 + i])

        def cp_r(i):
            r = pl.ds(pl.multiple_of(i * (D // 16), D // 16), D // 16)
            return pltpu.make_async_copy(wm_src.at[r, pl.ds(2 * D, 4 * D)], wr_v.at[r], sem_p.at[9 + i])

        cp_p = pltpu.make_async_copy(x_hbm.at[:, pl.ds(T - P, P), :], xp_v, sem_p.at[0])
        cp_p.start()
        start(0)

        cp_p.wait()

        def norm(i, carry):
            xn = _layernorm(xp_v[pl.ds(i * 8, 8)].astype(F32).reshape(8 * P, D))
            for c in range(n_kc):
                xn_v[c, pl.ds(pl.multiple_of(i * 8 * P, 8 * P), 8 * P), :] = xn[:, c * KC:(c + 1) * KC]
            return carry
        lax.fori_loop(0, n_seg // 8, norm, 0)
        start(1)
        raw2 = raw.reshape(3 * D // 2 * HP, Dh)

        def chunk(j, carry):
            t, c = j // n_kc, j % n_kc

            @pl.when(j < n_kc)
            def _():
                cp_m(c, 0).wait()
                cp_m(c, 1).wait()

                @pl.when(j + 2 < n_kc)
                def _():
                    start(j + 2)
                mod = _dot(silu_c(), pltpu.bitcast(wm_v[c], BF16))
                mod1_v[c] = mod
                h = xn_v[c] * (1.0 + mod[0:1, KC:]) + mod[0:1, :KC]
                for i, part in enumerate(_strassen_lhs(h, 1)):
                    hp_v[c, i] = pltpu.bitcast(part, U32)

            cp_w(j).wait()
            for src in (1, 2):
                @pl.when((j + 2) // n_kc == src)
                def _(src=src):
                    cp_w(j + 2, src).start()

            @pl.when(j >= n_j - 8)
            def _():
                cp_r(j - (n_j - 8)).start()
                cp_o(j - (n_j - 8)).start()

            @pl.when(j == n_j - 2)
            def _():
                cp_x.start()

            q4 = KC // 4
            for hp in range(H // 2):
                blk = []
                for half in range(2):
                    base = (j * 2 + half) * (q4 * HP) + hp
                    a = _unpack(raw2[pl.ds(base, q4, stride=HP), :])
                    b = _unpack(raw2[pl.ds(base + H // 2, q4, stride=HP), :])
                    blk += [jnp.stack([a[0], b[0]]), jnp.stack([a[1], b[1]])]
                tiles = [_pack(v) for v in blk]
                cols = [slice((2 * hp + i) * Dh, (2 * hp + i + 1) * Dh) for i in range(2)]
                for i, tile in enumerate(tiles):
                    wqkv[t, pl.ds(pl.multiple_of((2 * c + i // 2) * q4, q4), q4), cols[i % 2]] = tile
                part = _strassen_out([_dot(pltpu.bitcast(hp_v[c, i], BF16), pltpu.bitcast(_pack(w), BF16))
                                      for i, w in enumerate(_strassen_rhs(blk))])
                pair = slice(2 * hp * Dh, (2 * hp + 2) * Dh)
                part = jnp.where(c > 0, acc_v[:, pair], 0.0) + part
                acc_v[:, pair] = part
                pre_v[t, :, hp * Dh:(hp + 1) * Dh] = _pack((part[:, :Dh], part[:, Dh:]))
            return carry

        lax.fori_loop(0, n_j, chunk, 0)
        for c in range(n_kc):
            mod_v[:, c * KC:(c + 1) * KC] = mod1_v[c, :, :KC]
            mod_v[:, D + c * KC:D + (c + 1) * KC] = mod1_v[c, :, KC:]
        for i in range(8):
            cp_r(i).wait()
        mod_v[:, 2 * D:6 * D] = _dot(silu_c(), pltpu.bitcast(wr_v[...], BF16))
        for i in range(8):
            cp_o(i).wait()

    pl.run_scoped(startup,
                  pltpu.VMEM((n_kc, D // 2, 2 * KC), U32), pltpu.VMEM((D // 2, 4 * D), U32),
                  pltpu.VMEM((3 * D // 2, HP, Dh), U32),
                  pltpu.VMEM((n_seg, P, D), x_hbm.dtype), pltpu.VMEM((n_kc, n_seg * P, KC), F32),
                  pltpu.VMEM((n_kc, 7, n_seg * P // 4, KC // 2), U32), pltpu.VMEM((n_seg * P, HD), F32),
                  pltpu.SemaphoreType.DMA((2 * n_kc,)), pltpu.SemaphoreType.DMA((3 * n_kc,)),
                  pltpu.SemaphoreType.DMA((17,)))

    ffn_cfg = ((w1_hbm, LV), (w3_hbm, LV), (w2_hbm, LV))

    def main(e1_v, e3_v, e2_v, h2_v, sem_f, sem_y):
        cp_f, pieces = [], []
        for (src, lv), e in zip(ffn_cfg, (e1_v, e3_v, e2_v)):
            R, n = e.shape[1] - 8, e.shape[2]
            for bi, bj, slot in _strassen_blocks(lv):
                cp_f.append(pltpu.make_async_copy(src.bitcast(U32).at[pl.ds(bi * R, R), pl.ds(bj * n, n)],
                                                  e.at[slot, pl.ds(0, R)], sem_f.at[len(cp_f)]))
                e[slot, R:R + 8, 0:128] = jnp.zeros((8, 128), U32)
            per_it = pl.cdiv(R // 8 * (n // 128), n_it - first_prep)
            groups = [range(7)] if lv == 1 else [range(7 * o, 7 * o + 7) for o in (0, 5, 6, 2, 3, 1, 4)]
            pieces += [(e, lv, per_it, u, grp) for u in range(per_it) for grp in groups]

        def prep_ffn(i, site, n_sites, anchor):
            per = pl.cdiv(len(pieces), n_sites)
            for k, (e, lv, per_it, u, grp) in enumerate(pieces[site * per:(site + 1) * per]):
                tie = after(anchor[:, (k * 128) % anchor.shape[1]:])
                n_r, n_c = e.shape[1] // 8 - 1, e.shape[2] // 128
                pos = jnp.maximum(i - first_prep, 0) * per_it + u
                live = (i >= first_prep) & (pos < n_r * n_c)
                rows = pl.ds(pl.multiple_of(jnp.where(live, lax.rem(pos, n_r), n_r) * 8, 8), 8)
                cols = pl.ds(pl.multiple_of(jnp.where(live, lax.div(pos, n_r), 0) * 128, 128), 128)
                blocks = [_unpack(e[slot, rows, cols] | tie) for _, _, slot in _strassen_blocks(lv)]
                for slot, w in enumerate(_strassen_rhs(blocks)):
                    if slot in grp and not any(w is blk for blk in blocks):
                        e[slot, rows, cols] = _pack(w)

        cp_x.wait()
        cp_x2.start()
        for cp in cp_f:
            cp.start()
        hs_v[...] = pltpu.bitcast(
            jnp.concatenate([mem0_ref[...].astype(F32), ada1(x_v[0])], axis=0).astype(BF16), U32)
        scale = Dh ** -0.5
        n_g = H // G

        def step(s, side):
            ri = lax.broadcasted_iota(jnp.int32, (2 * L, 2 * L), 0)
            ci = lax.broadcasted_iota(jnp.int32, (2 * L, 2 * L), 1)
            same = (ri >= L) == (ci >= L)
            rl = jnp.where(ri >= L, ri - L, ri)
            cl = jnp.where(ci >= L, ci - L, ci)
            keep = same & ((rl < M) | (rl >= cl))
            fill = jnp.where(same, -1e9 / scale, -jnp.inf).astype(F32)
            early = pl.ds(pl.multiple_of(s * P, P), P)

            def gcols(g):
                return slice(g * G * Dh, (g + 1) * G * Dh)

            def proj(t, g):
                return _dot(pltpu.bitcast(hs_v[...], BF16), pltpu.bitcast(wqkv[t, :, gcols(g)], BF16))

            def stack(a, t, g, p):
                hp = g * G // 2 + p
                pre = _unpack(pre_v[t, early, hp * Dh:(hp + 1) * Dh])
                return jnp.concatenate([a[:, (2 * p) * Dh:(2 * p + 1) * Dh], pre[0],
                                        a[:, (2 * p + 1) * Dh:(2 * p + 2) * Dh], pre[1]], axis=0).astype(BF16)

            def scores(g, q, k):
                res = []
                for p in range(G // 2):
                    sc = jnp.where(keep, _dot(stack(q, 0, g, p), stack(k, 1, g, p), _NT), fill)
                    e = jnp.exp2((sc - jnp.max(sc, axis=-1, keepdims=True)) * (scale * _LOG2E))
                    den = jnp.sum(e, axis=-1, keepdims=True)
                    r = pl.reciprocal(den, approx=True)
                    res.append((e.astype(BF16), r * (2.0 - den * r)))
                return res

            def values(g, res, v):
                for p, (e, inv) in enumerate(res):
                    o = _dot(e, stack(v, 2, g, p)) * inv
                    h0 = g * G + 2 * p
                    o_v[:, h0 * Dh:(h0 + 1) * Dh] = o[0:L]
                    o_v[:, (h0 + 1) * Dh:(h0 + 2) * Dh] = o[L:2 * L]

            def outp(g):
                return _dot(o_v[:, gcols(g)],
                            pltpu.bitcast(wo32[g * G * Dh // 2:(g + 1) * G * Dh // 2, :], BF16))

            h_next = ada1(x_v[jnp.minimum(s + 1, n_seg - 1)])
            qk, sm, vv = {}, {}, {}
            for g in range(n_g):
                qk[g] = proj(0, g), proj(1, g)
                if g >= 1:
                    sm[g - 1] = scores(g - 1, *qk.pop(g - 1))
            for g in range(n_g):
                vv[g] = proj(2, g)
                side(g, vv[g])
                if g == 0:
                    sm[n_g - 1] = scores(n_g - 1, *qk.pop(n_g - 1))
                else:
                    values(g - 1, sm.pop(g - 1), vv.pop(g - 1))
            acc = outp(0)
            values(n_g - 1, sm.pop(n_g - 1), vv.pop(n_g - 1))
            for g in range(1, n_g):
                side(n_g - 1 + g, acc)
                acc = acc + outp(g)
            hs_v[...] = pltpu.bitcast(jnp.concatenate([acc[0:M], h_next], axis=0).astype(BF16), U32)
            x_v[s] = (x_v[s].astype(F32) + mod_v[0:1, 2 * D:3 * D] * acc[M:L]).astype(x_v.dtype)

        def steps(i, carry):
            for j in range(UN):
                per = 2 * n_g - 1
                step(i * UN + j, lambda k, anchor, j=j: prep_ffn(i, j * per + k, UN * per, anchor))
            return carry

        def phase(ph, carry):
            @pl.when(ph == 1)
            def _():
                cp_x2.wait()
                for cp in cp_f:
                    cp.wait()
            return lax.fori_loop(ph * first_prep, jnp.where(ph == 0, first_prep, n_it), steps, carry)

        lax.fori_loop(0, 2, phase, 0)

        def resid(i):
            return x_v[pl.ds(i * (BM // T), BM // T)].astype(F32).reshape(BM, D)

        def ada2(i):
            h2 = _layernorm(resid(i)) * (1.0 + mod_v[0:1, 4 * D:5 * D]) + mod_v[0:1, 3 * D:4 * D]
            return _strassen_lhs(h2, LV)

        def matmul(lhs, e, cols=slice(None)):
            return _strassen_out([_dot(a, pltpu.bitcast(e[k, 0:e.shape[1] - 8, cols], BF16))
                                  for k, a in enumerate(lhs)])

        def put_h2(parts):
            for j, part in enumerate(parts):
                h2_v[j] = part

        put_h2(ada2(0))

        def out_copy(i):
            r = pl.ds(i * (BM // T), BM // T)
            return pltpu.make_async_copy(x_v.at[r], out_hbm.at[r], sem_y.at[i])

        def ffn(i, carry):
            h2_next = ada2(jnp.minimum(i + 1, S // BM - 1))
            acts = []
            for c0 in range(0, e1_v.shape[2], FC):
                cols = slice(c0, c0 + FC)
                gate, up = [matmul([h2_v[j] for j in range(7 ** LV)], e, cols)
                            for e in (e1_v, e3_v)]
                act = _silu(gate) * up
                acts.append(_strassen_lhs(act, LV))
            put_h2(h2_next)
            ffn_out = matmul([jnp.concatenate(parts, axis=1) for parts in zip(*acts)], e2_v)
            y = resid(i) + mod_v[0:1, 5 * D:6 * D] * ffn_out
            x_v[pl.ds(i * (BM // T), BM // T)] = y.reshape(BM // T, T, D).astype(x_v.dtype)
            out_copy(i).start()
            return carry

        lax.fori_loop(0, S // BM, ffn, 0)
        for i in range(S // BM):
            out_copy(i).wait()

    pl.run_scoped(main,
                  *[pltpu.VMEM((7 ** lv, (w.shape[0] >> (lv + 1)) + 8, w.shape[1] >> lv), U32)
                    for w, lv in ffn_cfg],
                  pltpu.VMEM((7 ** LV, BM >> LV, D >> LV), BF16),
                  pltpu.SemaphoreType.DMA((sum(4 ** lv for _, lv in ffn_cfg),)),
                  pltpu.SemaphoreType.DMA((S // BM,)))


@functools.partial(jax.jit, static_argnames=("A_seg_len",))
def pallas_adaLN_cond__memory_aug_recurrent_mem_tr__glu_gated_swiglu__prompt_kernel(
    A_x, A_mem0, A_Wq, A_Wk, A_Wv, A_Wo, A_seg_len, B_x, B_w1, B_w3, B_w2, c, w_mod,
):
    del B_x
    B, S, D = A_x.shape
    _, H, Dh = A_Wq.shape
    M, T, F = A_mem0.shape[1], int(A_seg_len), B_w1.shape[1]
    assert B == 1 and S % T == 0
    L, HD = M + T, H * Dh
    hbm = pl.BlockSpec(memory_space=pl.ANY)
    vmem = pl.BlockSpec(memory_space=pltpu.VMEM)
    body = functools.partial(_body, S=S, D=D, H=H, Dh=Dh, M=M, T=T, F=F, G=8, BM=128, FC=128, LV=2)
    out = pl.pallas_call(
        body,
        out_shape=jax.ShapeDtypeStruct((S // T, T, D), A_x.dtype),
        in_specs=[hbm, vmem, hbm, hbm, hbm, hbm, hbm, hbm, hbm, vmem, hbm],
        out_specs=hbm,
        scratch_shapes=[
            pltpu.VMEM((3, D // 2, HD), U32), pltpu.VMEM((HD // 2, D), U32),
            pltpu.VMEM((3, S // T * 8, HD // 2), U32),
            pltpu.VMEM((S // T, T, D), A_x.dtype), pltpu.VMEM((8, 6 * D), F32),
            pltpu.VMEM((D // 256, 8, 512), F32),
            pltpu.VMEM(((L - 8) // 2, D), U32), pltpu.VMEM((L, HD), F32), pltpu.VMEM((8, 128), U32),
            pltpu.SemaphoreType.DMA((2,)),
        ],
        compiler_params=pltpu.CompilerParams(vmem_limit_bytes=126 * 2**20, flags={'XLA_TPU_EVENLY_DISTRIBUTE_CRITICAL_NODES': True}),
    )(A_x.reshape(S // T, T, D), A_mem0.reshape(M, D),
      A_Wq.reshape(D // 2, 2 * H, Dh), A_Wk.reshape(D // 2, 2 * H, Dh), A_Wv.reshape(D // 2, 2 * H, Dh), A_Wo.reshape(HD, D),
      B_w1, B_w3, B_w2, c, w_mod)
    return out.reshape(B, S, D)
```

```python
import functools

import numpy as np
import jax
import jax.numpy as jnp
from jax import lax
import jax.experimental.pallas as pl
import jax.experimental.pallas.tpu as pltpu

F32, BF16, U32 = jnp.float32, jnp.bfloat16, jnp.uint32
_HIGH = np.uint32(0xFFFF0000)
_LOG2E = 1.4426950408889634
_NN = (((1,), (0,)), ((), ()))
_NT = (((1,), (1,)), ((), ()))


def _dot(a, b, dims=_NN):
    return lax.dot_general(a, b, dims, preferred_element_type=F32)


def _layernorm(x, eps=1e-5):
    m = jnp.mean(x, axis=-1, keepdims=True)
    d = x - m
    v = jnp.mean(d * d, axis=-1, keepdims=True)
    return d * lax.rsqrt(v + eps)


def _silu(x):
    h = 0.5 * x
    return h + h * jnp.tanh(h)


def _unpack(w):
    return jnp.stack([lax.bitcast_convert_type(v, F32) for v in (w << 16, w & _HIGH)])


def _pack(x, exact=False):
    lo, hi = (lax.bitcast_convert_type(v if exact else v.astype(BF16).astype(F32), U32) for v in (x[0], x[1]))
    return (lo >> 16) | hi


def _strassen_lhs(a, levels):
    if levels == 0:
        return [a.astype(BF16)]
    m, k = a.shape[0] // 2, a.shape[1] // 2
    a11, a12, a21, a22 = a[:m, :k], a[:m, k:], a[m:, :k], a[m:, k:]
    return [x for v in (a11 + a22, a21 + a22, a11, a22, a11 + a12, a21 - a11, a12 - a22)
            for x in _strassen_lhs(v, levels - 1)]


def _strassen_rhs(blocks):
    if len(blocks) == 1:
        return blocks
    n = len(blocks) // 4
    b11, b12, b21, b22 = (blocks[i * n:(i + 1) * n] for i in range(4))
    add = lambda x, y: [u + v for u, v in zip(x, y)]
    sub = lambda x, y: [u - v for u, v in zip(x, y)]
    return [x for v in (add(b11, b22), b11, sub(b12, b22), sub(b21, b11), b22, add(b11, b12), add(b21, b22))
            for x in _strassen_rhs(v)]


def _strassen_blocks(levels):
    out = [(0, 0, 0)]
    for _ in range(levels):
        out = [(2 * i + q // 2, 2 * j + q % 2, 7 * slot + 1 + q) for i, j, slot in out for q in range(4)]
    return out


def _strassen_out(m):
    if len(m) == 1:
        return m[0]
    n = len(m) // 7
    m1, m2, m3, m4, m5, m6, m7 = (_strassen_out(m[i * n:(i + 1) * n]) for i in range(7))
    return jnp.concatenate([jnp.concatenate([m1 + m4 - m5 + m7, m3 + m5], axis=1),
                            jnp.concatenate([m2 + m4, m1 - m2 + m3 + m6], axis=1)], axis=0)


def _body(x_hbm, mem0_ref, wq_hbm, wk_hbm, wv_hbm, wo_hbm, w1_hbm, w3_hbm, w2_hbm,
          c_ref, wm_hbm, out_hbm,
          wqkv, wo32, pre_v, x_v, mod_v, mod1_v, hs_v, o_v, zero_v, sems,
          *, S, D, H, Dh, M, T, F, G, BM, FC, LV):
    n_seg = S // T
    L = M + T
    HD = H * Dh
    UN = 2
    P = 8
    KC = 256
    n_kc = D // KC
    wo_src = wo_hbm.bitcast(U32)
    wm_src = wm_hbm.bitcast(U32)
    HP = H + 8
    CP = KC // 2 + 1
    n_it = n_seg // UN
    first_prep = n_it // 8
    XA = first_prep * UN + 1
    cp_x = pltpu.make_async_copy(x_hbm.at[pl.ds(0, XA)], x_v.at[pl.ds(0, XA)], sems.at[0])
    cp_x2 = pltpu.make_async_copy(x_hbm.at[pl.ds(XA, n_seg - XA)], x_v.at[pl.ds(XA, n_seg - XA)], sems.at[1])

    zero_v[...] = jnp.zeros(zero_v.shape, U32)

    def after(anchor):
        return pltpu.bitcast(anchor[0:8, 0:128], U32) & zero_v[...]

    def silu_c():
        return jnp.broadcast_to(_silu(c_ref[...].astype(F32)), (8, D)).astype(BF16)

    def ada1(x):
        return _layernorm(x.astype(F32)[:T - P]) * (1.0 + mod_v[0:1, D:2 * D]) + mod_v[0:1, 0:D]

    def startup(wm_v, wr_v, raw, xp_v, xn_v, hp_v, acc_v, sem_m, sem_w, sem_p):
        srcs = [w.bitcast(U32) for w in (wq_hbm, wk_hbm, wv_hbm)]
        n_j = 3 * n_kc
        R = n_seg * P

        def cp_w(j, t=0):
            return pltpu.make_async_copy(srcs[t].at[pl.ds((j % n_kc) * (KC // 2), KC // 2)],
                                         raw.at[pl.ds(j * CP, KC // 2), pl.ds(0, H)], sem_w.at[j])

        def cp_m(c, i):
            return pltpu.make_async_copy(wm_src.at[:, pl.ds(pl.multiple_of(i * D + c * KC, KC), KC)],
                                         wm_v.at[c, :, pl.ds(i * KC, KC)], sem_m.at[2 * c + i])

        def start(j):
            cp_m(j, 0).start()
            cp_m(j, 1).start()
            cp_w(j).start()

        def cp_o(i):
            r = pl.ds(pl.multiple_of(i * (HD // 16), HD // 16), HD // 16)
            return pltpu.make_async_copy(wo_src.at[r], wo32.at[r], sem_p.at[1 + i])

        def cp_r(i):
            r = pl.ds(pl.multiple_of(i * (D // 16), D // 16), D // 16)
            return pltpu.make_async_copy(wm_src.at[r, pl.ds(2 * D, 4 * D)], wr_v.at[r], sem_p.at[9 + i])

        cp_p = pltpu.make_async_copy(x_hbm.at[:, pl.ds(T - P, P), :], xp_v, sem_p.at[0])
        cp_p.start()
        start(0)

        cp_p.wait()

        def norm(i, carry):
            xn = _layernorm(xp_v[pl.ds(i * 8, 8)].astype(F32).reshape(8 * P, D))
            for c in range(n_kc):
                xn_v[c, pl.ds(pl.multiple_of(i * 8 * P, 8 * P), 8 * P), :] = xn[:, c * KC:(c + 1) * KC]
            return carry
        lax.fori_loop(0, n_seg // 8, norm, 0)
        start(1)
        raw2 = raw.reshape(n_j * CP * HP, Dh)

        def chunk(j, carry):
            t, c = j // n_kc, j % n_kc

            @pl.when(j < n_kc)
            def _():
                cp_m(c, 0).wait()
                cp_m(c, 1).wait()

                @pl.when(j + 2 < n_kc)
                def _():
                    start(j + 2)
                mod = _dot(silu_c(), pltpu.bitcast(wm_v[c], BF16))
                mod1_v[c] = mod
                h = xn_v[c] * (1.0 + mod[0:1, KC:]) + mod[0:1, :KC]
                for i, part in enumerate(_strassen_lhs(h, 1)):
                    hp_v[c, i] = pltpu.bitcast(part, U32)

            cp_w(j).wait()
            for src in (1, 2):
                @pl.when((j + 2) // n_kc == src)
                def _(src=src):
                    cp_w(j + 2, src).start()

            @pl.when(j >= n_j - 8)
            def _():
                cp_r(j - (n_j - 8)).start()
                cp_o(j - (n_j - 8)).start()

            @pl.when(j == n_j - 2)
            def _():
                cp_x.start()

            q4 = KC // 4
            for hp in range(H // 2):
                blk = []
                for half in range(2):
                    base = (j * CP + half * q4) * HP + hp
                    a = _unpack(raw2[pl.ds(base, q4, stride=HP), :])
                    b = _unpack(raw2[pl.ds(base + H // 2, q4, stride=HP), :])
                    blk += [jnp.stack([a[0], b[0]]), jnp.stack([a[1], b[1]])]
                tiles = [_pack(v, exact=True) for v in blk]
                cols = [slice((2 * hp + i) * Dh, (2 * hp + i + 1) * Dh) for i in range(2)]
                for i, tile in enumerate(tiles):
                    wqkv[t, pl.ds(pl.multiple_of((2 * c + i // 2) * q4, q4), q4), cols[i % 2]] = tile
                part = _strassen_out([_dot(pltpu.bitcast(hp_v[c, i], BF16), pltpu.bitcast(_pack(w, exact=i in (1, 4)), BF16))
                                      for i, w in enumerate(_strassen_rhs(blk))])
                pair = slice(2 * hp * Dh, (2 * hp + 2) * Dh)
                part = jnp.where(c > 0, acc_v[:, pair], 0.0) + part
                acc_v[:, pair] = part
                pre_v[t, :, hp * Dh:(hp + 1) * Dh] = _pack((part[:, :Dh], part[:, Dh:]))
            return carry

        lax.fori_loop(0, n_j, chunk, 0)
        for c in range(n_kc):
            mod_v[:, c * KC:(c + 1) * KC] = mod1_v[c, :, :KC]
            mod_v[:, D + c * KC:D + (c + 1) * KC] = mod1_v[c, :, KC:]
        for i in range(8):
            cp_r(i).wait()
        mod_v[:, 2 * D:6 * D] = _dot(silu_c(), pltpu.bitcast(wr_v[...], BF16))
        for i in range(8):
            cp_o(i).wait()

    pl.run_scoped(startup,
                  pltpu.VMEM((n_kc, D // 2, 2 * KC), U32), pltpu.VMEM((D // 2, 4 * D), U32),
                  pltpu.VMEM((3 * n_kc * CP, HP, Dh), U32),
                  pltpu.VMEM((n_seg, P, D), x_hbm.dtype), pltpu.VMEM((n_kc, n_seg * P, KC), F32),
                  pltpu.VMEM((n_kc, 7, n_seg * P // 4, KC // 2), U32), pltpu.VMEM((n_seg * P, HD), F32),
                  pltpu.SemaphoreType.DMA((2 * n_kc,)), pltpu.SemaphoreType.DMA((3 * n_kc,)),
                  pltpu.SemaphoreType.DMA((17,)))

    ffn_cfg = ((w1_hbm, LV), (w3_hbm, LV), (w2_hbm, LV))

    def main(e1_v, e3_v, e2_v, h2_v, sem_f, sem_y):
        cp_f, pieces = [], []
        for (src, lv), e in zip(ffn_cfg, (e1_v, e3_v, e2_v)):
            R, n = e.shape[1] - 8, e.shape[2]
            for bi, bj, slot in _strassen_blocks(lv):
                cp_f.append(pltpu.make_async_copy(src.bitcast(U32).at[pl.ds(bi * R, R), pl.ds(bj * n, n)],
                                                  e.at[slot, pl.ds(0, R)], sem_f.at[len(cp_f)]))
                e[slot, R:R + 8, 0:128] = jnp.zeros((8, 128), U32)
            per_it = pl.cdiv(R // 8 * (n // 128), n_it - first_prep)
            groups = [range(7)] if lv == 1 else [range(7 * o, 7 * o + 7) for o in (0, 5, 6, 2, 3, 1, 4)]
            pieces += [(e, lv, per_it, u, grp) for u in range(per_it) for grp in groups]

        def prep_ffn(i, site, n_sites, anchor):
            per = pl.cdiv(len(pieces), n_sites)
            for k, (e, lv, per_it, u, grp) in enumerate(pieces[site * per:(site + 1) * per]):
                tie = after(anchor[:, (k * 128) % anchor.shape[1]:])
                n_r, n_c = e.shape[1] // 8 - 1, e.shape[2] // 128
                pos = jnp.maximum(i - first_prep, 0) * per_it + u
                live = (i >= first_prep) & (pos < n_r * n_c)
                rows = pl.ds(pl.multiple_of(jnp.where(live, lax.rem(pos, n_r), n_r) * 8, 8), 8)
                cols = pl.ds(pl.multiple_of(jnp.where(live, lax.div(pos, n_r), 0) * 128, 128), 128)
                blocks = [_unpack(e[slot, rows, cols] | tie) for _, _, slot in _strassen_blocks(lv)]
                for slot, w in enumerate(_strassen_rhs(blocks)):
                    if slot in grp and not any(w is blk for blk in blocks):
                        e[slot, rows, cols] = _pack(w)

        cp_x.wait()
        cp_x2.start()
        for cp in cp_f:
            cp.start()
        hs_v[...] = pltpu.bitcast(
            jnp.concatenate([mem0_ref[...].astype(F32), ada1(x_v[0])], axis=0).astype(BF16), U32)
        scale = Dh ** -0.5
        n_g = H // G

        def step(s, side):
            ri = lax.broadcasted_iota(jnp.int32, (2 * L, 2 * L), 0)
            ci = lax.broadcasted_iota(jnp.int32, (2 * L, 2 * L), 1)
            same = (ri >= L) == (ci >= L)
            rl = jnp.where(ri >= L, ri - L, ri)
            cl = jnp.where(ci >= L, ci - L, ci)
            keep = same & ((rl < M) | (rl >= cl))
            fill = jnp.where(same, -1e9 / scale, -jnp.inf).astype(F32)
            early = pl.ds(pl.multiple_of(s * P, P), P)

            def gcols(g):
                return slice(g * G * Dh, (g + 1) * G * Dh)

            def proj(t, g):
                return _dot(pltpu.bitcast(hs_v[...], BF16), pltpu.bitcast(wqkv[t, :, gcols(g)], BF16))

            def stack(a, t, g, p):
                hp = g * G // 2 + p
                pre = _unpack(pre_v[t, early, hp * Dh:(hp + 1) * Dh])
                return jnp.concatenate([a[:, (2 * p) * Dh:(2 * p + 1) * Dh], pre[0],
                                        a[:, (2 * p + 1) * Dh:(2 * p + 2) * Dh], pre[1]], axis=0).astype(BF16)

            def scores(g, q, k):
                res = []
                for p in range(G // 2):
                    sc = jnp.where(keep, _dot(stack(q, 0, g, p), stack(k, 1, g, p), _NT), fill)
                    e = jnp.exp2((sc - jnp.max(sc, axis=-1, keepdims=True)) * (scale * _LOG2E))
                    den = jnp.sum(e, axis=-1, keepdims=True)
                    r = pl.reciprocal(den, approx=True)
                    res.append((e.astype(BF16), r * (2.0 - den * r)))
                return res

            def values(g, res, v):
                for p, (e, inv) in enumerate(res):
                    o = _dot(e, stack(v, 2, g, p)) * inv
                    h0 = g * G + 2 * p
                    o_v[:, h0 * Dh:(h0 + 1) * Dh] = o[0:L]
                    o_v[:, (h0 + 1) * Dh:(h0 + 2) * Dh] = o[L:2 * L]

            def outp(g):
                return _dot(o_v[:, gcols(g)],
                            pltpu.bitcast(wo32[g * G * Dh // 2:(g + 1) * G * Dh // 2, :], BF16))

            h_next = ada1(x_v[jnp.minimum(s + 1, n_seg - 1)])
            qk, sm, vv = {}, {}, {}
            for g in range(n_g):
                qk[g] = proj(0, g), proj(1, g)
                if g >= 1:
                    sm[g - 1] = scores(g - 1, *qk.pop(g - 1))
            for g in range(n_g):
                vv[g] = proj(2, g)
                side(g, vv[g])
                if g == 0:
                    sm[n_g - 1] = scores(n_g - 1, *qk.pop(n_g - 1))
                else:
                    values(g - 1, sm.pop(g - 1), vv.pop(g - 1))
            acc = outp(0)
            values(n_g - 1, sm.pop(n_g - 1), vv.pop(n_g - 1))
            for g in range(1, n_g):
                side(n_g - 1 + g, acc)
                acc = acc + outp(g)
            hs_v[...] = pltpu.bitcast(jnp.concatenate([acc[0:M], h_next], axis=0).astype(BF16), U32)
            x_v[s] = (x_v[s].astype(F32) + mod_v[0:1, 2 * D:3 * D] * acc[M:L]).astype(x_v.dtype)

        def steps(i, carry):
            for j in range(UN):
                per = 2 * n_g - 1
                step(i * UN + j, lambda k, anchor, j=j: prep_ffn(i, j * per + k, UN * per, anchor))
            return carry

        def phase(ph, carry):
            @pl.when(ph == 1)
            def _():
                cp_x2.wait()
                for cp in cp_f:
                    cp.wait()
            return lax.fori_loop(ph * first_prep, jnp.where(ph == 0, first_prep, n_it), steps, carry)

        lax.fori_loop(0, 2, phase, 0)

        def resid(i):
            return x_v[pl.ds(i * (BM // T), BM // T)].astype(F32).reshape(BM, D)

        def ada2(i):
            h2 = _layernorm(resid(i)) * (1.0 + mod_v[0:1, 4 * D:5 * D]) + mod_v[0:1, 3 * D:4 * D]
            return _strassen_lhs(h2, LV)

        def matmul(lhs, e, cols=slice(None)):
            return _strassen_out([_dot(a, pltpu.bitcast(e[k, 0:e.shape[1] - 8, cols], BF16))
                                  for k, a in enumerate(lhs)])

        def put_h2(parts):
            for j, part in enumerate(parts):
                h2_v[j] = part

        put_h2(ada2(0))

        def out_copy(i):
            r = pl.ds(i * (BM // T), BM // T)
            return pltpu.make_async_copy(x_v.at[r], out_hbm.at[r], sem_y.at[i])

        def ffn(i, carry):
            h2_next = ada2(jnp.minimum(i + 1, S // BM - 1))
            acts = []
            for c0 in range(0, e1_v.shape[2], FC):
                cols = slice(c0, c0 + FC)
                gate, up = [matmul([h2_v[j] for j in range(7 ** LV)], e, cols)
                            for e in (e1_v, e3_v)]
                act = _silu(gate) * up
                acts.append(_strassen_lhs(act, LV))
            put_h2(h2_next)
            ffn_out = matmul([jnp.concatenate(parts, axis=1) for parts in zip(*acts)], e2_v)
            y = resid(i) + mod_v[0:1, 5 * D:6 * D] * ffn_out
            x_v[pl.ds(i * (BM // T), BM // T)] = y.reshape(BM // T, T, D).astype(x_v.dtype)
            out_copy(i).start()
            return carry

        lax.fori_loop(0, S // BM, ffn, 0)
        for i in range(S // BM):
            out_copy(i).wait()

    pl.run_scoped(main,
                  *[pltpu.VMEM((7 ** lv, (w.shape[0] >> (lv + 1)) + 8, w.shape[1] >> lv), U32)
                    for w, lv in ffn_cfg],
                  pltpu.VMEM((7 ** LV, BM >> LV, D >> LV), BF16),
                  pltpu.SemaphoreType.DMA((sum(4 ** lv for _, lv in ffn_cfg),)),
                  pltpu.SemaphoreType.DMA((S // BM,)))


@functools.partial(jax.jit, static_argnames=("A_seg_len",))
def pallas_adaLN_cond__memory_aug_recurrent_mem_tr__glu_gated_swiglu__prompt_kernel(
    A_x, A_mem0, A_Wq, A_Wk, A_Wv, A_Wo, A_seg_len, B_x, B_w1, B_w3, B_w2, c, w_mod,
):
    del B_x
    B, S, D = A_x.shape
    _, H, Dh = A_Wq.shape
    M, T, F = A_mem0.shape[1], int(A_seg_len), B_w1.shape[1]
    assert B == 1 and S % T == 0
    L, HD = M + T, H * Dh
    hbm = pl.BlockSpec(memory_space=pl.ANY)
    vmem = pl.BlockSpec(memory_space=pltpu.VMEM)
    body = functools.partial(_body, S=S, D=D, H=H, Dh=Dh, M=M, T=T, F=F, G=8, BM=128, FC=128, LV=2)
    out = pl.pallas_call(
        body,
        out_shape=jax.ShapeDtypeStruct((S // T, T, D), A_x.dtype),
        in_specs=[hbm, vmem, hbm, hbm, hbm, hbm, hbm, hbm, hbm, vmem, hbm],
        out_specs=hbm,
        scratch_shapes=[
            pltpu.VMEM((3, D // 2, HD), U32), pltpu.VMEM((HD // 2, D), U32),
            pltpu.VMEM((3, S // T * 8, HD // 2), U32),
            pltpu.VMEM((S // T, T, D), A_x.dtype), pltpu.VMEM((8, 6 * D), F32),
            pltpu.VMEM((D // 256, 8, 512), F32),
            pltpu.VMEM(((L - 8) // 2, D), U32), pltpu.VMEM((L, HD), F32), pltpu.VMEM((8, 128), U32),
            pltpu.SemaphoreType.DMA((2,)),
        ],
        compiler_params=pltpu.CompilerParams(vmem_limit_bytes=126 * 2**20, flags={'XLA_TPU_EVENLY_DISTRIBUTE_CRITICAL_NODES': True}),
    )(A_x.reshape(S // T, T, D), A_mem0.reshape(M, D),
      A_Wq.reshape(D // 2, 2 * H, Dh), A_Wk.reshape(D // 2, 2 * H, Dh), A_Wv.reshape(D // 2, 2 * H, Dh), A_Wo.reshape(HD, D),
      B_w1, B_w3, B_w2, c, w_mod)
    return out.reshape(B, S, D)
```

```python
import functools

import numpy as np
import jax
import jax.numpy as jnp
from jax import lax
import jax.experimental.pallas as pl
import jax.experimental.pallas.tpu as pltpu

F32, BF16, U32 = jnp.float32, jnp.bfloat16, jnp.uint32
_HIGH = np.uint32(0xFFFF0000)
_LOG2E = 1.4426950408889634
_NN = (((1,), (0,)), ((), ()))
_NT = (((1,), (1,)), ((), ()))


def _dot(a, b, dims=_NN):
    return lax.dot_general(a, b, dims, preferred_element_type=F32)


def _layernorm(x, eps=1e-5):
    m = jnp.mean(x, axis=-1, keepdims=True)
    d = x - m
    v = jnp.mean(d * d, axis=-1, keepdims=True)
    return d * lax.rsqrt(v + eps)


def _silu(x):
    h = 0.5 * x
    return h + h * jnp.tanh(h)


def _unpack(w):
    return jnp.stack([lax.bitcast_convert_type(v, F32) for v in (w << 16, w & _HIGH)])


def _pack(x, exact=False):
    lo, hi = (lax.bitcast_convert_type(v if exact else v.astype(BF16).astype(F32), U32) for v in (x[0], x[1]))
    return (lo >> 16) | hi


def _strassen_lhs(a, levels):
    if levels == 0:
        return [a.astype(BF16)]
    m, k = a.shape[0] // 2, a.shape[1] // 2
    a11, a12, a21, a22 = a[:m, :k], a[:m, k:], a[m:, :k], a[m:, k:]
    return [x for v in (a11 + a22, a21 + a22, a11, a22, a11 + a12, a21 - a11, a12 - a22)
            for x in _strassen_lhs(v, levels - 1)]


def _strassen_rhs(blocks):
    if len(blocks) == 1:
        return blocks
    n = len(blocks) // 4
    b11, b12, b21, b22 = (blocks[i * n:(i + 1) * n] for i in range(4))
    add = lambda x, y: [u + v for u, v in zip(x, y)]
    sub = lambda x, y: [u - v for u, v in zip(x, y)]
    return [x for v in (add(b11, b22), b11, sub(b12, b22), sub(b21, b11), b22, add(b11, b12), add(b21, b22))
            for x in _strassen_rhs(v)]


def _strassen_blocks(levels):
    out = [(0, 0, 0)]
    for _ in range(levels):
        out = [(2 * i + q // 2, 2 * j + q % 2, 7 * slot + 1 + q) for i, j, slot in out for q in range(4)]
    return out


def _strassen_out(m):
    if len(m) == 1:
        return m[0]
    n = len(m) // 7
    m1, m2, m3, m4, m5, m6, m7 = (_strassen_out(m[i * n:(i + 1) * n]) for i in range(7))
    return jnp.concatenate([jnp.concatenate([m1 + m4 - m5 + m7, m3 + m5], axis=1),
                            jnp.concatenate([m2 + m4, m1 - m2 + m3 + m6], axis=1)], axis=0)


def _body(x_hbm, mem0_ref, wq_hbm, wk_hbm, wv_hbm, wo_hbm, w1_hbm, w3_hbm, w2_hbm,
          c_ref, wm_hbm, out_hbm,
          wqkv, wo32, pre_v, x_v, mod_v, mod1_v, hs_v, o_v, zero_v, sems,
          *, S, D, H, Dh, M, T, F, G, BM, FC, LV):
    n_seg = S // T
    L = M + T
    HD = H * Dh
    UN = 2
    P = 8
    KC = 256
    n_kc = D // KC
    wo_src = wo_hbm.bitcast(U32)
    wm_src = wm_hbm.bitcast(U32)
    HP = H // 2 + 8
    CP = KC + 1
    n_it = n_seg // UN
    first_prep = n_it // 8
    XA = first_prep * UN + 1
    cp_x = pltpu.make_async_copy(x_hbm.at[pl.ds(0, XA)], x_v.at[pl.ds(0, XA)], sems.at[0])
    cp_x2 = pltpu.make_async_copy(x_hbm.at[pl.ds(XA, n_seg - XA)], x_v.at[pl.ds(XA, n_seg - XA)], sems.at[1])

    zero_v[...] = jnp.zeros(zero_v.shape, U32)

    def after(anchor):
        return pltpu.bitcast(anchor[0:8, 0:128], U32) & zero_v[...]

    def silu_c():
        return jnp.broadcast_to(_silu(c_ref[...].astype(F32)), (8, D)).astype(BF16)

    def ada1(x):
        return _layernorm(x.astype(F32)[:T - P]) * (1.0 + mod_v[0:1, D:2 * D]) + mod_v[0:1, 0:D]

    def startup(wm_v, wr_v, raw, xp_v, xn_v, hp_v, acc_v, sem_m, sem_w, sem_p):
        srcs = [w.bitcast(U32) for w in (wq_hbm, wk_hbm, wv_hbm)]
        n_j = 3 * n_kc
        R = n_seg * P

        def cp_w(j, t=0):
            return pltpu.make_async_copy(srcs[t].at[pl.ds((j % n_kc) * KC, KC)],
                                         raw.at[pl.ds(j * CP, KC), pl.ds(0, H // 2)], sem_w.at[j])

        def cp_m(c, i):
            return pltpu.make_async_copy(wm_src.at[:, pl.ds(pl.multiple_of(i * D + c * KC, KC), KC)],
                                         wm_v.at[c, :, pl.ds(i * KC, KC)], sem_m.at[2 * c + i])

        def start(j):
            cp_m(j, 0).start()
            cp_m(j, 1).start()
            cp_w(j).start()

        def cp_o(i):
            r = pl.ds(pl.multiple_of(i * (HD // 16), HD // 16), HD // 16)
            return pltpu.make_async_copy(wo_src.at[r], wo32.at[r], sem_p.at[1 + i])

        def cp_r(i):
            r = pl.ds(pl.multiple_of(i * (D // 16), D // 16), D // 16)
            return pltpu.make_async_copy(wm_src.at[r, pl.ds(2 * D, 4 * D)], wr_v.at[r], sem_p.at[9 + i])

        cp_p = pltpu.make_async_copy(x_hbm.at[:, pl.ds(T - P, P), :], xp_v, sem_p.at[0])
        cp_p.start()
        start(0)

        cp_p.wait()

        def norm(i, carry):
            xn = _layernorm(xp_v[pl.ds(i * 8, 8)].astype(F32).reshape(8 * P, D))
            for c in range(n_kc):
                xn_v[c, pl.ds(pl.multiple_of(i * 8 * P, 8 * P), 8 * P), :] = xn[:, c * KC:(c + 1) * KC]
            return carry
        lax.fori_loop(0, n_seg // 8, norm, 0)
        start(1)
        raw2 = raw.reshape(n_j * CP * HP, Dh)

        def chunk(j, carry):
            t, c = j // n_kc, j % n_kc

            @pl.when(j < n_kc)
            def _():
                cp_m(c, 0).wait()
                cp_m(c, 1).wait()

                @pl.when(j + 2 < n_kc)
                def _():
                    start(j + 2)
                mod = _dot(silu_c(), pltpu.bitcast(wm_v[c], BF16))
                mod1_v[c] = mod
                h = xn_v[c] * (1.0 + mod[0:1, KC:]) + mod[0:1, :KC]
                for i, part in enumerate(_strassen_lhs(h, 1)):
                    hp_v[c, i] = pltpu.bitcast(part, U32)

            cp_w(j).wait()
            for src in (1, 2):
                @pl.when((j + 2) // n_kc == src)
                def _(src=src):
                    cp_w(j + 2, src).start()

            @pl.when(j >= n_j - 8)
            def _():
                cp_r(j - (n_j - 8)).start()
                cp_o(j - (n_j - 8)).start()

            @pl.when(j == n_j - 2)
            def _():
                cp_x.start()

            q4 = KC // 4
            for hp in range(H // 2):
                blk = []
                for half in range(2):
                    w = _unpack(raw2[pl.ds((j * CP + half * 2 * q4) * HP + hp, 2 * q4, stride=HP), :])
                    blk += [w[0], w[1]]
                tiles = [pltpu.bitcast(v.astype(BF16), U32) for v in blk]
                cols = [slice((2 * hp + i) * Dh, (2 * hp + i + 1) * Dh) for i in range(2)]
                for i, tile in enumerate(tiles):
                    wqkv[t, pl.ds(pl.multiple_of((2 * c + i // 2) * q4, q4), q4), cols[i % 2]] = tile
                part = _strassen_out([_dot(pltpu.bitcast(hp_v[c, i], BF16), w.astype(BF16))
                                      for i, w in enumerate(_strassen_rhs(blk))])
                pair = slice(2 * hp * Dh, (2 * hp + 2) * Dh)
                part = jnp.where(c > 0, acc_v[:, pair], 0.0) + part
                acc_v[:, pair] = part
                pre_v[t, :, :, pair] = part.reshape(n_seg, P, 2 * Dh).astype(BF16)
            return carry

        lax.fori_loop(0, n_j, chunk, 0)
        for c in range(n_kc):
            mod_v[:, c * KC:(c + 1) * KC] = mod1_v[c, :, :KC]
            mod_v[:, D + c * KC:D + (c + 1) * KC] = mod1_v[c, :, KC:]
        for i in range(8):
            cp_r(i).wait()
        mod_v[:, 2 * D:6 * D] = _dot(silu_c(), pltpu.bitcast(wr_v[...], BF16))
        for i in range(8):
            cp_o(i).wait()

    pl.run_scoped(startup,
                  pltpu.VMEM((n_kc, D // 2, 2 * KC), U32), pltpu.VMEM((D // 2, 4 * D), U32),
                  pltpu.VMEM((3 * n_kc * CP, HP, Dh), U32),
                  pltpu.VMEM((n_seg, P, D), x_hbm.dtype), pltpu.VMEM((n_kc, n_seg * P, KC), F32),
                  pltpu.VMEM((n_kc, 7, n_seg * P // 4, KC // 2), U32), pltpu.VMEM((n_seg * P, HD), F32),
                  pltpu.SemaphoreType.DMA((2 * n_kc,)), pltpu.SemaphoreType.DMA((3 * n_kc,)),
                  pltpu.SemaphoreType.DMA((17,)))

    ffn_cfg = ((w1_hbm, LV), (w3_hbm, LV), (w2_hbm, LV))

    def main(e1_v, e3_v, e2_v, h2_v, sem_f, sem_y):
        cp_f, pieces = [], []
        for (src, lv), e in zip(ffn_cfg, (e1_v, e3_v, e2_v)):
            R, n = e.shape[1] - 8, e.shape[2]
            for bi, bj, slot in _strassen_blocks(lv):
                cp_f.append(pltpu.make_async_copy(src.bitcast(U32).at[pl.ds(bi * R, R), pl.ds(bj * n, n)],
                                                  e.at[slot, pl.ds(0, R)], sem_f.at[len(cp_f)]))
                e[slot, R:R + 8, 0:128] = jnp.zeros((8, 128), U32)
            per_it = pl.cdiv(R // 8 * (n // 128), n_it - first_prep)
            groups = [range(7)] if lv == 1 else [range(7 * o, 7 * o + 7) for o in (0, 5, 6, 2, 3, 1, 4)]
            pieces += [(e, lv, per_it, u, grp) for u in range(per_it) for grp in groups]

        def prep_ffn(i, site, n_sites, anchor):
            per = pl.cdiv(len(pieces), n_sites)
            for k, (e, lv, per_it, u, grp) in enumerate(pieces[site * per:(site + 1) * per]):
                tie = after(anchor[:, (k * 128) % anchor.shape[1]:])
                n_r, n_c = e.shape[1] // 8 - 1, e.shape[2] // 128
                pos = jnp.maximum(i - first_prep, 0) * per_it + u
                live = (i >= first_prep) & (pos < n_r * n_c)
                rows = pl.ds(pl.multiple_of(jnp.where(live, lax.rem(pos, n_r), n_r) * 8, 8), 8)
                cols = pl.ds(pl.multiple_of(jnp.where(live, lax.div(pos, n_r), 0) * 128, 128), 128)
                blocks = [_unpack(e[slot, rows, cols] | tie) for _, _, slot in _strassen_blocks(lv)]
                for slot, w in enumerate(_strassen_rhs(blocks)):
                    if slot in grp and not any(w is blk for blk in blocks):
                        e[slot, rows, cols] = _pack(w)

        cp_x.wait()
        cp_x2.start()
        for cp in cp_f:
            cp.start()
        hs_v[...] = pltpu.bitcast(
            jnp.concatenate([mem0_ref[...].astype(F32), ada1(x_v[0])], axis=0).astype(BF16), U32)
        scale = Dh ** -0.5
        n_g = H // G

        def step(s, side):
            ri = lax.broadcasted_iota(jnp.int32, (2 * L, 2 * L), 0)
            ci = lax.broadcasted_iota(jnp.int32, (2 * L, 2 * L), 1)
            same = (ri >= L) == (ci >= L)
            rl = jnp.where(ri >= L, ri - L, ri)
            cl = jnp.where(ci >= L, ci - L, ci)
            keep = same & ((rl < M) | (rl >= cl))
            fill = jnp.where(same, -1e9 / scale, -jnp.inf).astype(F32)

            def gcols(g):
                return slice(g * G * Dh, (g + 1) * G * Dh)

            def proj(t, g):
                return _dot(pltpu.bitcast(hs_v[...], BF16), pltpu.bitcast(wqkv[t, :, gcols(g)], BF16))

            def stack(a, t, g, p):
                hp = g * G // 2 + p
                pre = pre_v[t, s, :, 2 * hp * Dh:(2 * hp + 2) * Dh].astype(F32)
                return jnp.concatenate([a[:, (2 * p) * Dh:(2 * p + 1) * Dh], pre[:, :Dh],
                                        a[:, (2 * p + 1) * Dh:(2 * p + 2) * Dh], pre[:, Dh:]], axis=0).astype(BF16)

            def scores(g, q, k):
                res = []
                for p in range(G // 2):
                    sc = jnp.where(keep, _dot(stack(q, 0, g, p), stack(k, 1, g, p), _NT), fill)
                    e = jnp.exp2((sc - jnp.max(sc, axis=-1, keepdims=True)) * (scale * _LOG2E))
                    den = jnp.sum(e, axis=-1, keepdims=True)
                    r = pl.reciprocal(den, approx=True)
                    res.append((e.astype(BF16), r * (2.0 - den * r)))
                return res

            def values(g, res, v):
                for p, (e, inv) in enumerate(res):
                    o = _dot(e, stack(v, 2, g, p)) * inv
                    h0 = g * G + 2 * p
                    o_v[:, h0 * Dh:(h0 + 1) * Dh] = o[0:L]
                    o_v[:, (h0 + 1) * Dh:(h0 + 2) * Dh] = o[L:2 * L]

            def outp(g):
                return _dot(o_v[:, gcols(g)],
                            pltpu.bitcast(wo32[g * G * Dh // 2:(g + 1) * G * Dh // 2, :], BF16))

            h_next = ada1(x_v[jnp.minimum(s + 1, n_seg - 1)])
            qk, sm, vv = {}, {}, {}
            for g in range(n_g):
                qk[g] = proj(0, g), proj(1, g)
                if g >= 1:
                    sm[g - 1] = scores(g - 1, *qk.pop(g - 1))
            for g in range(n_g):
                vv[g] = proj(2, g)
                side(g, vv[g])
                if g == 0:
                    sm[n_g - 1] = scores(n_g - 1, *qk.pop(n_g - 1))
                else:
                    values(g - 1, sm.pop(g - 1), vv.pop(g - 1))
            acc = outp(0)
            values(n_g - 1, sm.pop(n_g - 1), vv.pop(n_g - 1))
            for g in range(1, n_g):
                side(n_g - 1 + g, acc)
                acc = acc + outp(g)
            hs_v[...] = pltpu.bitcast(jnp.concatenate([acc[0:M], h_next], axis=0).astype(BF16), U32)
            x_v[s] = (x_v[s].astype(F32) + mod_v[0:1, 2 * D:3 * D] * acc[M:L]).astype(x_v.dtype)

        def steps(i, carry):
            for j in range(UN):
                per = 2 * n_g - 1
                step(i * UN + j, lambda k, anchor, j=j: prep_ffn(i, j * per + k, UN * per, anchor))
            return carry

        def phase(ph, carry):
            @pl.when(ph == 1)
            def _():
                cp_x2.wait()
                for cp in cp_f:
                    cp.wait()
            return lax.fori_loop(ph * first_prep, jnp.where(ph == 0, first_prep, n_it), steps, carry)

        lax.fori_loop(0, 2, phase, 0)

        def resid(i):
            return x_v[pl.ds(i * (BM // T), BM // T)].astype(F32).reshape(BM, D)

        def ada2(i):
            h2 = _layernorm(resid(i)) * (1.0 + mod_v[0:1, 4 * D:5 * D]) + mod_v[0:1, 3 * D:4 * D]
            return _strassen_lhs(h2, LV)

        def matmul(lhs, e, cols=slice(None)):
            return _strassen_out([_dot(a, pltpu.bitcast(e[k, 0:e.shape[1] - 8, cols], BF16))
                                  for k, a in enumerate(lhs)])

        def put_h2(parts):
            for j, part in enumerate(parts):
                h2_v[j] = part

        put_h2(ada2(0))

        def out_copy(i):
            r = pl.ds(i * (BM // T), BM // T)
            return pltpu.make_async_copy(x_v.at[r], out_hbm.at[r], sem_y.at[i])

        def ffn(i, carry):
            h2_next = ada2(jnp.minimum(i + 1, S // BM - 1))
            acts = []
            for c0 in range(0, e1_v.shape[2], FC):
                cols = slice(c0, c0 + FC)
                gate, up = [matmul([h2_v[j] for j in range(7 ** LV)], e, cols)
                            for e in (e1_v, e3_v)]
                act = _silu(gate) * up
                acts.append(_strassen_lhs(act, LV))
            put_h2(h2_next)
            ffn_out = matmul([jnp.concatenate(parts, axis=1) for parts in zip(*acts)], e2_v)
            y = resid(i) + mod_v[0:1, 5 * D:6 * D] * ffn_out
            x_v[pl.ds(i * (BM // T), BM // T)] = y.reshape(BM // T, T, D).astype(x_v.dtype)
            out_copy(i).start()
            return carry

        lax.fori_loop(0, S // BM, ffn, 0)
        for i in range(S // BM):
            out_copy(i).wait()

    pl.run_scoped(main,
                  *[pltpu.VMEM((7 ** lv, (w.shape[0] >> (lv + 1)) + 8, w.shape[1] >> lv), U32)
                    for w, lv in ffn_cfg],
                  pltpu.VMEM((7 ** LV, BM >> LV, D >> LV), BF16),
                  pltpu.SemaphoreType.DMA((sum(4 ** lv for _, lv in ffn_cfg),)),
                  pltpu.SemaphoreType.DMA((S // BM,)))


@functools.partial(jax.jit, static_argnames=("A_seg_len",))
def pallas_adaLN_cond__memory_aug_recurrent_mem_tr__glu_gated_swiglu__prompt_kernel(
    A_x, A_mem0, A_Wq, A_Wk, A_Wv, A_Wo, A_seg_len, B_x, B_w1, B_w3, B_w2, c, w_mod,
):
    del B_x
    B, S, D = A_x.shape
    _, H, Dh = A_Wq.shape
    M, T, F = A_mem0.shape[1], int(A_seg_len), B_w1.shape[1]
    assert B == 1 and S % T == 0
    L, HD = M + T, H * Dh
    hbm = pl.BlockSpec(memory_space=pl.ANY)
    vmem = pl.BlockSpec(memory_space=pltpu.VMEM)
    body = functools.partial(_body, S=S, D=D, H=H, Dh=Dh, M=M, T=T, F=F, G=8, BM=128, FC=128, LV=2)
    out = pl.pallas_call(
        body,
        out_shape=jax.ShapeDtypeStruct((S // T, T, D), A_x.dtype),
        in_specs=[hbm, vmem, hbm, hbm, hbm, hbm, hbm, hbm, hbm, vmem, hbm],
        out_specs=hbm,
        scratch_shapes=[
            pltpu.VMEM((3, D // 2, HD), U32), pltpu.VMEM((HD // 2, D), U32),
            pltpu.VMEM((3, S // T, 8, HD), BF16),
            pltpu.VMEM((S // T, T, D), A_x.dtype), pltpu.VMEM((8, 6 * D), F32),
            pltpu.VMEM((D // 256, 8, 512), F32),
            pltpu.VMEM(((L - 8) // 2, D), U32), pltpu.VMEM((L, HD), F32), pltpu.VMEM((8, 128), U32),
            pltpu.SemaphoreType.DMA((2,)),
        ],
        compiler_params=pltpu.CompilerParams(vmem_limit_bytes=126 * 2**20, flags={'XLA_TPU_EVENLY_DISTRIBUTE_CRITICAL_NODES': True}),
    )(A_x.reshape(S // T, T, D), A_mem0.reshape(M, D),
      A_Wq, A_Wk, A_Wv, A_Wo.reshape(HD, D),
      B_w1, B_w3, B_w2, c, w_mod)
    return out.reshape(B, S, D)
```

```python
import functools

import numpy as np
import jax
import jax.numpy as jnp
from jax import lax
import jax.experimental.pallas as pl
import jax.experimental.pallas.tpu as pltpu

F32, BF16, U32 = jnp.float32, jnp.bfloat16, jnp.uint32
_HIGH = np.uint32(0xFFFF0000)
_LOG2E = 1.4426950408889634
_NN = (((1,), (0,)), ((), ()))
_NT = (((1,), (1,)), ((), ()))


def _dot(a, b, dims=_NN):
    return lax.dot_general(a, b, dims, preferred_element_type=F32)


def _layernorm(x, eps=1e-5):
    m = jnp.mean(x, axis=-1, keepdims=True)
    d = x - m
    v = jnp.mean(d * d, axis=-1, keepdims=True)
    return d * lax.rsqrt(v + eps)


def _silu(x):
    h = 0.5 * x
    return h + h * jnp.tanh(h)


def _unpack(w):
    return jnp.stack([lax.bitcast_convert_type(v, F32) for v in (w << 16, w & _HIGH)])


def _pack(x, exact=False):
    lo, hi = (lax.bitcast_convert_type(v if exact else v.astype(BF16).astype(F32), U32) for v in (x[0], x[1]))
    return (lo >> 16) | hi


def _strassen_lhs(a, levels):
    if levels == 0:
        return [a.astype(BF16)]
    m, k = a.shape[0] // 2, a.shape[1] // 2
    a11, a12, a21, a22 = a[:m, :k], a[:m, k:], a[m:, :k], a[m:, k:]
    return [x for v in (a11 + a22, a21 + a22, a11, a22, a11 + a12, a21 - a11, a12 - a22)
            for x in _strassen_lhs(v, levels - 1)]


def _strassen_rhs(blocks):
    if len(blocks) == 1:
        return blocks
    n = len(blocks) // 4
    b11, b12, b21, b22 = (blocks[i * n:(i + 1) * n] for i in range(4))
    add = lambda x, y: [u + v for u, v in zip(x, y)]
    sub = lambda x, y: [u - v for u, v in zip(x, y)]
    return [x for v in (add(b11, b22), b11, sub(b12, b22), sub(b21, b11), b22, add(b11, b12), add(b21, b22))
            for x in _strassen_rhs(v)]


def _strassen_blocks(levels):
    out = [(0, 0, 0)]
    for _ in range(levels):
        out = [(2 * i + q // 2, 2 * j + q % 2, 7 * slot + 1 + q) for i, j, slot in out for q in range(4)]
    return out


def _strassen_out(m):
    if len(m) == 1:
        return m[0]
    n = len(m) // 7
    m1, m2, m3, m4, m5, m6, m7 = (_strassen_out(m[i * n:(i + 1) * n]) for i in range(7))
    return jnp.concatenate([jnp.concatenate([m1 + m4 - m5 + m7, m3 + m5], axis=1),
                            jnp.concatenate([m2 + m4, m1 - m2 + m3 + m6], axis=1)], axis=0)


def _body(x_hbm, mem0_hbm, wq_hbm, wk_hbm, wv_hbm, wo_hbm, w1_hbm, w3_hbm, w2_hbm,
          c_hbm, wm_hbm, out_hbm,
          wqkv, wo32, pre_v, x_v, mod_v, mod1_v, hs_v, o_v, zero_v, mem0_ref, c_ref, sems,
          *, S, D, H, Dh, M, T, F, G, BM, FC, LV):
    n_seg = S // T
    L = M + T
    HD = H * Dh
    UN = 2
    P = 8
    KC = 256
    n_kc = D // KC
    wo_src = wo_hbm.bitcast(U32)
    wm_src = wm_hbm.bitcast(U32)
    HP = H // 2 + 8
    CP = KC + 1
    n_it = n_seg // UN
    first_prep = n_it // 8
    XA = first_prep * UN + 1
    cp_x = pltpu.make_async_copy(x_hbm.at[pl.ds(0, XA)], x_v.at[pl.ds(0, XA)], sems.at[0])
    cp_x2 = pltpu.make_async_copy(x_hbm.at[pl.ds(XA, n_seg - XA)], x_v.at[pl.ds(XA, n_seg - XA)], sems.at[1])

    zero_v[...] = jnp.zeros(zero_v.shape, U32)

    def after(anchor):
        return pltpu.bitcast(anchor[0:8, 0:128], U32) & zero_v[...]

    def silu_c():
        return jnp.broadcast_to(_silu(c_ref[...].astype(F32)), (8, D)).astype(BF16)

    def ada1(x):
        return _layernorm(x.astype(F32)[:T - P]) * (1.0 + mod_v[0:1, D:2 * D]) + mod_v[0:1, 0:D]

    def startup(wm_v, wr_v, raw, xp_v, xn_v, hp_v, acc_v, sem_m, sem_w, sem_p):
        srcs = [w.bitcast(U32) for w in (wq_hbm, wk_hbm, wv_hbm)]
        n_j = 3 * n_kc
        R = n_seg * P

        def cp_w(j, t=0):
            return pltpu.make_async_copy(srcs[t].at[pl.ds((j % n_kc) * KC, KC)],
                                         raw.at[pl.ds(j * CP, KC), pl.ds(0, H // 2)], sem_w.at[j])

        def cp_m(c, i):
            return pltpu.make_async_copy(wm_src.at[:, pl.ds(pl.multiple_of(i * D + c * KC, KC), KC)],
                                         wm_v.at[c, :, pl.ds(i * KC, KC)], sem_m.at[2 * c + i])

        def start(j):
            cp_m(j, 0).start()
            cp_m(j, 1).start()
            cp_w(j).start()

        cp_r = pltpu.make_async_copy(wm_src.at[:, pl.ds(2 * D, 4 * D)], wr_v, sem_p.at[1])
        cp_o = pltpu.make_async_copy(wo_src, wo32, sem_p.at[2])
        cp_p = pltpu.make_async_copy(x_hbm.at[:, pl.ds(T - P, P), :], xp_v, sem_p.at[0])
        small = [pltpu.make_async_copy(c_hbm, c_ref, sems.at[2]),
                 pltpu.make_async_copy(mem0_hbm, mem0_ref, sems.at[3])]
        cp_p.start()
        for cp in small:
            cp.start()
        start(0)
        cp_p.wait()
        for cp in small:
            cp.wait()

        def norm(i, carry):
            xn = _layernorm(xp_v[pl.ds(i * 8, 8)].astype(F32).reshape(8 * P, D))
            for c in range(n_kc):
                xn_v[c, pl.ds(pl.multiple_of(i * 8 * P, 8 * P), 8 * P), :] = xn[:, c * KC:(c + 1) * KC]
            return carry
        lax.fori_loop(0, n_seg // 8, norm, 0)
        for j in range(1, n_j):
            if j < n_kc:
                start(j)
            else:
                cp_w(j, j // n_kc).start()
        for cp in (cp_r, cp_o, cp_x):
            cp.start()
        raw2 = raw.reshape(n_j * CP * HP, Dh)

        def chunk(j, carry):
            t, c = j // n_kc, j % n_kc

            @pl.when(j < n_kc)
            def _():
                cp_m(c, 0).wait()
                cp_m(c, 1).wait()
                mod = _dot(silu_c(), pltpu.bitcast(wm_v[c], BF16))
                mod1_v[c] = mod
                h = xn_v[c] * (1.0 + mod[0:1, KC:]) + mod[0:1, :KC]
                for i, part in enumerate(_strassen_lhs(h, 1)):
                    hp_v[c, i] = pltpu.bitcast(part, U32)

            cp_w(j).wait()

            q4 = KC // 4
            for hp in range(H // 2):
                blk = []
                for half in range(2):
                    w = _unpack(raw2[pl.ds((j * CP + half * 2 * q4) * HP + hp, 2 * q4, stride=HP), :])
                    blk += [w[0], w[1]]
                tiles = [pltpu.bitcast(v.astype(BF16), U32) for v in blk]
                cols = [slice((2 * hp + i) * Dh, (2 * hp + i + 1) * Dh) for i in range(2)]
                for i, tile in enumerate(tiles):
                    wqkv[t, pl.ds(pl.multiple_of((2 * c + i // 2) * q4, q4), q4), cols[i % 2]] = tile
                part = _strassen_out([_dot(pltpu.bitcast(hp_v[c, i], BF16), w.astype(BF16))
                                      for i, w in enumerate(_strassen_rhs(blk))])
                pair = slice(2 * hp * Dh, (2 * hp + 2) * Dh)
                part = jnp.where(c > 0, acc_v[:, pair], 0.0) + part
                acc_v[:, pair] = part
                pre_v[t, :, :, pair] = part.reshape(n_seg, P, 2 * Dh).astype(BF16)
            return carry

        lax.fori_loop(0, n_j, chunk, 0)
        for c in range(n_kc):
            mod_v[:, c * KC:(c + 1) * KC] = mod1_v[c, :, :KC]
            mod_v[:, D + c * KC:D + (c + 1) * KC] = mod1_v[c, :, KC:]
        cp_r.wait()
        mod_v[:, 2 * D:6 * D] = _dot(silu_c(), pltpu.bitcast(wr_v[...], BF16))
        cp_o.wait()

    pl.run_scoped(startup,
                  pltpu.VMEM((n_kc, D // 2, 2 * KC), U32), pltpu.VMEM((D // 2, 4 * D), U32),
                  pltpu.VMEM((3 * n_kc * CP, HP, Dh), U32),
                  pltpu.VMEM((n_seg, P, D), x_hbm.dtype), pltpu.VMEM((n_kc, n_seg * P, KC), F32),
                  pltpu.VMEM((n_kc, 7, n_seg * P // 4, KC // 2), U32), pltpu.VMEM((n_seg * P, HD), F32),
                  pltpu.SemaphoreType.DMA((2 * n_kc,)), pltpu.SemaphoreType.DMA((3 * n_kc,)),
                  pltpu.SemaphoreType.DMA((3,)))

    ffn_cfg = ((w1_hbm, LV), (w3_hbm, LV), (w2_hbm, LV))

    def main(e1_v, e3_v, e2_v, h2_v, sem_f, sem_y):
        cp_f, pieces = [], []
        for (src, lv), e in zip(ffn_cfg, (e1_v, e3_v, e2_v)):
            R, n = e.shape[1] - 8, e.shape[2]
            for bi, bj, slot in _strassen_blocks(lv):
                cp_f.append(pltpu.make_async_copy(src.bitcast(U32).at[pl.ds(bi * R, R), pl.ds(bj * n, n)],
                                                  e.at[slot, pl.ds(0, R)], sem_f.at[len(cp_f)]))
                e[slot, R:R + 8, 0:128] = jnp.zeros((8, 128), U32)
            per_it = pl.cdiv(R // 8 * (n // 128), n_it - first_prep)
            groups = [range(7)] if lv == 1 else [range(7 * o, 7 * o + 7) for o in (0, 5, 6, 2, 3, 1, 4)]
            pieces += [(e, lv, per_it, u, grp) for u in range(per_it) for grp in groups]

        def prep_ffn(i, site, n_sites, anchor):
            per = pl.cdiv(len(pieces), n_sites)
            for k, (e, lv, per_it, u, grp) in enumerate(pieces[site * per:(site + 1) * per]):
                tie = after(anchor[:, (k * 128) % anchor.shape[1]:])
                n_r, n_c = e.shape[1] // 8 - 1, e.shape[2] // 128
                pos = jnp.maximum(i - first_prep, 0) * per_it + u
                live = (i >= first_prep) & (pos < n_r * n_c)
                rows = pl.ds(pl.multiple_of(jnp.where(live, lax.rem(pos, n_r), n_r) * 8, 8), 8)
                cols = pl.ds(pl.multiple_of(jnp.where(live, lax.div(pos, n_r), 0) * 128, 128), 128)
                blocks = [_unpack(e[slot, rows, cols] | tie) for _, _, slot in _strassen_blocks(lv)]
                for slot, w in enumerate(_strassen_rhs(blocks)):
                    if slot in grp and not any(w is blk for blk in blocks):
                        e[slot, rows, cols] = _pack(w)

        cp_x.wait()
        cp_x2.start()
        for cp in cp_f:
            cp.start()
        hs_v[...] = pltpu.bitcast(
            jnp.concatenate([mem0_ref[...].astype(F32), ada1(x_v[0])], axis=0).astype(BF16), U32)
        scale = Dh ** -0.5
        n_g = H // G

        def step(s, side):
            ri = lax.broadcasted_iota(jnp.int32, (2 * L, 2 * L), 0)
            ci = lax.broadcasted_iota(jnp.int32, (2 * L, 2 * L), 1)
            same = (ri >= L) == (ci >= L)
            rl = jnp.where(ri >= L, ri - L, ri)
            cl = jnp.where(ci >= L, ci - L, ci)
            keep = same & ((rl < M) | (rl >= cl))
            fill = jnp.where(same, -1e9 / scale, -jnp.inf).astype(F32)

            def gcols(g):
                return slice(g * G * Dh, (g + 1) * G * Dh)

            def proj(t, g):
                return _dot(pltpu.bitcast(hs_v[...], BF16), pltpu.bitcast(wqkv[t, :, gcols(g)], BF16))

            def stack(a, t, g, p):
                hp = g * G // 2 + p
                pre = pre_v[t, s, :, 2 * hp * Dh:(2 * hp + 2) * Dh].astype(F32)
                return jnp.concatenate([a[:, (2 * p) * Dh:(2 * p + 1) * Dh], pre[:, :Dh],
                                        a[:, (2 * p + 1) * Dh:(2 * p + 2) * Dh], pre[:, Dh:]], axis=0).astype(BF16)

            def scores(g, q, k):
                res = []
                for p in range(G // 2):
                    sc = jnp.where(keep, _dot(stack(q, 0, g, p), stack(k, 1, g, p), _NT), fill)
                    e = jnp.exp2((sc - jnp.max(sc, axis=-1, keepdims=True)) * (scale * _LOG2E))
                    den = jnp.sum(e, axis=-1, keepdims=True)
                    r = pl.reciprocal(den, approx=True)
                    res.append((e.astype(BF16), r * (2.0 - den * r)))
                return res

            def values(g, res, v):
                for p, (e, inv) in enumerate(res):
                    o = _dot(e, stack(v, 2, g, p)) * inv
                    h0 = g * G + 2 * p
                    o_v[:, h0 * Dh:(h0 + 1) * Dh] = o[0:L]
                    o_v[:, (h0 + 1) * Dh:(h0 + 2) * Dh] = o[L:2 * L]

            def outp(g):
                return _dot(o_v[:, gcols(g)],
                            pltpu.bitcast(wo32[g * G * Dh // 2:(g + 1) * G * Dh // 2, :], BF16))

            h_next = ada1(x_v[jnp.minimum(s + 1, n_seg - 1)])
            qk, sm, vv = {}, {}, {}
            for g in range(n_g):
                qk[g] = proj(0, g), proj(1, g)
                if g >= 1:
                    sm[g - 1] = scores(g - 1, *qk.pop(g - 1))
            for g in range(n_g):
                vv[g] = proj(2, g)
                side(g, vv[g])
                if g == 0:
                    sm[n_g - 1] = scores(n_g - 1, *qk.pop(n_g - 1))
                else:
                    values(g - 1, sm.pop(g - 1), vv.pop(g - 1))
            acc = outp(0)
            values(n_g - 1, sm.pop(n_g - 1), vv.pop(n_g - 1))
            for g in range(1, n_g):
                side(n_g - 1 + g, acc)
                acc = acc + outp(g)
            hs_v[...] = pltpu.bitcast(jnp.concatenate([acc[0:M], h_next], axis=0).astype(BF16), U32)
            x_v[s] = (x_v[s].astype(F32) + mod_v[0:1, 2 * D:3 * D] * acc[M:L]).astype(x_v.dtype)

        def steps(i, carry):
            for j in range(UN):
                per = 2 * n_g - 1
                step(i * UN + j, lambda k, anchor, j=j: prep_ffn(i, j * per + k, UN * per, anchor))
            return carry

        def phase(ph, carry):
            @pl.when(ph == 1)
            def _():
                cp_x2.wait()
                for cp in cp_f:
                    cp.wait()
            return lax.fori_loop(ph * first_prep, jnp.where(ph == 0, first_prep, n_it), steps, carry)

        lax.fori_loop(0, 2, phase, 0)

        def resid(i):
            return x_v[pl.ds(i * (BM // T), BM // T)].astype(F32).reshape(BM, D)

        def ada2(i):
            h2 = _layernorm(resid(i)) * (1.0 + mod_v[0:1, 4 * D:5 * D]) + mod_v[0:1, 3 * D:4 * D]
            return _strassen_lhs(h2, LV)

        def matmul(lhs, e, cols=slice(None)):
            return _strassen_out([_dot(a, pltpu.bitcast(e[k, 0:e.shape[1] - 8, cols], BF16))
                                  for k, a in enumerate(lhs)])

        def put_h2(parts):
            for j, part in enumerate(parts):
                h2_v[j] = part

        put_h2(ada2(0))

        def out_copy(i):
            r = pl.ds(i * (BM // T), BM // T)
            return pltpu.make_async_copy(x_v.at[r], out_hbm.at[r], sem_y.at[i])

        def ffn(i, carry):
            h2_next = ada2(jnp.minimum(i + 1, S // BM - 1))
            acts = []
            for c0 in range(0, e1_v.shape[2], FC):
                cols = slice(c0, c0 + FC)
                gate, up = [matmul([h2_v[j] for j in range(7 ** LV)], e, cols)
                            for e in (e1_v, e3_v)]
                act = _silu(gate) * up
                acts.append(_strassen_lhs(act, LV))
            put_h2(h2_next)
            ffn_out = matmul([jnp.concatenate(parts, axis=1) for parts in zip(*acts)], e2_v)
            y = resid(i) + mod_v[0:1, 5 * D:6 * D] * ffn_out
            x_v[pl.ds(i * (BM // T), BM // T)] = y.reshape(BM // T, T, D).astype(x_v.dtype)
            out_copy(i).start()
            return carry

        lax.fori_loop(0, S // BM, ffn, 0)
        for i in range(S // BM):
            out_copy(i).wait()

    pl.run_scoped(main,
                  *[pltpu.VMEM((7 ** lv, (w.shape[0] >> (lv + 1)) + 8, w.shape[1] >> lv), U32)
                    for w, lv in ffn_cfg],
                  pltpu.VMEM((7 ** LV, BM >> LV, D >> LV), BF16),
                  pltpu.SemaphoreType.DMA((sum(4 ** lv for _, lv in ffn_cfg),)),
                  pltpu.SemaphoreType.DMA((S // BM,)))


@functools.partial(jax.jit, static_argnames=("A_seg_len",))
def pallas_adaLN_cond__memory_aug_recurrent_mem_tr__glu_gated_swiglu__prompt_kernel(
    A_x, A_mem0, A_Wq, A_Wk, A_Wv, A_Wo, A_seg_len, B_x, B_w1, B_w3, B_w2, c, w_mod,
):
    del B_x
    B, S, D = A_x.shape
    _, H, Dh = A_Wq.shape
    M, T, F = A_mem0.shape[1], int(A_seg_len), B_w1.shape[1]
    assert B == 1 and S % T == 0
    L, HD = M + T, H * Dh
    hbm = pl.BlockSpec(memory_space=pl.ANY)
    body = functools.partial(_body, S=S, D=D, H=H, Dh=Dh, M=M, T=T, F=F, G=8, BM=128, FC=128, LV=2)
    out = pl.pallas_call(
        body,
        out_shape=jax.ShapeDtypeStruct((S // T, T, D), A_x.dtype),
        in_specs=[hbm] * 11,
        out_specs=hbm,
        scratch_shapes=[
            pltpu.VMEM((3, D // 2, HD), U32), pltpu.VMEM((HD // 2, D), U32),
            pltpu.VMEM((3, S // T, 8, HD), BF16),
            pltpu.VMEM((S // T, T, D), A_x.dtype), pltpu.VMEM((8, 6 * D), F32),
            pltpu.VMEM((D // 256, 8, 512), F32),
            pltpu.VMEM(((L - 8) // 2, D), U32), pltpu.VMEM((L, HD), F32), pltpu.VMEM((8, 128), U32),
            pltpu.VMEM((M, D), A_mem0.dtype), pltpu.VMEM(c.shape, c.dtype),
            pltpu.SemaphoreType.DMA((4,)),
        ],
        compiler_params=pltpu.CompilerParams(vmem_limit_bytes=126 * 2**20, flags={'XLA_TPU_EVENLY_DISTRIBUTE_CRITICAL_NODES': True}),
    )(A_x.reshape(S // T, T, D), A_mem0.reshape(M, D),
      A_Wq, A_Wk, A_Wv, A_Wo.reshape(HD, D),
      B_w1, B_w3, B_w2, c, w_mod)
    return out.reshape(B, S, D)
```

```python
import functools

import numpy as np
import jax
import jax.numpy as jnp
from jax import lax
import jax.experimental.pallas as pl
import jax.experimental.pallas.tpu as pltpu

F32, BF16, U32 = jnp.float32, jnp.bfloat16, jnp.uint32
_EARLY, _CHUNK = 8, 256
_HIGH = np.uint32(0xFFFF0000)
_LOG2E = 1.4426950408889634
_NN = (((1,), (0,)), ((), ()))
_NT = (((1,), (1,)), ((), ()))


def _dot(a, b, dims=_NN):
    return lax.dot_general(a, b, dims, preferred_element_type=F32)


def _layernorm(x, eps=1e-5):
    m = jnp.mean(x, axis=-1, keepdims=True)
    d = x - m
    v = jnp.mean(d * d, axis=-1, keepdims=True)
    return d * lax.rsqrt(v + eps)


def _silu(x):
    h = 0.5 * x
    return h + h * jnp.tanh(h)


def _unpack(w):
    return jnp.stack([lax.bitcast_convert_type(v, F32) for v in (w << 16, w & _HIGH)])


def _pack(x):
    lo, hi = (lax.bitcast_convert_type(v.astype(BF16).astype(F32), U32) for v in (x[0], x[1]))
    return (lo >> 16) | hi


def _strassen_lhs(a, levels):
    if levels == 0:
        return [a.astype(BF16)]
    m, k = a.shape[0] // 2, a.shape[1] // 2
    a11, a12, a21, a22 = a[:m, :k], a[:m, k:], a[m:, :k], a[m:, k:]
    return [x for v in (a11 + a22, a21 + a22, a11, a22, a11 + a12, a21 - a11, a12 - a22)
            for x in _strassen_lhs(v, levels - 1)]


def _strassen_rhs(blocks):
    if len(blocks) == 1:
        return blocks
    n = len(blocks) // 4
    b11, b12, b21, b22 = (blocks[i * n:(i + 1) * n] for i in range(4))
    add = lambda x, y: [u + v for u, v in zip(x, y)]
    sub = lambda x, y: [u - v for u, v in zip(x, y)]
    return [x for v in (add(b11, b22), b11, sub(b12, b22), sub(b21, b11), b22, add(b11, b12), add(b21, b22))
            for x in _strassen_rhs(v)]


def _strassen_blocks(levels):
    out = [(0, 0, 0)]
    for _ in range(levels):
        out = [(2 * i + q // 2, 2 * j + q % 2, 7 * slot + 1 + q) for i, j, slot in out for q in range(4)]
    return out


def _strassen_out(m):
    if len(m) == 1:
        return m[0]
    n = len(m) // 7
    m1, m2, m3, m4, m5, m6, m7 = (_strassen_out(m[i * n:(i + 1) * n]) for i in range(7))
    return jnp.concatenate([jnp.concatenate([m1 + m4 - m5 + m7, m3 + m5], axis=1),
                            jnp.concatenate([m2 + m4, m1 - m2 + m3 + m6], axis=1)], axis=0)


def _body(x_hbm, mem0_hbm, wq_hbm, wk_hbm, wv_hbm, wo_hbm, w1_hbm, w3_hbm, w2_hbm,
          c_hbm, wm_hbm, out_hbm,
          wqkv, wo32, pre_v, x_v, mod_v, mod1_v, hs_v, o_v, zero_v, mem0_ref, c_ref, sems,
          *, S, D, H, Dh, M, T, F, G, BM, FC, LV):
    n_seg = S // T
    L = M + T
    HD = H * Dh
    UN = 2
    P = _EARLY
    KC = _CHUNK
    n_kc = D // KC
    wo_src = wo_hbm.bitcast(U32)
    wm_src = wm_hbm.bitcast(U32)
    HP = H // 2 + 8
    CP = KC + 1
    n_it = n_seg // UN
    first_prep = n_it // 8
    XA = first_prep * UN + 1
    cp_x = pltpu.make_async_copy(x_hbm.at[pl.ds(0, XA)], x_v.at[pl.ds(0, XA)], sems.at[0])
    cp_x2 = pltpu.make_async_copy(x_hbm.at[pl.ds(XA, n_seg - XA)], x_v.at[pl.ds(XA, n_seg - XA)], sems.at[1])

    zero_v[...] = jnp.zeros(zero_v.shape, U32)

    def after(anchor):
        return pltpu.bitcast(anchor[0:8, 0:128], U32) & zero_v[...]

    def silu_c():
        return jnp.broadcast_to(_silu(c_ref[...].astype(F32)), (8, D)).astype(BF16)

    def ada1(x):
        return _layernorm(x.astype(F32)[:T - P]) * (1.0 + mod_v[0:1, D:2 * D]) + mod_v[0:1, 0:D]

    def startup(wm_v, wr_v, raw, xp_v, xn_v, hp_v, acc_v, sem_m, sem_w, sem_p):
        srcs = [w.bitcast(U32) for w in (wq_hbm, wk_hbm, wv_hbm)]
        n_j = 3 * n_kc

        def cp_w(j, t=0):
            return pltpu.make_async_copy(srcs[t].at[pl.ds((j % n_kc) * KC, KC)],
                                         raw.at[pl.ds(j * CP, KC), pl.ds(0, H // 2)], sem_w.at[j])

        def cp_m(c, i):
            return pltpu.make_async_copy(wm_src.at[:, pl.ds(pl.multiple_of(i * D + c * KC, KC), KC)],
                                         wm_v.at[c, :, pl.ds(i * KC, KC)], sem_m.at[2 * c + i])

        def start(j):
            cp_m(j, 0).start()
            cp_m(j, 1).start()
            cp_w(j).start()

        cp_r = pltpu.make_async_copy(wm_src.at[:, pl.ds(2 * D, 4 * D)], wr_v, sem_p.at[1])
        cp_o = pltpu.make_async_copy(wo_src, wo32, sem_p.at[2])
        cp_p = pltpu.make_async_copy(x_hbm.at[:, pl.ds(T - P, P), :], xp_v, sem_p.at[0])
        small = [pltpu.make_async_copy(c_hbm, c_ref, sems.at[2]),
                 pltpu.make_async_copy(mem0_hbm, mem0_ref, sems.at[3])]
        cp_p.start()
        for cp in small:
            cp.start()
        start(0)
        cp_p.wait()
        for cp in small:
            cp.wait()

        def norm(i, carry):
            xn = _layernorm(xp_v[pl.ds(i * 8, 8)].astype(F32).reshape(8 * P, D))
            for c in range(n_kc):
                xn_v[c, pl.ds(pl.multiple_of(i * 8 * P, 8 * P), 8 * P), :] = xn[:, c * KC:(c + 1) * KC]
            return carry
        lax.fori_loop(0, n_seg // 8, norm, 0)
        for j in range(1, n_j):
            if j < n_kc:
                start(j)
            else:
                cp_w(j, j // n_kc).start()
        for cp in (cp_r, cp_o, cp_x):
            cp.start()
        raw2 = raw.reshape(n_j * CP * HP, Dh)

        def chunk(j, carry):
            t, c = j // n_kc, j % n_kc

            @pl.when(j < n_kc)
            def _():
                cp_m(c, 0).wait()
                cp_m(c, 1).wait()
                mod = _dot(silu_c(), pltpu.bitcast(wm_v[c], BF16))
                mod1_v[c] = mod
                h = xn_v[c] * (1.0 + mod[0:1, KC:]) + mod[0:1, :KC]
                for i, part in enumerate(_strassen_lhs(h, 1)):
                    hp_v[c, i] = pltpu.bitcast(part, U32)

            cp_w(j).wait()

            q4 = KC // 4
            for hp in range(H // 2):
                blk = []
                for half in range(2):
                    w = _unpack(raw2[pl.ds((j * CP + half * 2 * q4) * HP + hp, 2 * q4, stride=HP), :])
                    blk += [w[0], w[1]]
                tiles = [pltpu.bitcast(v.astype(BF16), U32) for v in blk]
                cols = [slice((2 * hp + i) * Dh, (2 * hp + i + 1) * Dh) for i in range(2)]
                for i, tile in enumerate(tiles):
                    wqkv[t, pl.ds(pl.multiple_of((2 * c + i // 2) * q4, q4), q4), cols[i % 2]] = tile
                part = _strassen_out([_dot(pltpu.bitcast(hp_v[c, i], BF16), w.astype(BF16))
                                      for i, w in enumerate(_strassen_rhs(blk))])
                pair = slice(2 * hp * Dh, (2 * hp + 2) * Dh)
                part = jnp.where(c > 0, acc_v[:, pair], 0.0) + part
                acc_v[:, pair] = part
                pre_v[t, :, :, pair] = part.reshape(n_seg, P, 2 * Dh).astype(BF16)
            return carry

        lax.fori_loop(0, n_j, chunk, 0)
        for c in range(n_kc):
            mod_v[:, c * KC:(c + 1) * KC] = mod1_v[c, :, :KC]
            mod_v[:, D + c * KC:D + (c + 1) * KC] = mod1_v[c, :, KC:]
        cp_r.wait()
        mod_v[:, 2 * D:6 * D] = _dot(silu_c(), pltpu.bitcast(wr_v[...], BF16))
        cp_o.wait()

    pl.run_scoped(startup,
                  pltpu.VMEM((n_kc, D // 2, 2 * KC), U32), pltpu.VMEM((D // 2, 4 * D), U32),
                  pltpu.VMEM((3 * n_kc * CP, HP, Dh), U32),
                  pltpu.VMEM((n_seg, P, D), x_hbm.dtype), pltpu.VMEM((n_kc, n_seg * P, KC), F32),
                  pltpu.VMEM((n_kc, 7, n_seg * P // 4, KC // 2), U32), pltpu.VMEM((n_seg * P, HD), F32),
                  pltpu.SemaphoreType.DMA((2 * n_kc,)), pltpu.SemaphoreType.DMA((3 * n_kc,)),
                  pltpu.SemaphoreType.DMA((3,)))

    ffn_cfg = ((w1_hbm, LV), (w3_hbm, LV), (w2_hbm, LV))

    def main(e1_v, e3_v, e2_v, h2_v, sem_f, sem_y):
        cp_f, pieces = [], []
        for (src, lv), e in zip(ffn_cfg, (e1_v, e3_v, e2_v)):
            R, n = e.shape[1] - 8, e.shape[2]
            for bi, bj, slot in _strassen_blocks(lv):
                cp_f.append(pltpu.make_async_copy(src.bitcast(U32).at[pl.ds(bi * R, R), pl.ds(bj * n, n)],
                                                  e.at[slot, pl.ds(0, R)], sem_f.at[len(cp_f)]))
                e[slot, R:R + 8, 0:128] = jnp.zeros((8, 128), U32)
            per_it = pl.cdiv(R // 8 * (n // 128), n_it - first_prep)
            groups = [range(7)] if lv == 1 else [range(7 * o, 7 * o + 7) for o in (0, 5, 6, 2, 3, 1, 4)]
            pieces += [(e, lv, per_it, u, grp) for u in range(per_it) for grp in groups]

        def prep_ffn(i, site, n_sites, anchor):
            per = pl.cdiv(len(pieces), n_sites)
            for k, (e, lv, per_it, u, grp) in enumerate(pieces[site * per:(site + 1) * per]):
                tie = after(anchor[:, (k * 128) % anchor.shape[1]:])
                n_r, n_c = e.shape[1] // 8 - 1, e.shape[2] // 128
                pos = jnp.maximum(i - first_prep, 0) * per_it + u
                live = (i >= first_prep) & (pos < n_r * n_c)
                rows = pl.ds(pl.multiple_of(jnp.where(live, lax.rem(pos, n_r), n_r) * 8, 8), 8)
                cols = pl.ds(pl.multiple_of(jnp.where(live, lax.div(pos, n_r), 0) * 128, 128), 128)
                blocks = [_unpack(e[slot, rows, cols] | tie) for _, _, slot in _strassen_blocks(lv)]
                for slot, w in enumerate(_strassen_rhs(blocks)):
                    if slot in grp and not any(w is blk for blk in blocks):
                        e[slot, rows, cols] = _pack(w)

        cp_x.wait()
        cp_x2.start()
        for cp in cp_f:
            cp.start()
        hs_v[...] = pltpu.bitcast(
            jnp.concatenate([mem0_ref[...].astype(F32), ada1(x_v[0])], axis=0).astype(BF16), U32)
        scale = Dh ** -0.5
        n_g = H // G

        def step(s, side):
            ri = lax.broadcasted_iota(jnp.int32, (2 * L, 2 * L), 0)
            ci = lax.broadcasted_iota(jnp.int32, (2 * L, 2 * L), 1)
            same = (ri >= L) == (ci >= L)
            rl = jnp.where(ri >= L, ri - L, ri)
            cl = jnp.where(ci >= L, ci - L, ci)
            keep = same & ((rl < M) | (rl >= cl))
            fill = jnp.where(same, -1e9 / scale, -jnp.inf).astype(F32)

            def gcols(g):
                return slice(g * G * Dh, (g + 1) * G * Dh)

            def proj(t, g):
                return _dot(pltpu.bitcast(hs_v[...], BF16), pltpu.bitcast(wqkv[t, :, gcols(g)], BF16))

            def stack(a, t, g, p):
                hp = g * G // 2 + p
                pre = pre_v[t, s, :, 2 * hp * Dh:(2 * hp + 2) * Dh].astype(F32)
                return jnp.concatenate([a[:, (2 * p) * Dh:(2 * p + 1) * Dh], pre[:, :Dh],
                                        a[:, (2 * p + 1) * Dh:(2 * p + 2) * Dh], pre[:, Dh:]], axis=0).astype(BF16)

            def scores(g, q, k):
                res = []
                for p in range(G // 2):
                    sc = jnp.where(keep, _dot(stack(q, 0, g, p), stack(k, 1, g, p), _NT), fill)
                    e = jnp.exp2((sc - jnp.max(sc, axis=-1, keepdims=True)) * (scale * _LOG2E))
                    den = jnp.sum(e, axis=-1, keepdims=True)
                    r = pl.reciprocal(den, approx=True)
                    res.append((e.astype(BF16), r * (2.0 - den * r)))
                return res

            def values(g, res, v):
                for p, (e, inv) in enumerate(res):
                    o = _dot(e, stack(v, 2, g, p)) * inv
                    h0 = g * G + 2 * p
                    o_v[:, h0 * Dh:(h0 + 1) * Dh] = o[0:L]
                    o_v[:, (h0 + 1) * Dh:(h0 + 2) * Dh] = o[L:2 * L]

            def outp(g):
                return _dot(o_v[:, gcols(g)],
                            pltpu.bitcast(wo32[g * G * Dh // 2:(g + 1) * G * Dh // 2, :], BF16))

            h_next = ada1(x_v[jnp.minimum(s + 1, n_seg - 1)])
            qk, sm, vv = {}, {}, {}
            for g in range(n_g):
                qk[g] = proj(0, g), proj(1, g)
                if g >= 1:
                    sm[g - 1] = scores(g - 1, *qk.pop(g - 1))
            for g in range(n_g):
                vv[g] = proj(2, g)
                side(g, vv[g])
                if g == 0:
                    sm[n_g - 1] = scores(n_g - 1, *qk.pop(n_g - 1))
                else:
                    values(g - 1, sm.pop(g - 1), vv.pop(g - 1))
            acc = outp(0)
            values(n_g - 1, sm.pop(n_g - 1), vv.pop(n_g - 1))
            for g in range(1, n_g):
                side(n_g - 1 + g, acc)
                acc = acc + outp(g)
            hs_v[...] = pltpu.bitcast(jnp.concatenate([acc[0:M], h_next], axis=0).astype(BF16), U32)
            x_v[s] = (x_v[s].astype(F32) + mod_v[0:1, 2 * D:3 * D] * acc[M:L]).astype(x_v.dtype)

        def steps(i, carry):
            for j in range(UN):
                per = 2 * n_g - 1
                step(i * UN + j, lambda k, anchor, j=j: prep_ffn(i, j * per + k, UN * per, anchor))
            return carry

        def phase(ph, carry):
            @pl.when(ph == 1)
            def _():
                cp_x2.wait()
                for cp in cp_f:
                    cp.wait()
            return lax.fori_loop(ph * first_prep, jnp.where(ph == 0, first_prep, n_it), steps, carry)

        lax.fori_loop(0, 2, phase, 0)

        def resid(i):
            return x_v[pl.ds(i * (BM // T), BM // T)].astype(F32).reshape(BM, D)

        def ada2(i):
            h2 = _layernorm(resid(i)) * (1.0 + mod_v[0:1, 4 * D:5 * D]) + mod_v[0:1, 3 * D:4 * D]
            return _strassen_lhs(h2, LV)

        def matmul(lhs, e, cols=slice(None)):
            return _strassen_out([_dot(a, pltpu.bitcast(e[k, 0:e.shape[1] - 8, cols], BF16))
                                  for k, a in enumerate(lhs)])

        def put_h2(parts):
            for j, part in enumerate(parts):
                h2_v[j] = part

        put_h2(ada2(0))

        def out_copy(i):
            r = pl.ds(i * (BM // T), BM // T)
            return pltpu.make_async_copy(x_v.at[r], out_hbm.at[r], sem_y.at[i])

        def ffn(i, carry):
            h2_next = ada2(jnp.minimum(i + 1, S // BM - 1))
            acts = []
            for c0 in range(0, e1_v.shape[2], FC):
                cols = slice(c0, c0 + FC)
                gate, up = [matmul([h2_v[j] for j in range(7 ** LV)], e, cols)
                            for e in (e1_v, e3_v)]
                act = _silu(gate) * up
                acts.append(_strassen_lhs(act, LV))
            put_h2(h2_next)
            ffn_out = matmul([jnp.concatenate(parts, axis=1) for parts in zip(*acts)], e2_v)
            y = resid(i) + mod_v[0:1, 5 * D:6 * D] * ffn_out
            x_v[pl.ds(i * (BM // T), BM // T)] = y.reshape(BM // T, T, D).astype(x_v.dtype)
            out_copy(i).start()
            return carry

        lax.fori_loop(0, S // BM, ffn, 0)
        for i in range(S // BM):
            out_copy(i).wait()

    pl.run_scoped(main,
                  *[pltpu.VMEM((7 ** lv, (w.shape[0] >> (lv + 1)) + 8, w.shape[1] >> lv), U32)
                    for w, lv in ffn_cfg],
                  pltpu.VMEM((7 ** LV, BM >> LV, D >> LV), BF16),
                  pltpu.SemaphoreType.DMA((sum(4 ** lv for _, lv in ffn_cfg),)),
                  pltpu.SemaphoreType.DMA((S // BM,)))


@functools.partial(jax.jit, static_argnames=("A_seg_len",))
def pallas_adaLN_cond__memory_aug_recurrent_mem_tr__glu_gated_swiglu__prompt_kernel(
    A_x, A_mem0, A_Wq, A_Wk, A_Wv, A_Wo, A_seg_len, B_x, B_w1, B_w3, B_w2, c, w_mod,
):
    del B_x
    B, S, D = A_x.shape
    _, H, Dh = A_Wq.shape
    M, T, F = A_mem0.shape[1], int(A_seg_len), B_w1.shape[1]
    assert B == 1 and S % T == 0
    L, HD = M + T, H * Dh
    hbm = pl.BlockSpec(memory_space=pl.ANY)
    body = functools.partial(_body, S=S, D=D, H=H, Dh=Dh, M=M, T=T, F=F, G=8, BM=128, FC=128, LV=2)
    out = pl.pallas_call(
        body,
        out_shape=jax.ShapeDtypeStruct((S // T, T, D), A_x.dtype),
        in_specs=[hbm] * 11,
        out_specs=hbm,
        scratch_shapes=[
            pltpu.VMEM((3, D // 2, HD), U32), pltpu.VMEM((HD // 2, D), U32),
            pltpu.VMEM((3, S // T, _EARLY, HD), BF16),
            pltpu.VMEM((S // T, T, D), A_x.dtype), pltpu.VMEM((8, 6 * D), F32),
            pltpu.VMEM((D // _CHUNK, 8, 2 * _CHUNK), F32),
            pltpu.VMEM(((L - _EARLY) // 2, D), U32), pltpu.VMEM((L, HD), F32), pltpu.VMEM((8, 128), U32),
            pltpu.VMEM((M, D), A_mem0.dtype), pltpu.VMEM(c.shape, c.dtype),
            pltpu.SemaphoreType.DMA((4,)),
        ],
        compiler_params=pltpu.CompilerParams(
            vmem_limit_bytes=126 * 2**20, flags={'XLA_TPU_EVENLY_DISTRIBUTE_CRITICAL_NODES': True}),
    )(A_x.reshape(S // T, T, D), A_mem0.reshape(M, D),
      A_Wq, A_Wk, A_Wv, A_Wo.reshape(HD, D),
      B_w1, B_w3, B_w2, c, w_mod)
    return out.reshape(B, S, D)
```

```python
import functools

import numpy as np
import jax
import jax.numpy as jnp
from jax import lax
import jax.experimental.pallas as pl
import jax.experimental.pallas.tpu as pltpu

F32, BF16, U32 = jnp.float32, jnp.bfloat16, jnp.uint32
_EARLY, _CHUNK = 8, 256
_HIGH = np.uint32(0xFFFF0000)
_LOG2E = 1.4426950408889634
_NN = (((1,), (0,)), ((), ()))
_NT = (((1,), (1,)), ((), ()))


def _dot(a, b, dims=_NN):
    return lax.dot_general(a, b, dims, preferred_element_type=F32)


def _layernorm(x, eps=1e-5):
    m = jnp.mean(x, axis=-1, keepdims=True)
    d = x - m
    v = jnp.mean(d * d, axis=-1, keepdims=True)
    return d * lax.rsqrt(v + eps)


def _silu(x):
    h = 0.5 * x
    return h + h * jnp.tanh(h)


def _unpack(w):
    return jnp.stack([lax.bitcast_convert_type(v, F32) for v in (w << 16, w & _HIGH)])


def _pack(x):
    lo, hi = (lax.bitcast_convert_type(v.astype(BF16).astype(F32), U32) for v in (x[0], x[1]))
    return (lo >> 16) | hi


def _strassen_lhs(a, levels):
    if levels == 0:
        return [a.astype(BF16)]
    m, k = a.shape[0] // 2, a.shape[1] // 2
    a11, a12, a21, a22 = a[:m, :k], a[:m, k:], a[m:, :k], a[m:, k:]
    return [x for v in (a11 + a22, a21 + a22, a11, a22, a11 + a12, a21 - a11, a12 - a22)
            for x in _strassen_lhs(v, levels - 1)]


def _strassen_rhs(blocks):
    if len(blocks) == 1:
        return blocks
    n = len(blocks) // 4
    b11, b12, b21, b22 = (blocks[i * n:(i + 1) * n] for i in range(4))
    add = lambda x, y: [u + v for u, v in zip(x, y)]
    sub = lambda x, y: [u - v for u, v in zip(x, y)]
    return [x for v in (add(b11, b22), b11, sub(b12, b22), sub(b21, b11), b22, add(b11, b12), add(b21, b22))
            for x in _strassen_rhs(v)]


def _strassen_blocks(levels):
    out = [(0, 0, 0)]
    for _ in range(levels):
        out = [(2 * i + q // 2, 2 * j + q % 2, 7 * slot + 1 + q) for i, j, slot in out for q in range(4)]
    return out


def _strassen_out(product, levels, first=0):
    if levels == 0:
        return product(first)
    m6, m2, m4, m1, m3, m5, m7 = (_strassen_out(product, levels - 1, first + i * 7 ** (levels - 1))
                                  for i in (5, 1, 3, 0, 2, 4, 6))
    return jnp.concatenate([jnp.concatenate([m1 + m4 - m5 + m7, m3 + m5], axis=1),
                            jnp.concatenate([m2 + m4, m6 - m2 + m1 + m3], axis=1)], axis=0)


def _body(x_hbm, mem0_hbm, wq_hbm, wk_hbm, wv_hbm, wo_hbm, w1_hbm, w3_hbm, w2_hbm,
          c_hbm, wm_hbm, out_hbm,
          wqkv, wo32, pre_v, x_v, mod_v, mod1_v, hs_v, o_v, zero_v, mem0_ref, c_ref, sems,
          *, S, D, H, Dh, M, T, F, G, BM, FC, LV):
    n_seg = S // T
    L = M + T
    HD = H * Dh
    UN = 2
    P = _EARLY
    KC = _CHUNK
    n_kc = D // KC
    wo_src = wo_hbm.bitcast(U32)
    wm_src = wm_hbm.bitcast(U32)
    HP = H // 2 + 8
    CP = KC + 1
    n_it = n_seg // UN
    first_prep = n_it // 8
    XA = first_prep * UN + 1
    cp_x = pltpu.make_async_copy(x_hbm.at[pl.ds(0, XA)], x_v.at[pl.ds(0, XA)], sems.at[0])
    cp_x2 = pltpu.make_async_copy(x_hbm.at[pl.ds(XA, n_seg - XA)], x_v.at[pl.ds(XA, n_seg - XA)], sems.at[1])

    zero_v[...] = jnp.zeros(zero_v.shape, U32)

    def after(anchor):
        return pltpu.bitcast(anchor[0:8, 0:128], U32) & zero_v[...]

    def silu_c():
        return jnp.broadcast_to(_silu(c_ref[...].astype(F32)), (8, D)).astype(BF16)

    def ada1(x):
        return _layernorm(x.astype(F32)[:T - P]) * (1.0 + mod_v[0:1, D:2 * D]) + mod_v[0:1, 0:D]

    def startup(wm_v, wr_v, raw, xp_v, xn_v, hp_v, acc_v, sem_m, sem_w, sem_p):
        srcs = [w.bitcast(U32) for w in (wq_hbm, wk_hbm, wv_hbm)]
        n_j = 3 * n_kc

        def cp_w(j, t=0):
            return pltpu.make_async_copy(srcs[t].at[pl.ds((j % n_kc) * KC, KC)],
                                         raw.at[pl.ds(j * CP, KC), pl.ds(0, H // 2)], sem_w.at[j])

        def cp_m(c, i):
            return pltpu.make_async_copy(wm_src.at[:, pl.ds(pl.multiple_of(i * D + c * KC, KC), KC)],
                                         wm_v.at[c, :, pl.ds(i * KC, KC)], sem_m.at[2 * c + i])

        def start(j):
            cp_m(j, 0).start()
            cp_m(j, 1).start()
            cp_w(j).start()

        cp_r = pltpu.make_async_copy(wm_src.at[:, pl.ds(2 * D, 4 * D)], wr_v, sem_p.at[1])
        cp_o = pltpu.make_async_copy(wo_src, wo32, sem_p.at[2])
        cp_p = pltpu.make_async_copy(x_hbm.at[:, pl.ds(T - P, P), :], xp_v, sem_p.at[0])
        small = [pltpu.make_async_copy(c_hbm, c_ref, sems.at[2]),
                 pltpu.make_async_copy(mem0_hbm, mem0_ref, sems.at[3])]
        cp_p.start()
        for cp in small:
            cp.start()
        start(0)
        cp_p.wait()
        for cp in small:
            cp.wait()

        def norm(i, carry):
            xn = _layernorm(xp_v[pl.ds(i * 8, 8)].astype(F32).reshape(8 * P, D))
            for c in range(n_kc):
                xn_v[c, pl.ds(pl.multiple_of(i * 8 * P, 8 * P), 8 * P), :] = xn[:, c * KC:(c + 1) * KC]
            return carry
        lax.fori_loop(0, n_seg // 8, norm, 0)
        for j in range(1, n_j):
            if j < n_kc:
                start(j)
            else:
                cp_w(j, j // n_kc).start()
        for cp in (cp_r, cp_o, cp_x):
            cp.start()
        raw2 = raw.reshape(n_j * CP * HP, Dh)

        def chunk(j, carry):
            t, c = j // n_kc, j % n_kc

            @pl.when(j < n_kc)
            def _():
                cp_m(c, 0).wait()
                cp_m(c, 1).wait()
                mod = _dot(silu_c(), pltpu.bitcast(wm_v[c], BF16))
                mod1_v[c] = mod
                h = xn_v[c] * (1.0 + mod[0:1, KC:]) + mod[0:1, :KC]
                for i, part in enumerate(_strassen_lhs(h, 1)):
                    hp_v[c, i] = pltpu.bitcast(part, U32)

            cp_w(j).wait()

            q4 = KC // 4
            for hp in range(H // 2):
                blk = []
                for half in range(2):
                    w = _unpack(raw2[pl.ds((j * CP + half * 2 * q4) * HP + hp, 2 * q4, stride=HP), :])
                    blk += [w[0], w[1]]
                tiles = [pltpu.bitcast(v.astype(BF16), U32) for v in blk]
                cols = [slice((2 * hp + i) * Dh, (2 * hp + i + 1) * Dh) for i in range(2)]
                for i, tile in enumerate(tiles):
                    wqkv[t, pl.ds(pl.multiple_of((2 * c + i // 2) * q4, q4), q4), cols[i % 2]] = tile
                rhs = _strassen_rhs(blk)
                part = _strassen_out(lambda i: _dot(pltpu.bitcast(hp_v[c, i], BF16), rhs[i].astype(BF16)), 1)
                pair = slice(2 * hp * Dh, (2 * hp + 2) * Dh)
                part = jnp.where(c > 0, acc_v[:, pair], 0.0) + part
                acc_v[:, pair] = part
                pre_v[t, :, :, pair] = part.reshape(n_seg, P, 2 * Dh).astype(BF16)
            return carry

        lax.fori_loop(0, n_j, chunk, 0)
        for c in range(n_kc):
            mod_v[:, c * KC:(c + 1) * KC] = mod1_v[c, :, :KC]
            mod_v[:, D + c * KC:D + (c + 1) * KC] = mod1_v[c, :, KC:]
        cp_r.wait()
        mod_v[:, 2 * D:6 * D] = _dot(silu_c(), pltpu.bitcast(wr_v[...], BF16))
        cp_o.wait()

    pl.run_scoped(startup,
                  pltpu.VMEM((n_kc, D // 2, 2 * KC), U32), pltpu.VMEM((D // 2, 4 * D), U32),
                  pltpu.VMEM((3 * n_kc * CP, HP, Dh), U32),
                  pltpu.VMEM((n_seg, P, D), x_hbm.dtype), pltpu.VMEM((n_kc, n_seg * P, KC), F32),
                  pltpu.VMEM((n_kc, 7, n_seg * P // 4, KC // 2), U32), pltpu.VMEM((n_seg * P, HD), F32),
                  pltpu.SemaphoreType.DMA((2 * n_kc,)), pltpu.SemaphoreType.DMA((3 * n_kc,)),
                  pltpu.SemaphoreType.DMA((3,)))

    ffn_cfg = ((w1_hbm, LV), (w3_hbm, LV), (w2_hbm, LV))

    def main(e1_v, e3_v, e2_v, h2_v, sem_f, sem_y):
        cp_f, pieces = [], []
        for (src, lv), e in zip(ffn_cfg, (e1_v, e3_v, e2_v)):
            R, n = e.shape[1] - 8, e.shape[2]
            for bi, bj, slot in _strassen_blocks(lv):
                cp_f.append(pltpu.make_async_copy(src.bitcast(U32).at[pl.ds(bi * R, R), pl.ds(bj * n, n)],
                                                  e.at[slot, pl.ds(0, R)], sem_f.at[len(cp_f)]))
                e[slot, R:R + 8, 0:128] = jnp.zeros((8, 128), U32)
            per_it = pl.cdiv(R // 8 * (n // 128), n_it - first_prep)
            groups = [range(7)] if lv == 1 else [range(7 * o, 7 * o + 7) for o in (0, 5, 6, 2, 3, 1, 4)]
            pieces += [(e, lv, per_it, u, grp) for u in range(per_it) for grp in groups]

        def prep_ffn(i, site, n_sites, anchor):
            per = pl.cdiv(len(pieces), n_sites)
            for k, (e, lv, per_it, u, grp) in enumerate(pieces[site * per:(site + 1) * per]):
                tie = after(anchor[:, (k * 128) % anchor.shape[1]:])
                n_r, n_c = e.shape[1] // 8 - 1, e.shape[2] // 128
                pos = jnp.maximum(i - first_prep, 0) * per_it + u
                live = (i >= first_prep) & (pos < n_r * n_c)
                rows = pl.ds(pl.multiple_of(jnp.where(live, lax.rem(pos, n_r), n_r) * 8, 8), 8)
                cols = pl.ds(pl.multiple_of(jnp.where(live, lax.div(pos, n_r), 0) * 128, 128), 128)
                blocks = [_unpack(e[slot, rows, cols] | tie) for _, _, slot in _strassen_blocks(lv)]
                for slot, w in enumerate(_strassen_rhs(blocks)):
                    if slot in grp and not any(w is blk for blk in blocks):
                        e[slot, rows, cols] = _pack(w)

        cp_x.wait()
        cp_x2.start()
        for cp in cp_f:
            cp.start()
        hs_v[...] = pltpu.bitcast(
            jnp.concatenate([mem0_ref[...].astype(F32), ada1(x_v[0])], axis=0).astype(BF16), U32)
        scale = Dh ** -0.5
        n_g = H // G

        def step(s, side):
            ri = lax.broadcasted_iota(jnp.int32, (2 * L, 2 * L), 0)
            ci = lax.broadcasted_iota(jnp.int32, (2 * L, 2 * L), 1)
            same = (ri >= L) == (ci >= L)
            rl = jnp.where(ri >= L, ri - L, ri)
            cl = jnp.where(ci >= L, ci - L, ci)
            keep = same & ((rl < M) | (rl >= cl))
            fill = jnp.where(same, -1e9 / scale, -jnp.inf).astype(F32)

            def gcols(g):
                return slice(g * G * Dh, (g + 1) * G * Dh)

            def proj(t, g):
                return _dot(pltpu.bitcast(hs_v[...], BF16), pltpu.bitcast(wqkv[t, :, gcols(g)], BF16))

            def stack(a, t, g, p):
                hp = g * G // 2 + p
                pre = pre_v[t, s, :, 2 * hp * Dh:(2 * hp + 2) * Dh].astype(F32)
                return jnp.concatenate([a[:, (2 * p) * Dh:(2 * p + 1) * Dh], pre[:, :Dh],
                                        a[:, (2 * p + 1) * Dh:(2 * p + 2) * Dh], pre[:, Dh:]], axis=0).astype(BF16)

            def scores(g, q, k):
                res = []
                for p in range(G // 2):
                    sc = jnp.where(keep, _dot(stack(q, 0, g, p), stack(k, 1, g, p), _NT), fill)
                    e = jnp.exp2((sc - jnp.max(sc, axis=-1, keepdims=True)) * (scale * _LOG2E))
                    den = jnp.sum(e, axis=-1, keepdims=True)
                    r = pl.reciprocal(den, approx=True)
                    res.append((e.astype(BF16), r * (2.0 - den * r)))
                return res

            def values(g, res, v):
                for p, (e, inv) in enumerate(res):
                    o = _dot(e, stack(v, 2, g, p)) * inv
                    h0 = g * G + 2 * p
                    o_v[:, h0 * Dh:(h0 + 1) * Dh] = o[0:L]
                    o_v[:, (h0 + 1) * Dh:(h0 + 2) * Dh] = o[L:2 * L]

            def outp(g):
                return _dot(o_v[:, gcols(g)],
                            pltpu.bitcast(wo32[g * G * Dh // 2:(g + 1) * G * Dh // 2, :], BF16))

            h_next = ada1(x_v[jnp.minimum(s + 1, n_seg - 1)])
            qk, sm, vv = {}, {}, {}
            for g in range(n_g):
                q = proj(0, g)
                if g >= 1:
                    sm[g - 1] = scores(g - 1, *qk.pop(g - 1))
                qk[g] = q, proj(1, g)
            for g in range(n_g):
                vv[g] = proj(2, g)
                side(g, vv[g])
                if g == 0:
                    sm[n_g - 1] = scores(n_g - 1, *qk.pop(n_g - 1))
                else:
                    values(g - 1, sm.pop(g - 1), vv.pop(g - 1))
            acc = outp(0)
            values(n_g - 1, sm.pop(n_g - 1), vv.pop(n_g - 1))
            for g in range(1, n_g):
                side(n_g - 1 + g, acc)
                acc = acc + outp(g)
            hs_v[...] = pltpu.bitcast(jnp.concatenate([acc[0:M], h_next], axis=0).astype(BF16), U32)
            x_v[s] = (x_v[s].astype(F32) + mod_v[0:1, 2 * D:3 * D] * acc[M:L]).astype(x_v.dtype)

        def steps(i, carry):
            for j in range(UN):
                per = 2 * n_g - 1
                step(i * UN + j, lambda k, anchor, j=j: prep_ffn(i, j * per + k, UN * per, anchor))
            return carry

        def phase(ph, carry):
            @pl.when(ph == 1)
            def _():
                cp_x2.wait()
                for cp in cp_f:
                    cp.wait()
            return lax.fori_loop(ph * first_prep, jnp.where(ph == 0, first_prep, n_it), steps, carry)

        lax.fori_loop(0, 2, phase, 0)

        def resid(i):
            return x_v[pl.ds(i * (BM // T), BM // T)].astype(F32).reshape(BM, D)

        def ada2(i):
            h2 = _layernorm(resid(i)) * (1.0 + mod_v[0:1, 4 * D:5 * D]) + mod_v[0:1, 3 * D:4 * D]
            return _strassen_lhs(h2, LV)

        def matmul(lhs, e, cols=slice(None)):
            return _strassen_out(lambda k: _dot(lhs[k], pltpu.bitcast(e[k, 0:e.shape[1] - 8, cols], BF16)), LV)

        def put_h2(parts):
            for j, part in enumerate(parts):
                h2_v[j] = part

        put_h2(ada2(0))

        def out_copy(i):
            r = pl.ds(i * (BM // T), BM // T)
            return pltpu.make_async_copy(x_v.at[r], out_hbm.at[r], sem_y.at[i])

        def ffn(i, carry):
            h2_next = ada2(jnp.minimum(i + 1, S // BM - 1))
            acts = []
            for c0 in range(0, e1_v.shape[2], FC):
                cols = slice(c0, c0 + FC)
                gate, up = [matmul([h2_v[j] for j in range(7 ** LV)], e, cols)
                            for e in (e1_v, e3_v)]
                act = _silu(gate) * up
                acts.append(_strassen_lhs(act, LV))
            put_h2(h2_next)
            ffn_out = matmul([jnp.concatenate(parts, axis=1) for parts in zip(*acts)], e2_v)
            y = resid(i) + mod_v[0:1, 5 * D:6 * D] * ffn_out
            x_v[pl.ds(i * (BM // T), BM // T)] = y.reshape(BM // T, T, D).astype(x_v.dtype)
            out_copy(i).start()
            return carry

        lax.fori_loop(0, S // BM, ffn, 0)
        for i in range(S // BM):
            out_copy(i).wait()

    pl.run_scoped(main,
                  *[pltpu.VMEM((7 ** lv, (w.shape[0] >> (lv + 1)) + 8, w.shape[1] >> lv), U32)
                    for w, lv in ffn_cfg],
                  pltpu.VMEM((7 ** LV, BM >> LV, D >> LV), BF16),
                  pltpu.SemaphoreType.DMA((sum(4 ** lv for _, lv in ffn_cfg),)),
                  pltpu.SemaphoreType.DMA((S // BM,)))


@functools.partial(jax.jit, static_argnames=("A_seg_len",))
def pallas_adaLN_cond__memory_aug_recurrent_mem_tr__glu_gated_swiglu__prompt_kernel(
    A_x, A_mem0, A_Wq, A_Wk, A_Wv, A_Wo, A_seg_len, B_x, B_w1, B_w3, B_w2, c, w_mod,
):
    del B_x
    B, S, D = A_x.shape
    _, H, Dh = A_Wq.shape
    M, T, F = A_mem0.shape[1], int(A_seg_len), B_w1.shape[1]
    assert B == 1 and S % T == 0
    L, HD = M + T, H * Dh
    hbm = pl.BlockSpec(memory_space=pl.ANY)
    body = functools.partial(_body, S=S, D=D, H=H, Dh=Dh, M=M, T=T, F=F, G=8, BM=128, FC=128, LV=2)
    out = pl.pallas_call(
        body,
        out_shape=jax.ShapeDtypeStruct((S // T, T, D), A_x.dtype),
        in_specs=[hbm] * 11,
        out_specs=hbm,
        scratch_shapes=[
            pltpu.VMEM((3, D // 2, HD), U32), pltpu.VMEM((HD // 2, D), U32),
            pltpu.VMEM((3, S // T, _EARLY, HD), BF16),
            pltpu.VMEM((S // T, T, D), A_x.dtype), pltpu.VMEM((8, 6 * D), F32),
            pltpu.VMEM((D // _CHUNK, 8, 2 * _CHUNK), F32),
            pltpu.VMEM(((L - _EARLY) // 2, D), U32), pltpu.VMEM((L, HD), F32), pltpu.VMEM((8, 128), U32),
            pltpu.VMEM((M, D), A_mem0.dtype), pltpu.VMEM(c.shape, c.dtype),
            pltpu.SemaphoreType.DMA((4,)),
        ],
        compiler_params=pltpu.CompilerParams(
            vmem_limit_bytes=126 * 2**20, flags={'XLA_TPU_EVENLY_DISTRIBUTE_CRITICAL_NODES': True}),
    )(A_x.reshape(S // T, T, D), A_mem0.reshape(M, D),
      A_Wq, A_Wk, A_Wv, A_Wo.reshape(HD, D),
      B_w1, B_w3, B_w2, c, w_mod)
    return out.reshape(B, S, D)
```

```python
import functools

import numpy as np
import jax
import jax.numpy as jnp
from jax import lax
import jax.experimental.pallas as pl
import jax.experimental.pallas.tpu as pltpu

F32, BF16, U32 = jnp.float32, jnp.bfloat16, jnp.uint32
_EARLY, _CHUNK = 8, 256
_HIGH = np.uint32(0xFFFF0000)
_LOG2E = 1.4426950408889634
_NN = (((1,), (0,)), ((), ()))
_NT = (((1,), (1,)), ((), ()))


def _dot(a, b, dims=_NN):
    return lax.dot_general(a, b, dims, preferred_element_type=F32)


def _layernorm(x, eps=1e-5):
    m = jnp.mean(x, axis=-1, keepdims=True)
    d = x - m
    v = jnp.mean(d * d, axis=-1, keepdims=True)
    return d * lax.rsqrt(v + eps)


def _silu(x):
    h = 0.5 * x
    return h + h * jnp.tanh(h)


def _unpack(w):
    return jnp.stack([lax.bitcast_convert_type(v, F32) for v in (w << 16, w & _HIGH)])


def _pack(x):
    lo, hi = (lax.bitcast_convert_type(v.astype(BF16).astype(F32), U32) for v in (x[0], x[1]))
    return (lo >> 16) | hi


def _strassen_lhs(a, levels):
    if levels == 0:
        return [a.astype(BF16)]
    m, k = a.shape[0] // 2, a.shape[1] // 2
    a11, a12, a21, a22 = a[:m, :k], a[:m, k:], a[m:, :k], a[m:, k:]
    return [x for v in (a11 + a22, a21 + a22, a11, a22, a11 + a12, a21 - a11, a12 - a22)
            for x in _strassen_lhs(v, levels - 1)]


def _strassen_rhs(blocks):
    if len(blocks) == 1:
        return blocks
    n = len(blocks) // 4
    b11, b12, b21, b22 = (blocks[i * n:(i + 1) * n] for i in range(4))
    add = lambda x, y: [u + v for u, v in zip(x, y)]
    sub = lambda x, y: [u - v for u, v in zip(x, y)]
    return [x for v in (add(b11, b22), b11, sub(b12, b22), sub(b21, b11), b22, add(b11, b12), add(b21, b22))
            for x in _strassen_rhs(v)]


def _strassen_blocks(levels):
    out = [(0, 0, 0)]
    for _ in range(levels):
        out = [(2 * i + q // 2, 2 * j + q % 2, 7 * slot + 1 + q) for i, j, slot in out for q in range(4)]
    return out


def _strassen_out(product, levels, first=0):
    if levels == 0:
        return product(first)
    m6, m2, m4, m1, m3, m5, m7 = (_strassen_out(product, levels - 1, first + i * 7 ** (levels - 1))
                                  for i in (5, 1, 3, 0, 2, 4, 6))
    return jnp.concatenate([jnp.concatenate([m1 + m4 - m5 + m7, m3 + m5], axis=1),
                            jnp.concatenate([m2 + m4, m6 - m2 + m1 + m3], axis=1)], axis=0)


def _body(x_hbm, mem0_hbm, wq_hbm, wk_hbm, wv_hbm, wo_hbm, w1_hbm, w3_hbm, w2_hbm,
          c_hbm, wm_hbm, out_hbm,
          wqkv, wo32, pre_v, x_v, mod_v, mod1_v, hs_v, o_v, zero_v, mem0_ref, c_ref, sems,
          *, S, D, H, Dh, M, T, F, G, BM, FC, LV):
    n_seg = S // T
    L = M + T
    HD = H * Dh
    UN = 2
    P = _EARLY
    KC = _CHUNK
    n_kc = D // KC
    wo_src = wo_hbm.bitcast(U32)
    wm_src = wm_hbm.bitcast(U32)
    HP = H // 2 + 8
    CP = KC + 1
    n_it = n_seg // UN
    first_prep = n_it // 8
    XA = first_prep * UN + 1
    cp_x = pltpu.make_async_copy(x_hbm.at[pl.ds(0, XA)], x_v.at[pl.ds(0, XA)], sems.at[0])
    cp_x2 = pltpu.make_async_copy(x_hbm.at[pl.ds(XA, n_seg - XA)], x_v.at[pl.ds(XA, n_seg - XA)], sems.at[1])

    zero_v[...] = jnp.zeros(zero_v.shape, U32)

    def after(anchor):
        return pltpu.bitcast(anchor[0:8, 0:128], U32) & zero_v[...]

    def silu_c():
        return jnp.broadcast_to(_silu(c_ref[...].astype(F32)), (8, D)).astype(BF16)

    def ada1(x):
        return _layernorm(x.astype(F32)[:T - P]) * (1.0 + mod_v[0:1, D:2 * D]) + mod_v[0:1, 0:D]

    def startup(wm_v, wr_v, raw, xp_v, xn_v, hp_v, acc_v, sem_m, sem_w, sem_p):
        srcs = [w.bitcast(U32) for w in (wq_hbm, wk_hbm, wv_hbm)]
        n_j = 3 * n_kc

        def cp_w(j, t=0):
            return pltpu.make_async_copy(srcs[t].at[pl.ds((j % n_kc) * KC, KC)],
                                         raw.at[pl.ds(j * CP, KC), pl.ds(0, H // 2)], sem_w.at[j])

        def cp_m(c, i):
            return pltpu.make_async_copy(wm_src.at[:, pl.ds(pl.multiple_of(i * D + c * KC, KC), KC)],
                                         wm_v.at[c, :, pl.ds(i * KC, KC)], sem_m.at[2 * c + i])

        def start(j):
            cp_m(j, 0).start()
            cp_m(j, 1).start()
            cp_w(j).start()

        cp_r = pltpu.make_async_copy(wm_src.at[:, pl.ds(2 * D, 4 * D)], wr_v, sem_p.at[1])
        cp_o = pltpu.make_async_copy(wo_src, wo32, sem_p.at[2])
        cp_p = pltpu.make_async_copy(x_hbm.at[:, pl.ds(T - P, P), :], xp_v, sem_p.at[0])
        small = [pltpu.make_async_copy(c_hbm, c_ref, sems.at[2]),
                 pltpu.make_async_copy(mem0_hbm, mem0_ref, sems.at[3])]
        cp_p.start()
        for cp in small:
            cp.start()
        start(0)
        cp_p.wait()
        for cp in small:
            cp.wait()

        def norm(i, carry):
            xn = _layernorm(xp_v[pl.ds(i * 8, 8)].astype(F32).reshape(8 * P, D))
            for c in range(n_kc):
                xn_v[c, pl.ds(pl.multiple_of(i * 8 * P, 8 * P), 8 * P), :] = xn[:, c * KC:(c + 1) * KC]
            return carry
        lax.fori_loop(0, n_seg // 8, norm, 0)
        for j in range(1, n_j):
            if j < n_kc:
                start(j)
            else:
                cp_w(j, j // n_kc).start()
        for cp in (cp_r, cp_o, cp_x):
            cp.start()
        raw2 = raw.reshape(n_j * CP * HP, Dh)

        def chunk(j, carry):
            t, c = j // n_kc, j % n_kc

            @pl.when(j < n_kc)
            def _():
                cp_m(c, 0).wait()
                cp_m(c, 1).wait()
                mod = _dot(silu_c(), pltpu.bitcast(wm_v[c], BF16))
                mod1_v[c] = mod
                half = n_seg * P // 2
                for r in range(0, half, 16):
                    xn = jnp.concatenate([xn_v[c, r:r + 16], xn_v[c, half + r:half + r + 16]], axis=0)
                    h = xn * (1.0 + mod[0:1, KC:]) + mod[0:1, :KC]
                    for i, part in enumerate(_strassen_lhs(h, 1)):
                        hp_v[c, i, r // 2:r // 2 + 8] = pltpu.bitcast(part, U32)

            cp_w(j).wait()

            q4 = KC // 4
            for hp in range(H // 2):
                blk = []
                for half in range(2):
                    w = _unpack(raw2[pl.ds((j * CP + half * 2 * q4) * HP + hp, 2 * q4, stride=HP), :])
                    blk += [w[0], w[1]]
                tiles = [pltpu.bitcast(v.astype(BF16), U32) for v in blk]
                cols = [slice((2 * hp + i) * Dh, (2 * hp + i + 1) * Dh) for i in range(2)]
                for i, tile in enumerate(tiles):
                    wqkv[t, pl.ds(pl.multiple_of((2 * c + i // 2) * q4, q4), q4), cols[i % 2]] = tile
                rhs = _strassen_rhs(blk)
                part = _strassen_out(lambda i: _dot(pltpu.bitcast(hp_v[c, i], BF16), rhs[i].astype(BF16)), 1)
                pair = slice(2 * hp * Dh, (2 * hp + 2) * Dh)
                part = jnp.where(c > 0, acc_v[:, pair], 0.0) + part
                acc_v[:, pair] = part
                pre_v[t, :, :, pair] = part.reshape(n_seg, P, 2 * Dh).astype(BF16)
            return carry

        lax.fori_loop(0, n_j, chunk, 0)
        for c in range(n_kc):
            mod_v[:, c * KC:(c + 1) * KC] = mod1_v[c, :, :KC]
            mod_v[:, D + c * KC:D + (c + 1) * KC] = mod1_v[c, :, KC:]
        cp_r.wait()
        mod_v[:, 2 * D:6 * D] = _dot(silu_c(), pltpu.bitcast(wr_v[...], BF16))
        cp_o.wait()

    pl.run_scoped(startup,
                  pltpu.VMEM((n_kc, D // 2, 2 * KC), U32), pltpu.VMEM((D // 2, 4 * D), U32),
                  pltpu.VMEM((3 * n_kc * CP, HP, Dh), U32),
                  pltpu.VMEM((n_seg, P, D), x_hbm.dtype), pltpu.VMEM((n_kc, n_seg * P, KC), F32),
                  pltpu.VMEM((n_kc, 7, n_seg * P // 4, KC // 2), U32), pltpu.VMEM((n_seg * P, HD), F32),
                  pltpu.SemaphoreType.DMA((2 * n_kc,)), pltpu.SemaphoreType.DMA((3 * n_kc,)),
                  pltpu.SemaphoreType.DMA((3,)))

    ffn_cfg = ((w1_hbm, LV), (w3_hbm, LV), (w2_hbm, LV))

    def main(e1_v, e3_v, e2_v, h2_v, sem_f, sem_y):
        cp_f, pieces = [], []
        for (src, lv), e in zip(ffn_cfg, (e1_v, e3_v, e2_v)):
            R, n = e.shape[1] - 8, e.shape[2]
            for bi, bj, slot in _strassen_blocks(lv):
                cp_f.append(pltpu.make_async_copy(src.bitcast(U32).at[pl.ds(bi * R, R), pl.ds(bj * n, n)],
                                                  e.at[slot, pl.ds(0, R)], sem_f.at[len(cp_f)]))
                e[slot, R:R + 8, 0:128] = jnp.zeros((8, 128), U32)
            per_it = pl.cdiv(R // 8 * (n // 128), n_it - first_prep)
            groups = [range(7)] if lv == 1 else [range(7 * o, 7 * o + 7) for o in (0, 5, 6, 2, 3, 1, 4)]
            pieces += [(e, lv, per_it, u, grp) for u in range(per_it) for grp in groups]

        def prep_ffn(i, site, n_sites, anchor):
            per = pl.cdiv(len(pieces), n_sites)
            for k, (e, lv, per_it, u, grp) in enumerate(pieces[site * per:(site + 1) * per]):
                tie = after(anchor[:, (k * 128) % anchor.shape[1]:])
                n_r, n_c = e.shape[1] // 8 - 1, e.shape[2] // 128
                pos = jnp.maximum(i - first_prep, 0) * per_it + u
                live = (i >= first_prep) & (pos < n_r * n_c)
                rows = pl.ds(pl.multiple_of(jnp.where(live, lax.rem(pos, n_r), n_r) * 8, 8), 8)
                cols = pl.ds(pl.multiple_of(jnp.where(live, lax.div(pos, n_r), 0) * 128, 128), 128)
                blocks = [_unpack(e[slot, rows, cols] | tie) for _, _, slot in _strassen_blocks(lv)]
                for slot, w in enumerate(_strassen_rhs(blocks)):
                    if slot in grp and not any(w is blk for blk in blocks):
                        e[slot, rows, cols] = _pack(w)

        cp_x.wait()
        cp_x2.start()
        for cp in cp_f:
            cp.start()
        hs_v[...] = pltpu.bitcast(
            jnp.concatenate([mem0_ref[...].astype(F32), ada1(x_v[0])], axis=0).astype(BF16), U32)
        scale = Dh ** -0.5
        n_g = H // G

        def step(s, side):
            ri = lax.broadcasted_iota(jnp.int32, (2 * L, 2 * L), 0)
            ci = lax.broadcasted_iota(jnp.int32, (2 * L, 2 * L), 1)
            same = (ri >= L) == (ci >= L)
            rl = jnp.where(ri >= L, ri - L, ri)
            cl = jnp.where(ci >= L, ci - L, ci)
            keep = same & ((rl < M) | (rl >= cl))
            fill = jnp.where(same, -1e9 / scale, -jnp.inf).astype(F32)

            def gcols(g):
                return slice(g * G * Dh, (g + 1) * G * Dh)

            def proj(t, g):
                return _dot(pltpu.bitcast(hs_v[...], BF16), pltpu.bitcast(wqkv[t, :, gcols(g)], BF16))

            def stack(a, t, g, p):
                hp = g * G // 2 + p
                pre = pre_v[t, s, :, 2 * hp * Dh:(2 * hp + 2) * Dh].astype(F32)
                return jnp.concatenate([a[:, (2 * p) * Dh:(2 * p + 1) * Dh], pre[:, :Dh],
                                        a[:, (2 * p + 1) * Dh:(2 * p + 2) * Dh], pre[:, Dh:]], axis=0).astype(BF16)

            def scores(g, q, k):
                res = []
                for p in range(G // 2):
                    sc = jnp.where(keep, _dot(stack(q, 0, g, p), stack(k, 1, g, p), _NT), fill)
                    e = jnp.exp2((sc - jnp.max(sc, axis=-1, keepdims=True)) * (scale * _LOG2E))
                    den = jnp.sum(e, axis=-1, keepdims=True)
                    r = pl.reciprocal(den, approx=True)
                    res.append((e.astype(BF16), r * (2.0 - den * r)))
                return res

            def values(g, res, v):
                for p, (e, inv) in enumerate(res):
                    o = _dot(e, stack(v, 2, g, p)) * inv
                    h0 = g * G + 2 * p
                    o_v[:, h0 * Dh:(h0 + 1) * Dh] = o[0:L]
                    o_v[:, (h0 + 1) * Dh:(h0 + 2) * Dh] = o[L:2 * L]

            def outp(g):
                return _dot(o_v[:, gcols(g)],
                            pltpu.bitcast(wo32[g * G * Dh // 2:(g + 1) * G * Dh // 2, :], BF16))

            h_next = ada1(x_v[jnp.minimum(s + 1, n_seg - 1)])
            qk, sm, vv = {}, {}, {}
            for g in range(n_g):
                q = proj(0, g)
                if g >= 1:
                    sm[g - 1] = scores(g - 1, *qk.pop(g - 1))
                qk[g] = q, proj(1, g)
            for g in range(n_g):
                vv[g] = proj(2, g)
                side(g, vv[g])
                if g == 0:
                    sm[n_g - 1] = scores(n_g - 1, *qk.pop(n_g - 1))
                else:
                    values(g - 1, sm.pop(g - 1), vv.pop(g - 1))
            acc = outp(0)
            values(n_g - 1, sm.pop(n_g - 1), vv.pop(n_g - 1))
            for g in range(1, n_g):
                side(n_g - 1 + g, acc)
                acc = acc + outp(g)
            hs_v[...] = pltpu.bitcast(jnp.concatenate([acc[0:M], h_next], axis=0).astype(BF16), U32)
            x_v[s] = (x_v[s].astype(F32) + mod_v[0:1, 2 * D:3 * D] * acc[M:L]).astype(x_v.dtype)

        def steps(i, carry):
            for j in range(UN):
                per = 2 * n_g - 1
                step(i * UN + j, lambda k, anchor, j=j: prep_ffn(i, j * per + k, UN * per, anchor))
            return carry

        def phase(ph, carry):
            @pl.when(ph == 1)
            def _():
                cp_x2.wait()
                for cp in cp_f:
                    cp.wait()
            return lax.fori_loop(ph * first_prep, jnp.where(ph == 0, first_prep, n_it), steps, carry)

        lax.fori_loop(0, 2, phase, 0)

        def resid(i):
            return x_v[pl.ds(i * (BM // T), BM // T)].astype(F32).reshape(BM, D)

        def ada2(i):
            h2 = _layernorm(resid(i)) * (1.0 + mod_v[0:1, 4 * D:5 * D]) + mod_v[0:1, 3 * D:4 * D]
            return _strassen_lhs(h2, LV)

        def matmul(lhs, e, cols=slice(None)):
            return _strassen_out(lambda k: _dot(lhs[k], pltpu.bitcast(e[k, 0:e.shape[1] - 8, cols], BF16)), LV)

        def put_h2(parts):
            for j, part in enumerate(parts):
                h2_v[j] = part

        put_h2(ada2(0))

        def out_copy(i):
            r = pl.ds(i * (BM // T), BM // T)
            return pltpu.make_async_copy(x_v.at[r], out_hbm.at[r], sem_y.at[i])

        def ffn(i, carry):
            h2_next = ada2(jnp.minimum(i + 1, S // BM - 1))
            acts = []
            for c0 in range(0, e1_v.shape[2], FC):
                cols = slice(c0, c0 + FC)
                gate, up = [matmul([h2_v[j] for j in range(7 ** LV)], e, cols)
                            for e in (e1_v, e3_v)]
                act = _silu(gate) * up
                acts.append(_strassen_lhs(act, LV))
            put_h2(h2_next)
            ffn_out = matmul([jnp.concatenate(parts, axis=1) for parts in zip(*acts)], e2_v)
            y = resid(i) + mod_v[0:1, 5 * D:6 * D] * ffn_out
            x_v[pl.ds(i * (BM // T), BM // T)] = y.reshape(BM // T, T, D).astype(x_v.dtype)
            out_copy(i).start()
            return carry

        lax.fori_loop(0, S // BM, ffn, 0)
        for i in range(S // BM):
            out_copy(i).wait()

    pl.run_scoped(main,
                  *[pltpu.VMEM((7 ** lv, (w.shape[0] >> (lv + 1)) + 8, w.shape[1] >> lv), U32)
                    for w, lv in ffn_cfg],
                  pltpu.VMEM((7 ** LV, BM >> LV, D >> LV), BF16),
                  pltpu.SemaphoreType.DMA((sum(4 ** lv for _, lv in ffn_cfg),)),
                  pltpu.SemaphoreType.DMA((S // BM,)))


@functools.partial(jax.jit, static_argnames=("A_seg_len",))
def pallas_adaLN_cond__memory_aug_recurrent_mem_tr__glu_gated_swiglu__prompt_kernel(
    A_x, A_mem0, A_Wq, A_Wk, A_Wv, A_Wo, A_seg_len, B_x, B_w1, B_w3, B_w2, c, w_mod,
):
    del B_x
    B, S, D = A_x.shape
    _, H, Dh = A_Wq.shape
    M, T, F = A_mem0.shape[1], int(A_seg_len), B_w1.shape[1]
    assert B == 1 and S % T == 0
    L, HD = M + T, H * Dh
    hbm = pl.BlockSpec(memory_space=pl.ANY)
    body = functools.partial(_body, S=S, D=D, H=H, Dh=Dh, M=M, T=T, F=F, G=8, BM=128, FC=128, LV=2)
    out = pl.pallas_call(
        body,
        out_shape=jax.ShapeDtypeStruct((S // T, T, D), A_x.dtype),
        in_specs=[hbm] * 11,
        out_specs=hbm,
        scratch_shapes=[
            pltpu.VMEM((3, D // 2, HD), U32), pltpu.VMEM((HD // 2, D), U32),
            pltpu.VMEM((3, S // T, _EARLY, HD), BF16),
            pltpu.VMEM((S // T, T, D), A_x.dtype), pltpu.VMEM((8, 6 * D), F32),
            pltpu.VMEM((D // _CHUNK, 8, 2 * _CHUNK), F32),
            pltpu.VMEM(((L - _EARLY) // 2, D), U32), pltpu.VMEM((L, HD), F32), pltpu.VMEM((8, 128), U32),
            pltpu.VMEM((M, D), A_mem0.dtype), pltpu.VMEM(c.shape, c.dtype),
            pltpu.SemaphoreType.DMA((4,)),
        ],
        compiler_params=pltpu.CompilerParams(
            vmem_limit_bytes=126 * 2**20, flags={'XLA_TPU_EVENLY_DISTRIBUTE_CRITICAL_NODES': True}),
    )(A_x.reshape(S // T, T, D), A_mem0.reshape(M, D),
      A_Wq, A_Wk, A_Wv, A_Wo.reshape(HD, D),
      B_w1, B_w3, B_w2, c, w_mod)
    return out.reshape(B, S, D)
```
